```python
import jax
import jax.numpy as jnp

def _softmax(x, axis=-1):
    return jax.nn.softmax(x, axis=axis)
def _gelu(x):
    return jax.nn.gelu(x, approximate=True)
def _silu(x):
    return jax.nn.silu(x)
def _sigmoid(x):
    return jax.nn.sigmoid(x)
def _layernorm(x, axis=-1, eps=1e-5):
    m = jnp.mean(x, axis=axis, keepdims=True)
    v = jnp.var(x, axis=axis, keepdims=True)
    return (x - m) / jnp.sqrt(v + eps)
def _scatter_add(tgt, idx, src, axis=0):
    return tgt.at[idx].add(src)
def _segment_sum(src, seg, n):
    return jax.ops.segment_sum(src, seg, n)
class _Rng:
    def __init__(self, key):
        self._k = key
    def _next(self):
        self._k, sub = jax.random.split(self._k)
        return sub
    def normal(self, shape):
        return jax.random.normal(self._next(), shape, dtype=jnp.bfloat16)
    def randint(self, lo, hi, shape):
        return jax.random.randint(self._next(), shape, lo, hi, dtype=jnp.int32)
    def uniform(self, shape, lo=0.0, hi=1.0):
        return jax.random.uniform(self._next(), shape, jnp.bfloat16, lo, hi)
    def permutation(self, n):
        return jax.random.permutation(self._next(), n)


kernel_name = 'gated_mix__sliding_local_dilated__glu_gated_reglu__prompt'

def setup_inputs():
    _rng = _Rng(jax.random.key(int.from_bytes(__import__("os").urandom(4), "little")))
    _w = (lambda a: (lambda t: t.astype(jnp.bfloat16) if jnp.issubdtype(t.dtype, jnp.floating) else t)(jnp.asarray(a)))
    def _A_setup():
        B, S, D = 1, 2048, 1024
        return {
            "x": _w((lambda *s: _rng.normal(s) * 0.05)(B, S, D)),
            "wqkv": _w((lambda *s: _rng.normal(s) * 0.05)(D, 3 * D)),
            "wo": _w((lambda *s: _rng.normal(s) * 0.05)(D, D)),
        }
    _A_in = _A_setup()

    def _B_setup():
        B, S, D, F = 1, 2048, 1024, 3584
        return {
            "x": _w((lambda *s: _rng.normal(s) * 0.05)(B, S, D)),
            "W_gate": _w((lambda *s: _rng.normal(s) * 0.05)(D, F) * (2.0 / D) ** 0.5),
            "W_up": _w((lambda *s: _rng.normal(s) * 0.05)(D, F) * (2.0 / D) ** 0.5),
            "W_down": _w((lambda *s: _rng.normal(s) * 0.05)(F, D) * (1.0 / F) ** 0.5),
        }
    _B_in = _B_setup()

    return {
        "A_x": _A_in["x"],
        "A_wqkv": _A_in["wqkv"],
        "A_wo": _A_in["wo"],
        "B_x": _B_in["x"],
        "B_W_gate": _B_in["W_gate"],
        "B_W_up": _B_in["W_up"],
        "B_W_down": _B_in["W_down"],
        "gate_w": _w((lambda *s: _rng.normal(s) * 0.05)(1024)),
    }

def reference(A_x, A_wqkv, A_wo, B_x, B_W_gate, B_W_up, B_W_down, gate_w):
    def _A_ref(x, wqkv, wo):
        B, S, D = x.shape
        H = 32; Dh = D // H
        W, dil = 8, 2
        qkv = (lambda x, *d: x.transpose(*d))((x @ wqkv).reshape(B, S, 3, H, Dh), 2, 0, 3, 1, 4)
        q, k, v = qkv[0], qkv[1], qkv[2]
        scale = Dh ** -0.5
        pos = jnp.arange(S)
        off = jnp.arange(W) * dil
        idx = pos[:, None] - off[None, :]
        mask = idx >= 0
        idx_c = jnp.where(mask, idx, 0).reshape(-1)
        kg = k[:, :, idx_c, :].reshape(B, H, S, W, Dh)
        vg = v[:, :, idx_c, :].reshape(B, H, S, W, Dh)
        logits = jnp.einsum("bhsd,bhswd->bhsw", q, kg) * scale
        logits = jnp.where(mask[None, None, :, :], logits, -1e9)
        attn = _softmax(logits, axis=-1)
        o = jnp.einsum("bhsw,bhswd->bhsd", attn, vg)
        return (lambda x, *d: x.transpose(*d))(o, 0, 2, 1, 3).reshape(B, S, D) @ wo

    def _B_ref(x, W_gate, W_up, W_down):
        gate = jnp.einsum("bsd,df->bsf", x, W_gate)
        up = jnp.einsum("bsd,df->bsf", x, W_up)
        gate = gate * (lambda x, dt: x.astype(dt))(gate > 0, gate.dtype)
        h = gate * up
        return jnp.einsum("bsf,fd->bsd", h, W_down)

    x = A_x
    g = _sigmoid((x * gate_w).sum(-1, keepdims=True))
    a = _A_ref(x, A_wqkv, A_wo)
    b = _B_ref(x, B_W_gate, B_W_up, B_W_down)
    return g * a + (1 - g) * b
```

```python
import jax
import jax.numpy as jnp
import jax.experimental.pallas as pl
import jax.experimental.pallas.tpu as pltpu

S, D, F = 2048, 1024, 3584
H, DH, WIN, DIL = 32, 32, 8, 2
NB = D // 128
HALO = 16
FA = 768
TA = 512
TB = 256
FC = 256
RG = 8
SCALE = DH ** -0.5

f32 = jnp.float32
bf16 = jnp.bfloat16
u32 = jnp.uint32


def _dot(a, b):
    return jnp.dot(a, b, preferred_element_type=f32)


def _lane_bit_zero(shape, bit):
    lane = jax.lax.broadcasted_iota(jnp.int32, shape, 1)
    return (lane & (1 << bit)) == 0


def _reglu(x, wg, wu):
    g = _dot(x, wg)
    u = _dot(x, wu)
    return (jnp.maximum(g, 0.0) * u).astype(bf16)


def _kernel(x_hbm, wqkv_hbm, wo_hbm, wg_hbm, wu_hbm, wd_hbm, gw_ref, out_hbm,
            x_v, wqkv_v, wo_v, wg_v, wu_v, wd_v, wqkv_p, wo_p, bacc,
            q_s, k_s, v_s, o_s, out_v, sems, xsems, psems, osem):
    def cp(src, dst, sem):
        return pltpu.make_async_copy(src, dst, sem)

    def rows(ref, a, n):
        return ref.at[pl.ds(a, n), :]

    def cols(ref, a, n):
        return ref.at[:, pl.ds(a, n)]

    c_x0a = cp(rows(x_hbm, 0, 256), rows(x_v, 0, 256), sems.at[0])
    c_g0 = cp(cols(wg_hbm, 0, 256), cols(wg_v, 0, 256), sems.at[1])
    c_x0b = cp(rows(x_hbm, 256, 256), rows(x_v, 256, 256), sems.at[2])
    c_u0 = cp(cols(wu_hbm, 0, 256), cols(wu_v, 0, 256), sems.at[3])
    c_g1 = cp(cols(wg_hbm, 256, FA - 256), cols(wg_v, 256, FA - 256), sems.at[4])
    c_u1 = cp(cols(wu_hbm, 256, FA - 256), cols(wu_v, 256, FA - 256), sems.at[5])
    c_d0 = cp(rows(wd_hbm, 0, FA), rows(wd_v, 0, FA), sems.at[6])
    c_wo = cp(wo_hbm, wo_v, sems.at[7])
    c_g2 = cp(cols(wg_hbm, FA, F - FA), cols(wg_v, FA, F - FA), sems.at[8])
    c_u2 = cp(cols(wu_hbm, FA, F - FA), cols(wu_v, FA, F - FA), sems.at[9])
    c_d2 = cp(rows(wd_hbm, FA, F - FA), rows(wd_v, FA, F - FA), sems.at[10])

    def c_x(i):
        a = (i + 1) * TA
        if not isinstance(i, int):
            a = pl.multiple_of(a, TA)
        return cp(rows(x_hbm, a, TA), rows(x_v, a, TA), xsems.at[i])

    def c_p(i):
        return cp(cols(wqkv_hbm, i * D, D), wqkv_v.at[i], psems.at[i])

    def c_pw(i):
        return cp(wqkv_v.at[i], wqkv_v.at[i], psems.at[i])

    for c in (c_x0a, c_g0, c_x0b, c_u0, c_g1, c_u1, c_d0, c_wo):
        c.start()
    for i in range(3):
        c_x(i).start()
        c_p(i).start()
    for c in (c_g2, c_u2, c_d2):
        c.start()

    k_s[:, pl.ds(0, HALO), :] = jnp.zeros((NB, HALO, 128), f32)
    v_s[:, pl.ds(0, HALO), :] = jnp.zeros((NB, HALO, 128), f32)

    def permute_cols(i):
        RB = 64
        for r in range(0, D // 2, RB):
            blk = [pltpu.bitcast(wqkv_v[i, pl.ds(2 * r, 2 * RB), pl.ds(128 * j, 128)], u32)
                   for j in range(NB)]
            for bb, lb in ((2, 3), (1, 2), (0, 1)):
                keep = _lane_bit_zero((RB, 128), lb)
                sh = 1 << lb
                for j in range(NB):
                    if j & (1 << bb):
                        continue
                    a, b = blk[j], blk[j | (1 << bb)]
                    blk[j] = jnp.where(keep, a, pltpu.roll(b, sh, 1))
                    blk[j | (1 << bb)] = jnp.where(keep, pltpu.roll(a, 128 - sh, 1), b)
            for j in range(NB):
                wqkv_p[i, pl.ds(r, RB), pl.ds(128 * j, 128)] = blk[j]

    def permute_wo():
        for j in range(NB):
            for i in range(8):
                for m in range(8):
                    r = 64 * i + 8 * m
                    val = pltpu.bitcast(wo_v[pl.ds(2 * r, 16), pl.ds(128 * j, 128)], u32)
                    wo_p[j, pl.ds(8 * m + i, 8, stride=64), :] = val

    c_x0a.wait()
    c_g0.wait()
    g_a = _dot(x_v[pl.ds(0, 256), :], wg_v[:, pl.ds(0, 256)])
    c_x0b.wait()
    g_b = _dot(x_v[pl.ds(256, 256), :], wg_v[:, pl.ds(0, 256)])
    c_u0.wait()
    x0 = x_v[pl.ds(0, TA), :]
    u0 = _dot(x0, wu_v[:, pl.ds(0, 256)])
    h0 = (jnp.maximum(jnp.concatenate([g_a, g_b], axis=0), 0.0) * u0).astype(bf16)
    c_g1.wait()
    g1 = _dot(x0, wg_v[:, pl.ds(256, FA - 256)])
    c_u1.wait()
    u1 = _dot(x0, wu_v[:, pl.ds(256, FA - 256)])
    h1 = (jnp.maximum(g1, 0.0) * u1).astype(bf16)
    c_d0.wait()
    c_wo.wait()
    permute_wo()
    bacc[pl.ds(0, TA), :] = _dot(jnp.concatenate([h0, h1], axis=1), wd_v[pl.ds(0, FA), :])

    def phase_a(i, carry):
        c_x(i).wait()
        c_pw(i).wait()
        a = pl.multiple_of((i + 1) * TA, TA)
        x = x_v[pl.ds(a, TA), :]
        hs = [_reglu(x, wg_v[:, pl.ds(c, 256)], wu_v[:, pl.ds(c, 256)]) for c in range(0, FA, 256)]
        permute_cols(i)
        bacc[pl.ds(a, TA), :] = _dot(jnp.concatenate(hs, axis=1), wd_v[pl.ds(0, FA), :])
        return carry

    jax.lax.fori_loop(0, 3, phase_a, 0)
    c_g2.wait()
    c_u2.wait()
    c_d2.wait()

    m16 = _lane_bit_zero((RG, 128), 4)
    m1 = _lane_bit_zero((RG, 128), 0)

    def attend(r0, base):
        q = [q_s[j, pl.ds(r0, RG), :] for j in range(NB)]
        logits = []
        for w in range(WIN):
            off = HALO + r0 - DIL * w
            acc = q[0] * k_s[0, pl.ds(off, RG), :]
            for j in range(1, NB):
                acc = acc + q[j] * k_s[j, pl.ds(off, RG), :]
            acc = acc + jnp.where(m16, pltpu.roll(acc, 128 - 16, 1), pltpu.roll(acc, 16, 1))
            acc = acc + jnp.where(m1, pltpu.roll(acc, 128 - 1, 1), pltpu.roll(acc, 1, 1))
            acc = acc * SCALE
            if r0 < DIL * w:
                pos = base + r0 + jax.lax.broadcasted_iota(jnp.int32, (RG, 128), 0)
                acc = jnp.where(pos >= DIL * w, acc, -1e9)
            logits.append(acc)
        m = logits[0]
        for w in range(1, WIN):
            m = jnp.maximum(m, logits[w])
        e = [jnp.exp(l - m) for l in logits]
        s = e[0]
        for w in range(1, WIN):
            s = s + e[w]
        inv = 1.0 / s
        p = [x * inv for x in e]
        for j in range(NB):
            o = p[0] * v_s[j, pl.ds(HALO + r0, RG), :]
            for w in range(1, WIN):
                o = o + p[w] * v_s[j, pl.ds(HALO + r0 - DIL * w, RG), :]
            o_s[pl.ds(r0, RG), pl.ds(128 * j, 128)] = o

    def phase_b(t, carry):
        base = pl.multiple_of(t * TB, TB)
        x = x_v[pl.ds(base, TB), :]
        for i, (dst, off) in enumerate(((q_s, 0), (k_s, HALO), (v_s, HALO))):
            r = _dot(x, pltpu.bitcast(wqkv_p[i], bf16))
            for j in range(NB):
                dst[j, pl.ds(off, TB), :] = r[:, 128 * j:128 * (j + 1)]
        chunks = list(range(FA, F, FC))
        groups = list(range(0, TB, RG))
        per = -(-len(groups) // len(chunks))
        hs = []
        for n, c in enumerate(chunks):
            hs.append(_reglu(x, wg_v[:, pl.ds(c, FC)], wu_v[:, pl.ds(c, FC)]))
            for r0 in groups[n * per:(n + 1) * per]:
                attend(r0, base)
        k_s[:, pl.ds(0, HALO), :] = k_s[:, pl.ds(TB, HALO), :]
        v_s[:, pl.ds(0, HALO), :] = v_s[:, pl.ds(TB, HALO), :]
        z = jnp.sum(x.astype(f32) * gw_ref[...].astype(f32), axis=-1, keepdims=True)
        g = jax.nn.sigmoid(z)
        wo = jnp.concatenate([pltpu.bitcast(wo_p[j], bf16) for j in range(NB)], axis=1)
        a = _dot(o_s[...].astype(bf16), wo)
        b = bacc[pl.ds(base, TB), :] + _dot(jnp.concatenate(hs, axis=1), wd_v[pl.ds(FA, F - FA), :])
        out_v[pl.ds(base, TB), :] = (g * a + (1.0 - g) * b).astype(bf16)
        cp(rows(out_v, base, TB), rows(out_hbm, base, TB), osem).start()
        return carry

    jax.lax.fori_loop(0, S // TB, phase_b, 0)
    cp(out_v, out_hbm, osem).wait()


@jax.jit
def pallas_gated_mix__sliding_local_dilated__glu_gated_reglu__prompt_kernel(
    A_x: jax.Array,
    A_wqkv: jax.Array,
    A_wo: jax.Array,
    B_x: jax.Array,
    B_W_gate: jax.Array,
    B_W_up: jax.Array,
    B_W_down: jax.Array,
    gate_w: jax.Array,
):
    del B_x
    x = A_x.reshape(S, D)
    gw = gate_w.reshape(1, D)
    hbm = pl.BlockSpec(memory_space=pl.ANY)
    out = pl.pallas_call(
        _kernel,
        out_shape=jax.ShapeDtypeStruct((S, D), bf16),
        in_specs=[hbm] * 6 + [pl.BlockSpec(memory_space=pltpu.VMEM)],
        out_specs=hbm,
        scratch_shapes=[
            pltpu.VMEM((S, D), bf16),
            pltpu.VMEM((3, D, D), bf16),
            pltpu.VMEM((D, D), bf16),
            pltpu.VMEM((D, F), bf16),
            pltpu.VMEM((D, F), bf16),
            pltpu.VMEM((F, D), bf16),
            pltpu.VMEM((3, D // 2, D), u32),
            pltpu.VMEM((NB, D // 2, 128), u32),
            pltpu.VMEM((S, D), f32),
            pltpu.VMEM((NB, TB, 128), f32),
            pltpu.VMEM((NB, HALO + TB, 128), f32),
            pltpu.VMEM((NB, HALO + TB, 128), f32),
            pltpu.VMEM((TB, D), f32),
            pltpu.VMEM((S, D), bf16),
            pltpu.SemaphoreType.DMA((11,)),
            pltpu.SemaphoreType.DMA((3,)),
            pltpu.SemaphoreType.DMA((3,)),
            pltpu.SemaphoreType.DMA(()),
        ],
        compiler_params=pltpu.CompilerParams(vmem_limit_bytes=110 * 1024 * 1024),
    )(x, A_wqkv, A_wo, B_W_gate, B_W_up, B_W_down, gw)
    return out.reshape(1, S, D)
```

```python
import os
import jax
import jax.numpy as jnp
import jax.experimental.pallas as pl
import jax.experimental.pallas.tpu as pltpu

S, D, F = 2048, 1024, 3584
H, DH, WIN, DIL = 32, 32, 8, 2
NB = D // 128
HALO = 16
CA = 384
FA = 2 * CA
FB = F - FA
TA = 512
NA = (S // TA) * 2
TB = int(os.environ.get("TB", 256))
FC = 256
RG = 8
SCOPES = int(os.environ.get("SCOPES", 0))
PITCH = 65
CPU = 5
NCH = 4 * 8
SCALE = DH ** -0.5

f32 = jnp.float32
bf16 = jnp.bfloat16
u32 = jnp.uint32
i32 = jnp.int32


def _dot(a, b):
    return jnp.dot(a, b, preferred_element_type=f32)


def _lane(shape):
    return jax.lax.broadcasted_iota(i32, shape, 1)


class _NoScope:
    def __enter__(self):
        return self

    def __exit__(self, *a):
        return False


def _scope(name):
    return jax.named_scope(name) if SCOPES else _NoScope()


def _kernel(x_hbm, wqkv_hbm, wo_hbm, wg_hbm, wu_hbm, wd_hbm, gw_hbm, out_hbm,
            x_v, w_v, wga_v, wua_v, wda_v, wg_v, wu_v, wd_v, gw_v, w_p, bacc,
            qkv_s, o_s, out_v, zero_s, sems, osem):
    copies = []

    def cp(src, dst):
        c = pltpu.make_async_copy(src, dst, sems.at[len(copies)])
        copies.append(c)
        return c

    def rows(ref, a, n):
        return ref.at[pl.ds(a, n), :]

    def cols(ref, a, n):
        return ref.at[:, pl.ds(a, n)]

    def cp_x(a, n):
        return cp(rows(x_hbm, a, n), rows(x_v, a, n))

    def cp_chunks(u):
        lo, hi = CPU * (u - 1), min(CPU * u, NCH)
        out = []
        for p in range(4):
            a, b = max(lo, 8 * p), min(hi, 8 * p + 8)
            if a < b:
                r, n = 128 * (a - 8 * p), 128 * (b - a)
                src = (wqkv_hbm.at[pl.ds(r, n), pl.ds(p * D, D)] if p < 3 else rows(wo_hbm, r, n))
                out.append(cp(src, w_v.at[p, pl.ds(r, n), :]))
        return out

    c_s1 = [cp_x(0, 256), cp(cols(wg_hbm, 0, 256), wga_v.at[0, :, pl.ds(0, 256)])]
    c_s2 = [cp_x(256, 256)]
    c_s3 = [cp(cols(wu_hbm, 0, 256), wua_v.at[0, :, pl.ds(0, 256)])]
    c_s4 = [cp(cols(wg_hbm, 256, CA - 256), wga_v.at[0, :, pl.ds(256, CA - 256)]),
            cp(cols(wu_hbm, 256, CA - 256), wua_v.at[0, :, pl.ds(256, CA - 256)]),
            cp(rows(wd_hbm, 0, CA), wda_v.at[0])]
    c_unit = {}
    for u in range(1, NA):
        lst = []
        if u < 4:
            lst.append(cp_x(u * TA, TA))
        if u == 4:
            lst += [cp(cols(wg_hbm, CA, CA), wga_v.at[1]), cp(cols(wu_hbm, CA, CA), wua_v.at[1]),
                    cp(rows(wd_hbm, CA, CA), wda_v.at[1])]
        c_unit[u] = lst + cp_chunks(u)
    c_b = [cp(gw_hbm, gw_v), cp(cols(wg_hbm, FA, FB), wg_v), cp(cols(wu_hbm, FA, FB), wu_v),
           cp(rows(wd_hbm, FA, FB), wd_v)]
    for c in copies:
        c.start()

    def wait(cs, name):
        with _scope(name):
            for c in cs:
                c.wait()

    zero_s[0] = 0
    qkv_s[pl.ds(NB, 2 * NB), pl.ds(0, HALO), :] = jnp.zeros((2 * NB, HALO, 128), f32)

    def repack(ch):
        p = ch // 8
        rc = ch % 8
        on = jnp.where(ch < 24, -1, 0).astype(i32)
        r0 = pl.multiple_of(rc * 128, 128)
        blk = [pltpu.bitcast(w_v[p, pl.ds(r0, 128), pl.ds(128 * j, 128)], u32) for j in range(NB)]
        lane = _lane((64, 128))
        for bb, lb in ((2, 3), (1, 2), (0, 1)):
            sh = 1 << lb
            keep_a = (lane & (on & sh)) == 0
            take_a = ((lane & sh) | (~on & 1)) == 0
            for j in range(NB):
                if j & (1 << bb):
                    continue
                a, b = blk[j], blk[j | (1 << bb)]
                blk[j] = jnp.where(keep_a, a, pltpu.roll(b, sh, 1))
                blk[j | (1 << bb)] = jnp.where(take_a, pltpu.roll(a, 128 - sh, 1), b)
        for j in range(NB):
            w_p[p, j, pl.ds(rc * PITCH, 64), :] = blk[j]

    wait(c_s1, "w1")
    g_a = _dot(x_v[pl.ds(0, 256), :], wga_v[0, :, pl.ds(0, 256)])
    wait(c_s2, "w2")
    g_b = _dot(x_v[pl.ds(256, 256), :], wga_v[0, :, pl.ds(0, 256)])
    wait(c_s3, "w3")
    x0 = x_v[pl.ds(0, TA), :]
    u0 = _dot(x0, wua_v[0, :, pl.ds(0, 256)])
    h0 = (jnp.maximum(jnp.concatenate([g_a, g_b], axis=0), 0.0) * u0).astype(bf16)
    wait(c_s4, "w4")
    g1 = _dot(x0, wga_v[0, :, pl.ds(256, CA - 256)])
    u1 = _dot(x0, wua_v[0, :, pl.ds(256, CA - 256)])
    h1 = (jnp.maximum(g1, 0.0) * u1).astype(bf16)
    bacc[0, pl.ds(0, TA), :] = _dot(jnp.concatenate([h0, h1], axis=1), wda_v[0])

    def phase_a(u, carry):
        for k in range(1, NA):
            pl.when(u == k)(lambda k=k: wait(c_unit[k], "wA"))
        c = u // 4
        a = pl.multiple_of((u % 4) * TA, TA)
        x = x_v[pl.ds(a, TA), :]
        g = _dot(x, wga_v[c])
        up = _dot(x, wua_v[c])
        h = (jnp.maximum(g, 0.0) * up).astype(bf16)
        for k in range(CPU):
            repack(jnp.minimum(CPU * (u - 1) + k, NCH - 1))
        bacc[c, pl.ds(a, TA), :] = _dot(h, wda_v[c])
        return carry

    jax.lax.fori_loop(1, NA, phase_a, 0)
    wait(c_b, "wB")

    m16 = (_lane((RG, 128)) & 16) == 0
    m1 = (_lane((RG, 128)) & 1) == 0

    def attend(r0, base, scale):
        q = [qkv_s[j, pl.ds(HALO + r0, RG), :] * scale for j in range(NB)]
        logits = []
        for w in range(WIN):
            off = HALO + r0 - DIL * w
            acc = q[0] * qkv_s[NB, pl.ds(off, RG), :]
            for j in range(1, NB):
                acc = acc + q[j] * qkv_s[NB + j, pl.ds(off, RG), :]
            acc = acc + jnp.where(m16, pltpu.roll(acc, 128 - 16, 1), pltpu.roll(acc, 16, 1))
            acc = acc + jnp.where(m1, pltpu.roll(acc, 128 - 1, 1), pltpu.roll(acc, 1, 1))
            if r0 < DIL * w:
                pos = base + r0 + jax.lax.broadcasted_iota(i32, (RG, 128), 0)
                acc = jnp.where(pos >= DIL * w, acc, -1e9)
            logits.append(acc)
        m = logits[0]
        for w in range(1, WIN):
            m = jnp.maximum(m, logits[w])
        e = [jnp.exp(l - m) for l in logits]
        s = e[0]
        for w in range(1, WIN):
            s = s + e[w]
        inv = 1.0 / s
        p = [x * inv for x in e]
        for j in range(NB):
            o = p[0] * qkv_s[2 * NB + j, pl.ds(HALO + r0, RG), :]
            for w in range(1, WIN):
                o = o + p[w] * qkv_s[2 * NB + j, pl.ds(HALO + r0 - DIL * w, RG), :]
            o_s[j, pl.ds(r0, RG), :] = o

    def packed(pieces):
        return jnp.concatenate(
            [pltpu.bitcast(jnp.concatenate(ps, axis=0), bf16) for ps in pieces], axis=1)

    def phase_b(t, carry):
        base = pl.multiple_of(t * TB, TB)
        zero = zero_s[0]
        zvec = jnp.full((RG, 128), zero, i32)
        sbits = pltpu.bitcast(jnp.full((RG, 128), SCALE, f32), i32)
        x = x_v[pl.ds(base, TB), :]
        for i in range(3):
            w = packed([[w_p[i, j, pl.ds(PITCH * c, 64), :] for c in range(8)] for j in range(NB)])
            r = _dot(x, w)
            for j in range(NB):
                qkv_s[i * NB + j, pl.ds(HALO, TB), :] = r[:, 128 * j:128 * (j + 1)]
        groups = list(range(0, TB, RG))
        nslots = 2 * FB // 128 - 4
        hs = []
        slot = 0
        done = 0

        def release(anchor):
            nonlocal slot, done
            slot += 1
            want = min(len(groups), -(-slot * len(groups) // nslots))
            if want > done:
                scale = pltpu.bitcast(sbits | (pltpu.bitcast(anchor, i32) & zvec), f32)
                for r0 in groups[done:want]:
                    attend(r0, base, scale)
                done = want

        for c in range(0, FB, FC):
            g = _dot(x, wg_v[:, pl.ds(c, FC)])
            for n in range(FC // 128):
                release(g[TB - 8:, 128 * n:128 * (n + 1)])
            u = _dot(x, wu_v[:, pl.ds(c, FC)])
            for n in range(FC // 128):
                release(u[TB - 8:, 128 * n:128 * (n + 1)])
            hs.append((jnp.maximum(g, 0.0) * u).astype(bf16))
        assert done == len(groups)
        qkv_s[pl.ds(NB, 2 * NB), pl.ds(0, HALO), :] = qkv_s[pl.ds(NB, 2 * NB), pl.ds(TB, HALO), :]
        z = jnp.sum(x.astype(f32) * gw_v[...].astype(f32).reshape(1, D), axis=-1, keepdims=True)
        g = jax.nn.sigmoid(z)
        wo = packed([[w_p[3, j, pl.ds(8 * m + c, 8, stride=PITCH), :]
                      for c in range(8) for m in range(8)] for j in range(NB)])
        o_s[0, pl.ds(TB + zero, 8), :] = jnp.zeros((8, 128), f32)
        o = jnp.concatenate([o_s[j, pl.ds(0, TB), :] for j in range(NB)], axis=1)
        a = _dot(o.astype(bf16), wo)
        b = (bacc[0, pl.ds(base, TB), :] + bacc[1, pl.ds(base, TB), :]
             + _dot(jnp.concatenate(hs, axis=1), wd_v[...]))
        out_v[pl.ds(base, TB), :] = (g * a + (1.0 - g) * b).astype(bf16)
        pltpu.make_async_copy(rows(out_v, base, TB), rows(out_hbm, base, TB), osem).start()
        return carry

    with _scope("B"):
        jax.lax.fori_loop(0, S // TB, phase_b, 0)
    with _scope("wout"):
        pltpu.make_async_copy(out_v, out_hbm, osem).wait()


@jax.jit
def pallas_gated_mix__sliding_local_dilated__glu_gated_reglu__prompt_kernel(
    A_x: jax.Array,
    A_wqkv: jax.Array,
    A_wo: jax.Array,
    B_x: jax.Array,
    B_W_gate: jax.Array,
    B_W_up: jax.Array,
    B_W_down: jax.Array,
    gate_w: jax.Array,
):
    del B_x
    x = A_x.reshape(S, D)
    hbm = pl.BlockSpec(memory_space=pl.ANY)
    out = pl.pallas_call(
        _kernel,
        out_shape=jax.ShapeDtypeStruct((S, D), bf16),
        in_specs=[hbm] * 7,
        out_specs=hbm,
        scratch_shapes=[
            pltpu.VMEM((S, D), bf16),
            pltpu.VMEM((4, D, D), bf16),
            pltpu.VMEM((2, D, CA), bf16),
            pltpu.VMEM((2, D, CA), bf16),
            pltpu.VMEM((2, CA, D), bf16),
            pltpu.VMEM((D, FB), bf16),
            pltpu.VMEM((D, FB), bf16),
            pltpu.VMEM((FB, D), bf16),
            pltpu.VMEM((D,), bf16),
            pltpu.VMEM((4, NB, 8 * PITCH, 128), u32),
            pltpu.VMEM((2, S, D), f32),
            pltpu.VMEM((3 * NB, HALO + TB + 8, 128), f32),
            pltpu.VMEM((NB, TB + 8, 128), f32),
            pltpu.VMEM((S, D), bf16),
            pltpu.SMEM((1,), i32),
            pltpu.SemaphoreType.DMA((32,)),
            pltpu.SemaphoreType.DMA(()),
        ],
        compiler_params=pltpu.CompilerParams(vmem_limit_bytes=110 * 1024 * 1024),
    )(x, A_wqkv, A_wo, B_W_gate, B_W_up, B_W_down, gate_w)
    return out.reshape(1, S, D)
```

```python
import os
import jax
import jax.numpy as jnp
import jax.experimental.pallas as pl
import jax.experimental.pallas.tpu as pltpu

S, D, F = 2048, 1024, 3584
H, DH, WIN, DIL = 32, 32, 8, 2
NB = D // 128
NF = F // 128
HALO = 16
BA = 3
NFA = 2 * BA
TA = 512
NA = (S // TA) * 2
TB = 256
RG = 8
ANCH = int(os.environ.get('ANCH', 56))
NSK = int(os.environ.get('NSK', 6))
ORDER = int(os.environ.get('ORDER', 0))
SCOPES = int(os.environ.get("SCOPES", 0))
CHECKS = int(os.environ.get("CHECKS", 0))
PITCH = 65
CPU = 5
NCH = 4 * 8
LOG2E = 1.4426950408889634
SCALE = DH ** -0.5 * LOG2E
NEG = -1e9 * LOG2E

f32 = jnp.float32
bf16 = jnp.bfloat16
u32 = jnp.uint32
i32 = jnp.int32


def _dot(a, b):
    return jnp.dot(a, b, preferred_element_type=f32)


def _lane(shape):
    return jax.lax.broadcasted_iota(i32, shape, 1)


def _cat(blocks):
    return jnp.concatenate([pltpu.bitcast(b, bf16) for b in blocks], axis=1)


def _reglu(g, u):
    return (jnp.maximum(g, 0.0) * u).astype(bf16)


class _NoScope:
    def __enter__(self):
        return self

    def __exit__(self, *a):
        return False


def _scope(name):
    return jax.named_scope(name) if SCOPES else _NoScope()


def _kernel(x_hbm, wqkv_hbm, wo_hbm, wg_hbm, wu_hbm, wd_hbm, gw_hbm, out_hbm,
            x_v, w_v, wg_v, wu_v, wd_v, gw_v, w_p, bacc,
            qkv_s, o_s, out_v, zero_s, sems):
    def start(src, dst, grp):
        pltpu.make_async_copy(src, dst, sems.at[grp]).start()

    def wait(grp, *dsts):
        with _scope("w%d" % grp):
            for d in dsts:
                pltpu.make_async_copy(d, d, sems.at[grp]).wait()

    def xrows(a, n):
        return x_v.at[pl.ds(a, n), :]

    def get_x(a, n, grp):
        start(x_hbm.at[pl.ds(a, n), :], xrows(a, n), grp)

    def get_cols(hbm, dst, b0, b1, grp):
        for b in range(b0, b1):
            start(hbm.at[:, pl.ds(128 * b, 128)], dst.at[b], grp)

    def wd_rows(b0, b1):
        return wd_v.at[:, pl.ds(128 * b0, 128 * (b1 - b0)), :]

    def get_wd(b0, b1, grp):
        for j in range(NB):
            start(wd_hbm.at[pl.ds(128 * b0, 128 * (b1 - b0)), pl.ds(128 * j, 128)],
                  wd_v.at[j, pl.ds(128 * b0, 128 * (b1 - b0)), :], grp)

    def w_rows(c0, c1):
        out = []
        for p in range(4):
            a, b = max(c0, 8 * p), min(c1, 8 * p + 8)
            if a < b:
                out.append((p, 128 * (a - 8 * p), 128 * (b - a)))
        return out

    def w_dst(c0, c1):
        return [w_v.at[p, pl.ds(r, n), :] for p, r, n in w_rows(c0, c1)]

    def get_w(c0, c1, grp):
        for p, r, n in w_rows(c0, c1):
            src = (wqkv_hbm.at[pl.ds(r, n), pl.ds(p * D, D)] if p < 3
                   else wo_hbm.at[pl.ds(r, n), :])
            start(src, w_v.at[p, pl.ds(r, n), :], grp)

    get_x(0, 256, 0)
    get_cols(wg_hbm, wg_v, 0, 2, 0)
    get_x(256, 256, 1)
    get_cols(wu_hbm, wu_v, 0, 2, 2)
    get_cols(wg_hbm, wg_v, 2, BA, 3)
    get_cols(wu_hbm, wu_v, 2, BA, 3)
    get_wd(0, BA, 3)
    get_x(TA, TA, 4)
    get_w(0, CPU, 4)
    get_x(2 * TA, TA, 5)
    get_w(CPU, 2 * CPU, 5)
    get_x(3 * TA, TA, 6)
    get_w(2 * CPU, 3 * CPU, 6)
    get_cols(wg_hbm, wg_v, BA, NFA, 7)
    get_cols(wu_hbm, wu_v, BA, NFA, 7)
    get_wd(BA, NFA, 7)
    get_w(3 * CPU, NCH, 7)
    start(gw_hbm, gw_v, 8)
    get_wd(NFA, NF, 8)
    get_cols(wg_hbm, wg_v, NFA, NF, 8)

    wg_u, wu_u, wd_u = (r.bitcast(u32) for r in (wg_v, wu_v, wd_v))

    zero_s[0] = 0
    qkv_s[pl.ds(NB, 2 * NB), pl.ds(0, HALO), :] = jnp.zeros((2 * NB, HALO, 128), f32)

    def repack(ch):
        p = jax.lax.shift_right_logical(ch, 3)
        rc = ch & 7
        on = jnp.where(ch < 24, -1, 0).astype(i32)
        r0 = pl.multiple_of(rc * 128, 128)
        blk = [pltpu.bitcast(w_v[p, pl.ds(r0, 128), pl.ds(128 * j, 128)], u32) for j in range(NB)]
        lane = _lane((64, 128))
        for bb, lb in ((2, 3), (1, 2), (0, 1)):
            sh = 1 << lb
            keep_a = (lane & (on & sh)) == 0
            take_a = ((lane & sh) | (~on & 1)) == 0
            for j in range(NB):
                if j & (1 << bb):
                    continue
                a, b = blk[j], blk[j | (1 << bb)]
                blk[j] = jnp.where(keep_a, a, pltpu.roll(b, sh, 1))
                blk[j | (1 << bb)] = jnp.where(take_a, pltpu.roll(a, 128 - sh, 1), b)
        for j in range(NB):
            w_p[p, j, pl.ds(rc * PITCH, 64), :] = blk[j]

    wait(0, xrows(0, 256), wg_v.at[pl.ds(0, 2)])
    g_a = _dot(x_v[pl.ds(0, 256), :], _cat([wg_u[0], wg_u[1]]))
    wait(1, xrows(256, 256))
    g_b = _dot(x_v[pl.ds(256, 256), :], _cat([wg_u[0], wg_u[1]]))
    wait(2, wu_v.at[pl.ds(0, 2)])
    x0 = x_v[pl.ds(0, TA), :]
    h0 = _reglu(jnp.concatenate([g_a, g_b], axis=0), _dot(x0, _cat([wu_u[0], wu_u[1]])))
    wait(3, wg_v.at[2], wu_v.at[2], wd_rows(0, BA))
    h1 = _reglu(_dot(x0, _cat([wg_u[2]])), _dot(x0, _cat([wu_u[2]])))
    bacc[0, pl.ds(0, TA), :] = _dot(jnp.concatenate([h0, h1], axis=1),
                                    _cat([wd_u[j, pl.ds(0, 64 * BA), :] for j in range(NB)]))
    get_cols(wu_hbm, wu_v, NFA, NF, 8)

    def phase_a(u, carry):
        pl.when(u == 1)(lambda: wait(4, xrows(TA, TA), *w_dst(0, CPU)))
        pl.when(u == 2)(lambda: wait(5, xrows(2 * TA, TA), *w_dst(CPU, 2 * CPU)))
        pl.when(u == 3)(lambda: wait(6, xrows(3 * TA, TA), *w_dst(2 * CPU, 3 * CPU)))
        pl.when(u == 4)(lambda: wait(7, wg_v.at[pl.ds(BA, BA)], wu_v.at[pl.ds(BA, BA)],
                                     wd_rows(BA, NFA), *w_dst(3 * CPU, NCH)))
        c = jax.lax.shift_right_logical(u, 2)
        a = pl.multiple_of((u & 3) * TA, TA)
        x = x_v[pl.ds(a, TA), :]
        h = _reglu(_dot(x, _cat([wg_u[c * BA + k] for k in range(BA)])),
                   _dot(x, _cat([wu_u[c * BA + k] for k in range(BA)])))
        for k in range(CPU):
            repack(jnp.minimum(CPU * (u - 1) + k, NCH - 1))
        r = pl.multiple_of(c * (64 * BA), 64)
        bacc[c, pl.ds(a, TA), :] = _dot(h, _cat([wd_u[j, pl.ds(r, 64 * BA), :] for j in range(NB)]))
        return carry

    jax.lax.fori_loop(1, NA, phase_a, 0)
    wait(8, gw_v, wg_v.at[pl.ds(NFA, NF - NFA)], wu_v.at[pl.ds(NFA, NF - NFA)], wd_rows(NFA, NF))

    m16 = (_lane((RG, 128)) & 16) == 0
    m1 = (_lane((RG, 128)) & 1) == 0

    def attend(r0, base, scale):
        q = [qkv_s[j, pl.ds(HALO + r0, RG), :] * scale for j in range(NB)]
        logits = []
        for w in range(WIN):
            off = HALO + r0 - DIL * w
            acc = q[0] * qkv_s[NB, pl.ds(off, RG), :]
            for j in range(1, NB):
                acc = acc + q[j] * qkv_s[NB + j, pl.ds(off, RG), :]
            acc = acc + jnp.where(m16, pltpu.roll(acc, 128 - 16, 1), pltpu.roll(acc, 16, 1))
            acc = acc + jnp.where(m1, pltpu.roll(acc, 128 - 1, 1), pltpu.roll(acc, 1, 1))
            if r0 < DIL * w:
                pos = base + r0 + jax.lax.broadcasted_iota(i32, (RG, 128), 0)
                acc = jnp.where(pos >= DIL * w, acc, NEG)
            logits.append(acc)
        m = logits[0]
        for w in range(1, WIN):
            m = jnp.maximum(m, logits[w])
        e = [jnp.exp2(l - m) for l in logits]
        s = e[0]
        for w in range(1, WIN):
            s = s + e[w]
        inv = pl.reciprocal(s, approx=True)
        inv = inv * (2.0 - s * inv)
        p = [x * inv for x in e]
        for j in range(NB):
            o = p[0] * qkv_s[2 * NB + j, pl.ds(HALO + r0, RG), :]
            for w in range(1, WIN):
                o = o + p[w] * qkv_s[2 * NB + j, pl.ds(HALO + r0 - DIL * w, RG), :]
            o_s[j, pl.ds(r0, RG), :] = o

    def phase_b(t, carry):
        base = pl.multiple_of(t * TB, TB)
        zero = zero_s[0]
        zvec = jnp.full((RG, 128), zero, i32)
        sbits = pltpu.bitcast(jnp.full((RG, 128), SCALE, f32), i32)
        x = x_v[pl.ds(base, TB), :]
        for i in range(3):
            r = _dot(x, _cat([jnp.concatenate([w_p[i, j, pl.ds(PITCH * c, 64), :] for c in range(8)],
                                              axis=0) for j in range(NB)]))
            for j in range(NB):
                qkv_s[i * NB + j, pl.ds(HALO, TB), :] = r[:, 128 * j:128 * (j + 1)]
        groups = list(range(0, TB, RG))
        nslots = 2 * (NF - NFA) - NSK
        hs = []
        slot = 0
        done = 0

        def release(anchor):
            nonlocal slot, done
            slot += 1
            want = min(len(groups), -(-slot * len(groups) // nslots))
            if want > done:
                scale = pltpu.bitcast(sbits | (pltpu.bitcast(anchor, i32) & zvec), f32)
                for r0 in groups[done:want]:
                    attend(r0, base, scale)
                done = want

        for c in range(NFA, NF, 2):
            g = _dot(x, _cat([wg_u[c], wg_u[c + 1]]))
            for n in range(2):
                release(g[ANCH:ANCH + 8, 128 * n:128 * (n + 1)])
            u = _dot(x, _cat([wu_u[c], wu_u[c + 1]]))
            for n in range(2):
                release(u[ANCH:ANCH + 8, 128 * n:128 * (n + 1)])
            hs.append(_reglu(g, u))
        assert done == len(groups)
        qkv_s[pl.ds(NB, 2 * NB), pl.ds(0, HALO), :] = qkv_s[pl.ds(NB, 2 * NB), pl.ds(TB, HALO), :]
        z = jnp.sum(x.astype(f32) * gw_v[...].astype(f32).reshape(1, D), axis=-1, keepdims=True)
        g = jax.nn.sigmoid(z)

        def down():
            wd = _cat([wd_u[j, pl.ds(64 * NFA, 64 * (NF - NFA)), :] for j in range(NB)])
            return (bacc[0, pl.ds(base, TB), :] + bacc[1, pl.ds(base, TB), :]
                    + _dot(jnp.concatenate(hs, axis=1), wd))

        if ORDER == 1:
            b = down()
        wo = _cat([jnp.concatenate([w_p[3, j, pl.ds(8 * m + c, 8, stride=PITCH), :]
                                    for c in range(8) for m in range(8)], axis=0)
                   for j in range(NB)])
        o_s[0, pl.ds(TB + zero, 8), :] = jnp.zeros((8, 128), f32)
        o = jnp.concatenate([o_s[j, pl.ds(0, TB), :] for j in range(NB)], axis=1)
        a = _dot(o.astype(bf16), wo)
        if ORDER == 0:
            b = down()
        out_v[pl.ds(base, TB), :] = (g * a + (1.0 - g) * b).astype(bf16)
        start(out_v.at[pl.ds(base, TB), :], out_hbm.at[pl.ds(base, TB), :], 9)
        return carry

    with _scope("B"):
        jax.lax.fori_loop(0, S // TB, phase_b, 0)
    wait(9, out_v)


@jax.jit
def pallas_gated_mix__sliding_local_dilated__glu_gated_reglu__prompt_kernel(
    A_x: jax.Array,
    A_wqkv: jax.Array,
    A_wo: jax.Array,
    B_x: jax.Array,
    B_W_gate: jax.Array,
    B_W_up: jax.Array,
    B_W_down: jax.Array,
    gate_w: jax.Array,
):
    del B_x
    x = A_x.reshape(S, D)
    hbm = pl.BlockSpec(memory_space=pl.ANY)
    out = pl.pallas_call(
        _kernel,
        out_shape=jax.ShapeDtypeStruct((S, D), bf16),
        in_specs=[hbm] * 7,
        out_specs=hbm,
        scratch_shapes=[
            pltpu.VMEM((S, D), bf16),
            pltpu.VMEM((4, D, D), bf16),
            pltpu.VMEM((NF, D, 128), bf16),
            pltpu.VMEM((NF, D, 128), bf16),
            pltpu.VMEM((NB, F, 128), bf16),
            pltpu.VMEM((D,), bf16),
            pltpu.VMEM((4, NB, 8 * PITCH, 128), u32),
            pltpu.VMEM((2, S, D), f32),
            pltpu.VMEM((3 * NB, HALO + TB + 8, 128), f32),
            pltpu.VMEM((NB, TB + 8, 128), f32),
            pltpu.VMEM((S, D), bf16),
            pltpu.SMEM((1,), i32),
            pltpu.SemaphoreType.DMA((10,)),
        ],
        compiler_params=pltpu.CompilerParams(
            vmem_limit_bytes=110 * 1024 * 1024,
            disable_bounds_checks=not CHECKS,
            disable_semaphore_checks=not CHECKS,
        ),
    )(x, A_wqkv, A_wo, B_W_gate, B_W_up, B_W_down, gate_w)
    return out.reshape(1, S, D)
```

```python
import os
import jax
import jax.numpy as jnp
import jax.experimental.pallas as pl
import jax.experimental.pallas.tpu as pltpu

S, D, F = 2048, 1024, 3584
H, DH, WIN, DIL = 32, 32, 8, 2
NB = D // 128
NF = F // 128
HALO = 16
BA = 3
NFA = 2 * BA
TA = 512
NA = (S // TA) * 2
TB = 256
RG = 8
ANCH = int(os.environ.get('ANCH', 56))
NSK = int(os.environ.get('NSK', 6))
ORDER = int(os.environ.get('ORDER', 0))
OUTP = ((0, 512), (512, 768), (768, 1024))
SCOPES = int(os.environ.get("SCOPES", 0))
CHECKS = int(os.environ.get("CHECKS", 0))
PITCH = 65
CPU = 5
NCH = 4 * 8
LOG2E = 1.4426950408889634
SCALE = DH ** -0.5 * LOG2E
NEG = -1e9 * LOG2E

f32 = jnp.float32
bf16 = jnp.bfloat16
u32 = jnp.uint32
i32 = jnp.int32


def _dot(a, b):
    return jnp.dot(a, b, preferred_element_type=f32)


def _lane(shape):
    return jax.lax.broadcasted_iota(i32, shape, 1)


def _cat(blocks):
    return jnp.concatenate([pltpu.bitcast(b, bf16) for b in blocks], axis=1)


def _reglu(g, u):
    return pltpu.bitcast((jnp.maximum(g, 0.0) * u).astype(bf16), u32)


class _NoScope:
    def __enter__(self):
        return self

    def __exit__(self, *a):
        return False


def _scope(name):
    return jax.named_scope(name) if SCOPES else _NoScope()


def _kernel(x_hbm, wqkv_hbm, wo_hbm, wg_hbm, wu_hbm, wd_hbm, gw_hbm, out_hbm,
            x_v, w_v, wg_v, wu_v, wd_v, gw_v, w_p, bacc,
            qkv_s, o_s, g_s, out_v, zero_s, sems):
    def start(src, dst, grp):
        pltpu.make_async_copy(src, dst, sems.at[grp]).start()

    def wait(grp, *dsts):
        with _scope("w%d" % grp):
            for d in dsts:
                pltpu.make_async_copy(d, d, sems.at[grp]).wait()

    def xrows(a, n):
        return x_v.at[pl.ds(a, n), :]

    def get_x(a, n, grp):
        start(x_hbm.at[pl.ds(a, n), :], xrows(a, n), grp)

    def get_cols(hbm, dst, b0, b1, grp):
        for b in range(b0, b1):
            start(hbm.at[:, pl.ds(128 * b, 128)], dst.at[b], grp)

    def wd_rows(b0, b1):
        return wd_v.at[:, pl.ds(128 * b0, 128 * (b1 - b0)), :]

    def get_wd(b0, b1, grp):
        for j in range(NB):
            start(wd_hbm.at[pl.ds(128 * b0, 128 * (b1 - b0)), pl.ds(128 * j, 128)],
                  wd_v.at[j, pl.ds(128 * b0, 128 * (b1 - b0)), :], grp)

    def w_rows(c0, c1):
        out = []
        for p in range(4):
            a, b = max(c0, 8 * p), min(c1, 8 * p + 8)
            if a < b:
                out.append((p, 128 * (a - 8 * p), 128 * (b - a)))
        return out

    def w_dst(c0, c1):
        return [w_v.at[p, pl.ds(r, n), :] for p, r, n in w_rows(c0, c1)]

    def get_w(c0, c1, grp):
        for p, r, n in w_rows(c0, c1):
            src = (wqkv_hbm.at[pl.ds(r, n), pl.ds(p * D, D)] if p < 3
                   else wo_hbm.at[pl.ds(r, n), :])
            start(src, w_v.at[p, pl.ds(r, n), :], grp)

    get_x(0, 256, 0)
    get_cols(wg_hbm, wg_v, 0, 2, 0)
    get_x(256, 256, 1)
    get_cols(wu_hbm, wu_v, 0, 2, 2)
    get_cols(wg_hbm, wg_v, 2, BA, 3)
    get_cols(wu_hbm, wu_v, 2, BA, 3)
    get_wd(0, BA, 3)
    get_x(TA, TA, 4)
    get_w(0, CPU, 4)
    get_x(2 * TA, TA, 5)
    get_w(CPU, 2 * CPU, 5)
    get_x(3 * TA, TA, 6)
    get_w(2 * CPU, 3 * CPU, 6)
    get_cols(wg_hbm, wg_v, BA, NFA, 7)
    get_cols(wu_hbm, wu_v, BA, NFA, 7)
    get_wd(BA, NFA, 7)
    get_w(3 * CPU, NCH, 7)
    start(gw_hbm, gw_v, 8)
    get_wd(NFA, NF, 8)
    get_cols(wg_hbm, wg_v, NFA, NF, 8)

    wg_u, wu_u, wd_u = (r.bitcast(u32) for r in (wg_v, wu_v, wd_v))

    zero_s[0] = 0
    qkv_s[pl.ds(NB, 2 * NB), pl.ds(0, HALO), :] = jnp.zeros((2 * NB, HALO, 128), f32)

    def repack(ch):
        p = jax.lax.shift_right_logical(ch, 3)
        rc = ch & 7
        on = jnp.where(ch < 24, -1, 0).astype(i32)
        r0 = pl.multiple_of(rc * 128, 128)
        blk = [pltpu.bitcast(w_v[p, pl.ds(r0, 128), pl.ds(128 * j, 128)], u32) for j in range(NB)]
        lane = _lane((64, 128))
        for bb, lb in ((2, 3), (1, 2), (0, 1)):
            sh = 1 << lb
            keep_a = (lane & (on & sh)) == 0
            take_a = ((lane & sh) | (~on & 1)) == 0
            for j in range(NB):
                if j & (1 << bb):
                    continue
                a, b = blk[j], blk[j | (1 << bb)]
                blk[j] = jnp.where(keep_a, a, pltpu.roll(b, sh, 1))
                blk[j | (1 << bb)] = jnp.where(take_a, pltpu.roll(a, 128 - sh, 1), b)
        for j in range(NB):
            w_p[p, j, pl.ds(rc * PITCH, 64), :] = blk[j]

    wait(0, xrows(0, 256), wg_v.at[pl.ds(0, 2)])
    g_a = _dot(x_v[pl.ds(0, 256), :], _cat([wg_u[0], wg_u[1]]))
    wait(1, xrows(256, 256))
    g_b = _dot(x_v[pl.ds(256, 256), :], _cat([wg_u[0], wg_u[1]]))
    wait(2, wu_v.at[pl.ds(0, 2)])
    x0 = x_v[pl.ds(0, TA), :]
    h0 = _reglu(jnp.concatenate([g_a, g_b], axis=0), _dot(x0, _cat([wu_u[0], wu_u[1]])))
    wait(3, wg_v.at[2], wu_v.at[2], wd_rows(0, BA))
    h1 = _reglu(_dot(x0, _cat([wg_u[2]])), _dot(x0, _cat([wu_u[2]])))
    bacc[0, pl.ds(0, TA), :] = _dot(_cat([h0, h1]),
                                    _cat([wd_u[j, pl.ds(0, 64 * BA), :] for j in range(NB)]))
    get_cols(wu_hbm, wu_v, NFA, NF, 8)

    def phase_a(u, carry):
        pl.when(u == 1)(lambda: wait(4, xrows(TA, TA), *w_dst(0, CPU)))
        pl.when(u == 2)(lambda: wait(5, xrows(2 * TA, TA), *w_dst(CPU, 2 * CPU)))
        pl.when(u == 3)(lambda: wait(6, xrows(3 * TA, TA), *w_dst(2 * CPU, 3 * CPU)))
        pl.when(u == 4)(lambda: wait(7, wg_v.at[pl.ds(BA, BA)], wu_v.at[pl.ds(BA, BA)],
                                     wd_rows(BA, NFA), *w_dst(3 * CPU, NCH)))
        c = jax.lax.shift_right_logical(u, 2)
        a = pl.multiple_of((u & 3) * TA, TA)
        x = x_v[pl.ds(a, TA), :]
        h = _reglu(_dot(x, _cat([wg_u[c * BA + k] for k in range(BA)])),
                   _dot(x, _cat([wu_u[c * BA + k] for k in range(BA)])))
        for k in range(CPU):
            repack(jnp.minimum(CPU * (u - 1) + k, NCH - 1))
        r = pl.multiple_of(c * (64 * BA), 64)
        bacc[c, pl.ds(a, TA), :] = _dot(_cat([h]), _cat([wd_u[j, pl.ds(r, 64 * BA), :] for j in range(NB)]))
        return carry

    jax.lax.fori_loop(1, NA, phase_a, 0)
    wait(8, gw_v, wg_v.at[pl.ds(NFA, NF - NFA)], wu_v.at[pl.ds(NFA, NF - NFA)], wd_rows(NFA, NF))

    m16 = (_lane((RG, 128)) & 16) == 0
    m1 = (_lane((RG, 128)) & 1) == 0

    def attend(r0, base, scale):
        q = [qkv_s[j, pl.ds(HALO + r0, RG), :] * scale for j in range(NB)]
        logits = []
        for w in range(WIN):
            off = HALO + r0 - DIL * w
            acc = q[0] * qkv_s[NB, pl.ds(off, RG), :]
            for j in range(1, NB):
                acc = acc + q[j] * qkv_s[NB + j, pl.ds(off, RG), :]
            acc = acc + jnp.where(m16, pltpu.roll(acc, 128 - 16, 1), pltpu.roll(acc, 16, 1))
            acc = acc + jnp.where(m1, pltpu.roll(acc, 128 - 1, 1), pltpu.roll(acc, 1, 1))
            if r0 < DIL * w:
                pos = base + r0 + jax.lax.broadcasted_iota(i32, (RG, 128), 0)
                acc = jnp.where(pos >= DIL * w, acc, NEG)
            logits.append(acc)
        m = logits[0]
        for w in range(1, WIN):
            m = jnp.maximum(m, logits[w])
        e = [jnp.exp2(l - m) for l in logits]
        s = e[0]
        for w in range(1, WIN):
            s = s + e[w]
        inv = pl.reciprocal(s, approx=True)
        inv = inv * (2.0 - s * inv)
        p = [x * inv for x in e]
        for j in range(NB):
            o = p[0] * qkv_s[2 * NB + j, pl.ds(HALO + r0, RG), :]
            for w in range(1, WIN):
                o = o + p[w] * qkv_s[2 * NB + j, pl.ds(HALO + r0 - DIL * w, RG), :]
            o_s[j, pl.ds(r0, RG), :] = o

    def phase_b(t, carry):
        base = pl.multiple_of(t * TB, TB)
        zero = zero_s[0]
        zvec = jnp.full((RG, 128), zero, i32)
        sbits = pltpu.bitcast(jnp.full((RG, 128), SCALE, f32), i32)
        x = x_v[pl.ds(base, TB), :]
        gw = pltpu.bitcast(jnp.broadcast_to(gw_v[...].astype(f32).reshape(1, D), (8, D)), i32)

        def gate_rows(r0, anchor):
            dep = pltpu.bitcast(anchor, i32) & zvec
            xr = x_v[pl.ds(base + r0, 16), :].astype(f32)
            acc = None
            for j in range(NB):
                w = pltpu.bitcast(gw[:, 128 * j:128 * (j + 1)] | dep, f32)
                term = xr[:, 128 * j:128 * (j + 1)] * jnp.concatenate([w, w], axis=0)
                acc = term if acc is None else acc + term
            z = jnp.sum(acc, axis=-1, keepdims=True)
            g_s[pl.ds(r0, 16), :] = jnp.broadcast_to(jax.nn.sigmoid(z), (16, 128))

        for i in range(3):
            r = _dot(x, _cat([jnp.concatenate([w_p[i, j, pl.ds(PITCH * c, 64), :] for c in range(8)],
                                              axis=0) for j in range(NB)]))
            for j in range(NB):
                qkv_s[i * NB + j, pl.ds(HALO, TB), :] = r[:, 128 * j:128 * (j + 1)]
                if i * NB + j < TB // 16:
                    gate_rows(16 * (i * NB + j), r[ANCH:ANCH + 8, 128 * j:128 * (j + 1)])
        groups = list(range(0, TB, RG))
        nslots = 2 * (NF - NFA) - NSK
        hs = []
        slot = 0
        done = 0

        def release(anchor):
            nonlocal slot, done
            slot += 1
            want = min(len(groups), -(-slot * len(groups) // nslots))
            if want > done:
                scale = pltpu.bitcast(sbits | (pltpu.bitcast(anchor, i32) & zvec), f32)
                for r0 in groups[done:want]:
                    attend(r0, base, scale)
                done = want

        for c in range(NFA, NF, 2):
            g = _dot(x, _cat([wg_u[c], wg_u[c + 1]]))
            for n in range(2):
                release(g[ANCH:ANCH + 8, 128 * n:128 * (n + 1)])
            u = _dot(x, _cat([wu_u[c], wu_u[c + 1]]))
            for n in range(2):
                release(u[ANCH:ANCH + 8, 128 * n:128 * (n + 1)])
            hs.append(_reglu(g, u))
        assert done == len(groups)
        qkv_s[pl.ds(NB, 2 * NB), pl.ds(0, HALO), :] = qkv_s[pl.ds(NB, 2 * NB), pl.ds(TB, HALO), :]
        g = g_s[pl.ds(0, TB), :]
        g1 = 1.0 - g

        def down():
            wd = _cat([wd_u[j, pl.ds(64 * NFA, 64 * (NF - NFA)), :] for j in range(NB)])
            return (bacc[0, pl.ds(base, TB), :] + bacc[1, pl.ds(base, TB), :]
                    + _dot(_cat(hs), wd))

        if ORDER == 1:
            b = down()
        wo = _cat([jnp.concatenate([w_p[3, j, pl.ds(8 * m + c, 8, stride=PITCH), :]
                                    for c in range(8) for m in range(8)], axis=0)
                   for j in range(NB)])
        o_s[0, pl.ds(TB + zero, 8), :] = jnp.zeros((8, 128), f32)
        o = jnp.concatenate([o_s[j, pl.ds(0, TB), :] for j in range(NB)], axis=1)
        a = _dot(o.astype(bf16), wo)
        if ORDER == 0:
            b = down()
        for c0, c1 in OUTP:
            n = c1 - c0
            res = (jnp.concatenate([g] * (n // 128), axis=1) * a[:, c0:c1]
                   + jnp.concatenate([g1] * (n // 128), axis=1) * b[:, c0:c1])
            out_v[pl.ds(base, TB), pl.ds(c0, n)] = res.astype(bf16)
            start(out_v.at[pl.ds(base, TB), pl.ds(c0, n)], out_hbm.at[pl.ds(base, TB), pl.ds(c0, n)], 9)
        return carry

    with _scope("B"):
        jax.lax.fori_loop(0, S // TB, phase_b, 0)
    wait(9, out_v)


@jax.jit
def pallas_gated_mix__sliding_local_dilated__glu_gated_reglu__prompt_kernel(
    A_x: jax.Array,
    A_wqkv: jax.Array,
    A_wo: jax.Array,
    B_x: jax.Array,
    B_W_gate: jax.Array,
    B_W_up: jax.Array,
    B_W_down: jax.Array,
    gate_w: jax.Array,
):
    del B_x
    x = A_x.reshape(S, D)
    hbm = pl.BlockSpec(memory_space=pl.ANY)
    out = pl.pallas_call(
        _kernel,
        out_shape=jax.ShapeDtypeStruct((S, D), bf16),
        in_specs=[hbm] * 7,
        out_specs=hbm,
        scratch_shapes=[
            pltpu.VMEM((S, D), bf16),
            pltpu.VMEM((4, D, D), bf16),
            pltpu.VMEM((NF, D, 128), bf16),
            pltpu.VMEM((NF, D, 128), bf16),
            pltpu.VMEM((NB, F, 128), bf16),
            pltpu.VMEM((D,), bf16),
            pltpu.VMEM((4, NB, 8 * PITCH, 128), u32),
            pltpu.VMEM((2, S, D), f32),
            pltpu.VMEM((3 * NB, HALO + TB + 8, 128), f32),
            pltpu.VMEM((NB, TB + 8, 128), f32),
            pltpu.VMEM((TB + 8, 128), f32),
            pltpu.VMEM((S, D), bf16),
            pltpu.SMEM((1,), i32),
            pltpu.SemaphoreType.DMA((10,)),
        ],
        compiler_params=pltpu.CompilerParams(
            vmem_limit_bytes=110 * 1024 * 1024,
            disable_bounds_checks=not CHECKS,
            disable_semaphore_checks=not CHECKS,
        ),
    )(x, A_wqkv, A_wo, B_W_gate, B_W_up, B_W_down, gate_w)
    return out.reshape(1, S, D)
```

```python
import os
import jax
import jax.numpy as jnp
import jax.experimental.pallas as pl
import jax.experimental.pallas.tpu as pltpu

S, D, F = 2048, 1024, 3584
H, DH, WIN, DIL = 32, 32, 8, 2
NB = D // 128
NF = F // 128
HALO = 16
BA = 3
NFA = 2 * BA
TA = 512
NA = (S // TA) * 2
TB = 256
RG = 8
ANCH = int(os.environ.get('ANCH', 56))
NSK = int(os.environ.get('NSK', 2))
ORDER = int(os.environ.get('ORDER', 0))
OUTP = ((0, 512), (512, 768), (768, 1024))
GDEP = int(os.environ.get('GDEP', 1))
SCOPES = int(os.environ.get("SCOPES", 0))
CHECKS = int(os.environ.get("CHECKS", 0))
PITCH = 65
CPU = 5
NCH = 4 * 8
LOG2E = 1.4426950408889634
SCALE = DH ** -0.5 * LOG2E
NEG = -1e9 * LOG2E

f32 = jnp.float32
bf16 = jnp.bfloat16
u32 = jnp.uint32
i32 = jnp.int32


def _dot(a, b):
    return jnp.dot(a, b, preferred_element_type=f32)


def _lane(shape):
    return jax.lax.broadcasted_iota(i32, shape, 1)


def _cat(blocks):
    return jnp.concatenate([pltpu.bitcast(b, bf16) for b in blocks], axis=1)


def _reglu(g, u):
    return pltpu.bitcast((jnp.maximum(g, 0.0) * u).astype(bf16), u32)


class _NoScope:
    def __enter__(self):
        return self

    def __exit__(self, *a):
        return False


def _scope(name):
    return jax.named_scope(name) if SCOPES else _NoScope()


def _kernel(x_hbm, wqkv_hbm, wo_hbm, wg_hbm, wu_hbm, wd_hbm, gw_hbm, out_hbm,
            x_v, w_v, wg_v, wu_v, wd_v, gw_v, w_p, bacc,
            qkv_s, o_s, out_v, zero_s, sems):
    def start(src, dst, grp):
        pltpu.make_async_copy(src, dst, sems.at[grp]).start()

    def wait(grp, *dsts):
        with _scope("w%d" % grp):
            for d in dsts:
                pltpu.make_async_copy(d, d, sems.at[grp]).wait()

    def xrows(a, n):
        return x_v.at[pl.ds(a, n), :]

    def get_x(a, n, grp):
        start(x_hbm.at[pl.ds(a, n), :], xrows(a, n), grp)

    def get_cols(hbm, dst, b0, b1, grp):
        for b in range(b0, b1):
            start(hbm.at[:, pl.ds(128 * b, 128)], dst.at[b], grp)

    def wd_rows(b0, b1):
        return wd_v.at[:, pl.ds(128 * b0, 128 * (b1 - b0)), :]

    def get_wd(b0, b1, grp):
        for j in range(NB):
            start(wd_hbm.at[pl.ds(128 * b0, 128 * (b1 - b0)), pl.ds(128 * j, 128)],
                  wd_v.at[j, pl.ds(128 * b0, 128 * (b1 - b0)), :], grp)

    def w_rows(c0, c1):
        out = []
        for p in range(4):
            a, b = max(c0, 8 * p), min(c1, 8 * p + 8)
            if a < b:
                out.append((p, 128 * (a - 8 * p), 128 * (b - a)))
        return out

    def w_dst(c0, c1):
        return [w_v.at[p, pl.ds(r, n), :] for p, r, n in w_rows(c0, c1)]

    def get_w(c0, c1, grp):
        for p, r, n in w_rows(c0, c1):
            src = (wqkv_hbm.at[pl.ds(r, n), pl.ds(p * D, D)] if p < 3
                   else wo_hbm.at[pl.ds(r, n), :])
            start(src, w_v.at[p, pl.ds(r, n), :], grp)

    get_x(0, 256, 0)
    get_cols(wg_hbm, wg_v, 0, 2, 0)
    get_x(256, 256, 1)
    get_cols(wu_hbm, wu_v, 0, 2, 2)
    get_cols(wg_hbm, wg_v, 2, BA, 3)
    get_cols(wu_hbm, wu_v, 2, BA, 3)
    get_wd(0, BA, 3)
    get_x(TA, TA, 4)
    get_w(0, CPU, 4)
    get_x(2 * TA, TA, 5)
    get_w(CPU, 2 * CPU, 5)
    get_x(3 * TA, TA, 6)
    get_w(2 * CPU, 3 * CPU, 6)
    get_cols(wg_hbm, wg_v, BA, NFA, 7)
    get_cols(wu_hbm, wu_v, BA, NFA, 7)
    get_wd(BA, NFA, 7)
    get_w(3 * CPU, NCH, 7)
    start(gw_hbm, gw_v, 8)
    get_wd(NFA, NF, 8)
    get_cols(wg_hbm, wg_v, NFA, NF, 8)

    wg_u, wu_u, wd_u = (r.bitcast(u32) for r in (wg_v, wu_v, wd_v))

    zero_s[0] = 0
    qkv_s[pl.ds(NB, 2 * NB), pl.ds(0, HALO), :] = jnp.zeros((2 * NB, HALO, 128), f32)

    def repack(ch):
        p = jax.lax.shift_right_logical(ch, 3)
        rc = ch & 7
        on = jnp.where(ch < 24, -1, 0).astype(i32)
        r0 = pl.multiple_of(rc * 128, 128)
        blk = [pltpu.bitcast(w_v[p, pl.ds(r0, 128), pl.ds(128 * j, 128)], u32) for j in range(NB)]
        lane = _lane((64, 128))
        for bb, lb in ((2, 3), (1, 2), (0, 1)):
            sh = 1 << lb
            keep_a = (lane & (on & sh)) == 0
            take_a = ((lane & sh) | (~on & 1)) == 0
            for j in range(NB):
                if j & (1 << bb):
                    continue
                a, b = blk[j], blk[j | (1 << bb)]
                blk[j] = jnp.where(keep_a, a, pltpu.roll(b, sh, 1))
                blk[j | (1 << bb)] = jnp.where(take_a, pltpu.roll(a, 128 - sh, 1), b)
        for j in range(NB):
            w_p[p, j, pl.ds(rc * PITCH, 64), :] = blk[j]

    wait(0, xrows(0, 256), wg_v.at[pl.ds(0, 2)])
    g_a = _dot(x_v[pl.ds(0, 256), :], _cat([wg_u[0], wg_u[1]]))
    wait(1, xrows(256, 256))
    g_b = _dot(x_v[pl.ds(256, 256), :], _cat([wg_u[0], wg_u[1]]))
    wait(2, wu_v.at[pl.ds(0, 2)])
    x0 = x_v[pl.ds(0, TA), :]
    h0 = _reglu(jnp.concatenate([g_a, g_b], axis=0), _dot(x0, _cat([wu_u[0], wu_u[1]])))
    wait(3, wg_v.at[2], wu_v.at[2], wd_rows(0, BA))
    h1 = _reglu(_dot(x0, _cat([wg_u[2]])), _dot(x0, _cat([wu_u[2]])))
    bacc[0, pl.ds(0, TA), :] = _dot(_cat([h0, h1]),
                                    _cat([wd_u[j, pl.ds(0, 64 * BA), :] for j in range(NB)]))
    get_cols(wu_hbm, wu_v, NFA, NF, 8)

    def phase_a(u, carry):
        pl.when(u == 1)(lambda: wait(4, xrows(TA, TA), *w_dst(0, CPU)))
        pl.when(u == 2)(lambda: wait(5, xrows(2 * TA, TA), *w_dst(CPU, 2 * CPU)))
        pl.when(u == 3)(lambda: wait(6, xrows(3 * TA, TA), *w_dst(2 * CPU, 3 * CPU)))
        pl.when(u == 4)(lambda: wait(7, wg_v.at[pl.ds(BA, BA)], wu_v.at[pl.ds(BA, BA)],
                                     wd_rows(BA, NFA), *w_dst(3 * CPU, NCH)))
        c = jax.lax.shift_right_logical(u, 2)
        a = pl.multiple_of((u & 3) * TA, TA)
        x = x_v[pl.ds(a, TA), :]
        h = _reglu(_dot(x, _cat([wg_u[c * BA + k] for k in range(BA)])),
                   _dot(x, _cat([wu_u[c * BA + k] for k in range(BA)])))
        for k in range(CPU):
            repack(jnp.minimum(CPU * (u - 1) + k, NCH - 1))
        r = pl.multiple_of(c * (64 * BA), 64)
        bacc[c, pl.ds(a, TA), :] = _dot(_cat([h]), _cat([wd_u[j, pl.ds(r, 64 * BA), :] for j in range(NB)]))
        return carry

    jax.lax.fori_loop(1, NA, phase_a, 0)
    wait(8, gw_v, wg_v.at[pl.ds(NFA, NF - NFA)], wu_v.at[pl.ds(NFA, NF - NFA)], wd_rows(NFA, NF))

    m16 = (_lane((RG, 128)) & 16) == 0
    m1 = (_lane((RG, 128)) & 1) == 0

    def attend(r0, base, scale):
        q = [qkv_s[j, pl.ds(HALO + r0, RG), :] * scale for j in range(NB)]
        logits = []
        for w in range(WIN):
            off = HALO + r0 - DIL * w
            acc = q[0] * qkv_s[NB, pl.ds(off, RG), :]
            for j in range(1, NB):
                acc = acc + q[j] * qkv_s[NB + j, pl.ds(off, RG), :]
            acc = acc + jnp.where(m16, pltpu.roll(acc, 128 - 16, 1), pltpu.roll(acc, 16, 1))
            acc = acc + jnp.where(m1, pltpu.roll(acc, 128 - 1, 1), pltpu.roll(acc, 1, 1))
            if r0 < DIL * w:
                pos = base + r0 + jax.lax.broadcasted_iota(i32, (RG, 128), 0)
                acc = jnp.where(pos >= DIL * w, acc, NEG)
            logits.append(acc)
        m = logits[0]
        for w in range(1, WIN):
            m = jnp.maximum(m, logits[w])
        e = [jnp.exp2(l - m) for l in logits]
        s = e[0]
        for w in range(1, WIN):
            s = s + e[w]
        inv = pl.reciprocal(s, approx=True)
        inv = inv * (2.0 - s * inv)
        p = [x * inv for x in e]
        for j in range(NB):
            o = p[0] * qkv_s[2 * NB + j, pl.ds(HALO + r0, RG), :]
            for w in range(1, WIN):
                o = o + p[w] * qkv_s[2 * NB + j, pl.ds(HALO + r0 - DIL * w, RG), :]
            o_s[j, pl.ds(r0, RG), :] = o

    def phase_b(t, carry):
        base = pl.multiple_of(t * TB, TB)
        zero = zero_s[0]
        zvec = jnp.full((RG, 128), zero, i32)
        sbits = pltpu.bitcast(jnp.full((RG, 128), SCALE, f32), i32)
        x = x_v[pl.ds(base, TB), :]
        gw = pltpu.bitcast(jnp.broadcast_to(gw_v[...].astype(f32).reshape(1, D), (8, D)), i32)

        gates = []

        def gate_rows(r0, anchor):
            dep = pltpu.bitcast(anchor, i32) & zvec
            xr = x[r0:r0 + 16, :].astype(f32)
            acc = None
            for j in range(NB):
                w = pltpu.bitcast(gw[:, 128 * j:128 * (j + 1)] | dep, f32)
                term = xr[:, 128 * j:128 * (j + 1)] * jnp.concatenate([w, w], axis=0)
                acc = term if acc is None else acc + term
            z = jnp.sum(acc, axis=-1, keepdims=True)
            gates.append(jnp.broadcast_to(jax.nn.sigmoid(z), (16, 128)))

        for i in range(3):
            r = _dot(x, _cat([jnp.concatenate([w_p[i, j, pl.ds(PITCH * c, 64), :] for c in range(8)],
                                              axis=0) for j in range(NB)]))
            for j in range(NB):
                qkv_s[i * NB + j, pl.ds(HALO, TB), :] = r[:, 128 * j:128 * (j + 1)]
                if i * NB + j < TB // 16:
                    gate_rows(16 * (i * NB + j), r[ANCH:ANCH + 8, 128 * j:128 * (j + 1)])
        groups = list(range(0, TB, RG))
        nslots = 2 * (NF - NFA) - NSK
        hs = []
        slot = 0
        done = 0

        def release(anchor):
            nonlocal slot, done
            slot += 1
            want = min(len(groups), -(-slot * len(groups) // nslots))
            if want > done:
                for r0 in groups[done:want]:
                    dep = pltpu.bitcast(anchor, i32)
                    if GDEP:
                        dep = dep | pltpu.bitcast(gates[r0 // 16][r0 % 16:r0 % 16 + 8], i32)
                    attend(r0, base, pltpu.bitcast(sbits | (dep & zvec), f32))
                done = want

        for c in range(NFA, NF, 2):
            g = _dot(x, _cat([wg_u[c], wg_u[c + 1]]))
            for n in range(2):
                release(g[ANCH:ANCH + 8, 128 * n:128 * (n + 1)])
            u = _dot(x, _cat([wu_u[c], wu_u[c + 1]]))
            for n in range(2):
                release(u[ANCH:ANCH + 8, 128 * n:128 * (n + 1)])
            hs.append(_reglu(g, u))
        assert done == len(groups)
        qkv_s[pl.ds(NB, 2 * NB), pl.ds(0, HALO), :] = qkv_s[pl.ds(NB, 2 * NB), pl.ds(TB, HALO), :]
        g = jnp.concatenate(gates, axis=0)
        g1 = 1.0 - g

        def down():
            wd = _cat([wd_u[j, pl.ds(64 * NFA, 64 * (NF - NFA)), :] for j in range(NB)])
            return (bacc[0, pl.ds(base, TB), :] + bacc[1, pl.ds(base, TB), :]
                    + _dot(_cat(hs), wd))

        if ORDER == 1:
            b = down()
        wo = _cat([jnp.concatenate([w_p[3, j, pl.ds(8 * m + c, 8, stride=PITCH), :]
                                    for c in range(8) for m in range(8)], axis=0)
                   for j in range(NB)])
        o_s[0, pl.ds(TB + zero, 8), :] = jnp.zeros((8, 128), f32)
        o = jnp.concatenate([o_s[j, pl.ds(0, TB), :] for j in range(NB)], axis=1)
        a = _dot(o.astype(bf16), wo)
        if ORDER == 0:
            b = down()
        for c0, c1 in OUTP:
            n = c1 - c0
            res = (jnp.concatenate([g] * (n // 128), axis=1) * a[:, c0:c1]
                   + jnp.concatenate([g1] * (n // 128), axis=1) * b[:, c0:c1])
            out_v[pl.ds(base, TB), pl.ds(c0, n)] = res.astype(bf16)
            start(out_v.at[pl.ds(base, TB), pl.ds(c0, n)], out_hbm.at[pl.ds(base, TB), pl.ds(c0, n)], 9)
        return carry

    with _scope("B"):
        jax.lax.fori_loop(0, S // TB, phase_b, 0)
    wait(9, out_v)


@jax.jit
def pallas_gated_mix__sliding_local_dilated__glu_gated_reglu__prompt_kernel(
    A_x: jax.Array,
    A_wqkv: jax.Array,
    A_wo: jax.Array,
    B_x: jax.Array,
    B_W_gate: jax.Array,
    B_W_up: jax.Array,
    B_W_down: jax.Array,
    gate_w: jax.Array,
):
    del B_x
    x = A_x.reshape(S, D)
    hbm = pl.BlockSpec(memory_space=pl.ANY)
    out = pl.pallas_call(
        _kernel,
        out_shape=jax.ShapeDtypeStruct((S, D), bf16),
        in_specs=[hbm] * 7,
        out_specs=hbm,
        scratch_shapes=[
            pltpu.VMEM((S, D), bf16),
            pltpu.VMEM((4, D, D), bf16),
            pltpu.VMEM((NF, D, 128), bf16),
            pltpu.VMEM((NF, D, 128), bf16),
            pltpu.VMEM((NB, F, 128), bf16),
            pltpu.VMEM((D,), bf16),
            pltpu.VMEM((4, NB, 8 * PITCH, 128), u32),
            pltpu.VMEM((2, S, D), f32),
            pltpu.VMEM((3 * NB, HALO + TB + 8, 128), f32),
            pltpu.VMEM((NB, TB + 8, 128), f32),
            pltpu.VMEM((S, D), bf16),
            pltpu.SMEM((1,), i32),
            pltpu.SemaphoreType.DMA((10,)),
        ],
        compiler_params=pltpu.CompilerParams(
            vmem_limit_bytes=110 * 1024 * 1024,
            disable_bounds_checks=not CHECKS,
            disable_semaphore_checks=not CHECKS,
        ),
    )(x, A_wqkv, A_wo, B_W_gate, B_W_up, B_W_down, gate_w)
    return out.reshape(1, S, D)
```

```python
import os
import jax
import jax.numpy as jnp
import jax.experimental.pallas as pl
import jax.experimental.pallas.tpu as pltpu

S, D, F = 2048, 1024, 3584
H, DH, WIN, DIL = 32, 32, 8, 2
NB = D // 128
NF = F // 128
HALO = 16
BA = 3
NFA = 2 * BA
TA = 512
NA = (S // TA) * 2
TB = 256
RG = 8
ANCH = int(os.environ.get('ANCH', 248))
NSK = int(os.environ.get('NSK', 2))
ORDER = int(os.environ.get('ORDER', 0))
OUTP = ((0, 512), (512, 768), (768, 1024))
GDEP = int(os.environ.get('GDEP', 1))
PVS = int(os.environ.get('PVS', 2))
LGS = int(os.environ.get('LGS', 4))
SCOPES = int(os.environ.get("SCOPES", 0))
CHECKS = int(os.environ.get("CHECKS", 0))
PITCH = 65
CPU = 5
NCH = 4 * 8
LOG2E = 1.4426950408889634
SCALE = DH ** -0.5 * LOG2E
NEG = -1e9 * LOG2E

f32 = jnp.float32
bf16 = jnp.bfloat16
u32 = jnp.uint32
i32 = jnp.int32


def _dot(a, b):
    return jnp.dot(a, b, preferred_element_type=f32)


def _lane(shape):
    return jax.lax.broadcasted_iota(i32, shape, 1)


def _cat(blocks):
    return jnp.concatenate([pltpu.bitcast(b, bf16) for b in blocks], axis=1)


def _reglu(g, u):
    return pltpu.bitcast((jnp.maximum(g, 0.0) * u).astype(bf16), u32)


class _NoScope:
    def __enter__(self):
        return self

    def __exit__(self, *a):
        return False


def _scope(name):
    return jax.named_scope(name) if SCOPES else _NoScope()


def _kernel(x_hbm, wqkv_hbm, wo_hbm, wg_hbm, wu_hbm, wd_hbm, gw_hbm, out_hbm,
            x_v, w_v, wg_v, wu_v, wd_v, gw_v, w_p, bacc,
            qkv_s, o_s, out_v, zero_s, sems):
    def start(src, dst, grp):
        pltpu.make_async_copy(src, dst, sems.at[grp]).start()

    def wait(grp, *dsts):
        with _scope("w%d" % grp):
            for d in dsts:
                pltpu.make_async_copy(d, d, sems.at[grp]).wait()

    def xrows(a, n):
        return x_v.at[pl.ds(a, n), :]

    def get_x(a, n, grp):
        start(x_hbm.at[pl.ds(a, n), :], xrows(a, n), grp)

    def get_cols(hbm, dst, b0, b1, grp):
        for b in range(b0, b1):
            start(hbm.at[:, pl.ds(128 * b, 128)], dst.at[b], grp)

    def wd_rows(b0, b1):
        return wd_v.at[:, pl.ds(128 * b0, 128 * (b1 - b0)), :]

    def get_wd(b0, b1, grp):
        for j in range(NB):
            start(wd_hbm.at[pl.ds(128 * b0, 128 * (b1 - b0)), pl.ds(128 * j, 128)],
                  wd_v.at[j, pl.ds(128 * b0, 128 * (b1 - b0)), :], grp)

    def w_rows(c0, c1):
        out = []
        for p in range(4):
            a, b = max(c0, 8 * p), min(c1, 8 * p + 8)
            if a < b:
                out.append((p, 128 * (a - 8 * p), 128 * (b - a)))
        return out

    def w_dst(c0, c1):
        return [w_v.at[p, pl.ds(r, n), :] for p, r, n in w_rows(c0, c1)]

    def get_w(c0, c1, grp):
        for p, r, n in w_rows(c0, c1):
            src = (wqkv_hbm.at[pl.ds(r, n), pl.ds(p * D, D)] if p < 3
                   else wo_hbm.at[pl.ds(r, n), :])
            start(src, w_v.at[p, pl.ds(r, n), :], grp)

    get_x(0, 256, 0)
    get_cols(wg_hbm, wg_v, 0, 2, 0)
    get_x(256, 256, 1)
    get_cols(wu_hbm, wu_v, 0, 2, 2)
    get_cols(wg_hbm, wg_v, 2, BA, 3)
    get_cols(wu_hbm, wu_v, 2, BA, 3)
    get_wd(0, BA, 3)
    get_x(TA, TA, 4)
    get_w(0, CPU, 4)
    get_x(2 * TA, TA, 5)
    get_w(CPU, 2 * CPU, 5)
    get_x(3 * TA, TA, 6)
    get_w(2 * CPU, 3 * CPU, 6)
    get_cols(wg_hbm, wg_v, BA, NFA, 7)
    get_cols(wu_hbm, wu_v, BA, NFA, 7)
    get_wd(BA, NFA, 7)
    get_w(3 * CPU, NCH, 7)
    start(gw_hbm, gw_v, 8)
    get_wd(NFA, NF, 8)
    get_cols(wg_hbm, wg_v, NFA, NF, 8)

    wg_u, wu_u, wd_u = (r.bitcast(u32) for r in (wg_v, wu_v, wd_v))

    zero_s[0] = 0
    qkv_s[pl.ds(NB, 2 * NB), pl.ds(0, HALO), :] = jnp.zeros((2 * NB, HALO, 128), f32)

    def repack(ch):
        p = jax.lax.shift_right_logical(ch, 3)
        rc = ch & 7
        on = jnp.where(ch < 24, -1, 0).astype(i32)
        r0 = pl.multiple_of(rc * 128, 128)
        blk = [pltpu.bitcast(w_v[p, pl.ds(r0, 128), pl.ds(128 * j, 128)], u32) for j in range(NB)]
        lane = _lane((64, 128))
        for bb, lb in ((2, 3), (1, 2), (0, 1)):
            sh = 1 << lb
            keep_a = (lane & (on & sh)) == 0
            take_a = ((lane & sh) | (~on & 1)) == 0
            for j in range(NB):
                if j & (1 << bb):
                    continue
                a, b = blk[j], blk[j | (1 << bb)]
                blk[j] = jnp.where(keep_a, a, pltpu.roll(b, sh, 1))
                blk[j | (1 << bb)] = jnp.where(take_a, pltpu.roll(a, 128 - sh, 1), b)
        for j in range(NB):
            w_p[p, j, pl.ds(rc * PITCH, 64), :] = blk[j]

    wait(0, xrows(0, 256), wg_v.at[pl.ds(0, 2)])
    g_a = _dot(x_v[pl.ds(0, 256), :], _cat([wg_u[0], wg_u[1]]))
    wait(1, xrows(256, 256))
    g_b = _dot(x_v[pl.ds(256, 256), :], _cat([wg_u[0], wg_u[1]]))
    wait(2, wu_v.at[pl.ds(0, 2)])
    x0 = x_v[pl.ds(0, TA), :]
    h0 = _reglu(jnp.concatenate([g_a, g_b], axis=0), _dot(x0, _cat([wu_u[0], wu_u[1]])))
    wait(3, wg_v.at[2], wu_v.at[2], wd_rows(0, BA))
    h1 = _reglu(_dot(x0, _cat([wg_u[2]])), _dot(x0, _cat([wu_u[2]])))
    bacc[0, pl.ds(0, TA), :] = _dot(_cat([h0, h1]),
                                    _cat([wd_u[j, pl.ds(0, 64 * BA), :] for j in range(NB)]))
    get_cols(wu_hbm, wu_v, NFA, NF, 8)

    def phase_a(u, carry):
        pl.when(u == 1)(lambda: wait(4, xrows(TA, TA), *w_dst(0, CPU)))
        pl.when(u == 2)(lambda: wait(5, xrows(2 * TA, TA), *w_dst(CPU, 2 * CPU)))
        pl.when(u == 3)(lambda: wait(6, xrows(3 * TA, TA), *w_dst(2 * CPU, 3 * CPU)))
        pl.when(u == 4)(lambda: wait(7, wg_v.at[pl.ds(BA, BA)], wu_v.at[pl.ds(BA, BA)],
                                     wd_rows(BA, NFA), *w_dst(3 * CPU, NCH)))
        c = jax.lax.shift_right_logical(u, 2)
        a = pl.multiple_of((u & 3) * TA, TA)
        x = x_v[pl.ds(a, TA), :]
        h = _reglu(_dot(x, _cat([wg_u[c * BA + k] for k in range(BA)])),
                   _dot(x, _cat([wu_u[c * BA + k] for k in range(BA)])))
        for k in range(CPU):
            repack(jnp.minimum(CPU * (u - 1) + k, NCH - 1))
        r = pl.multiple_of(c * (64 * BA), 64)
        bacc[c, pl.ds(a, TA), :] = _dot(_cat([h]), _cat([wd_u[j, pl.ds(r, 64 * BA), :] for j in range(NB)]))
        return carry

    jax.lax.fori_loop(1, NA, phase_a, 0)
    wait(8, gw_v, wg_v.at[pl.ds(NFA, NF - NFA)], wu_v.at[pl.ds(NFA, NF - NFA)], wd_rows(NFA, NF))

    m16 = (_lane((RG, 128)) & 16) == 0
    m1 = (_lane((RG, 128)) & 1) == 0

    def attend(r0, base, scale, zvec):
        logits = []
        for w in range(WIN):
            if w % LGS == 0:
                if w:
                    scale = pltpu.bitcast(
                        pltpu.bitcast(scale, i32) | (pltpu.bitcast(raw, i32) & zvec), f32)
                q = [qkv_s[j, pl.ds(HALO + r0, RG), :] * scale for j in range(NB)]
            off = HALO + r0 - DIL * w
            acc = q[0] * qkv_s[NB, pl.ds(off, RG), :]
            for j in range(1, NB):
                acc = acc + q[j] * qkv_s[NB + j, pl.ds(off, RG), :]
            raw = acc
            acc = acc + jnp.where(m16, pltpu.roll(acc, 128 - 16, 1), pltpu.roll(acc, 16, 1))
            acc = acc + jnp.where(m1, pltpu.roll(acc, 128 - 1, 1), pltpu.roll(acc, 1, 1))
            if r0 < DIL * w:
                pos = base + r0 + jax.lax.broadcasted_iota(i32, (RG, 128), 0)
                acc = jnp.where(pos >= DIL * w, acc, NEG)
            logits.append(acc)
        m = logits[0]
        for w in range(1, WIN):
            m = jnp.maximum(m, logits[w])
        e = [jnp.exp2(l - m) for l in logits]
        s = e[0]
        for w in range(1, WIN):
            s = s + e[w]
        inv = pl.reciprocal(s, approx=True)
        inv = inv * (2.0 - s * inv)
        for j in range(NB):
            if j % PVS == 0:
                if j:
                    inv = pltpu.bitcast(pltpu.bitcast(inv, i32) | (pltpu.bitcast(o, i32) & zvec), f32)
                p = [x * inv for x in e]
            o = p[0] * qkv_s[2 * NB + j, pl.ds(HALO + r0, RG), :]
            for w in range(1, WIN):
                o = o + p[w] * qkv_s[2 * NB + j, pl.ds(HALO + r0 - DIL * w, RG), :]
            o_s[j, pl.ds(r0, RG), :] = o

    def phase_b(t, carry):
        base = pl.multiple_of(t * TB, TB)
        zero = zero_s[0]
        zvec = jnp.full((RG, 128), zero, i32)
        sbits = pltpu.bitcast(jnp.full((RG, 128), SCALE, f32), i32)
        x = x_v[pl.ds(base, TB), :]
        gw = pltpu.bitcast(jnp.broadcast_to(gw_v[...].astype(f32).reshape(1, D), (8, D)), i32)

        gates = []

        def gate_rows(r0, anchor):
            dep = pltpu.bitcast(anchor, i32) & zvec
            xr = x[r0:r0 + 16, :].astype(f32)
            acc = None
            for j in range(NB):
                w = pltpu.bitcast(gw[:, 128 * j:128 * (j + 1)] | dep, f32)
                term = xr[:, 128 * j:128 * (j + 1)] * jnp.concatenate([w, w], axis=0)
                acc = term if acc is None else acc + term
            z = jnp.sum(acc, axis=-1, keepdims=True)
            gates.append(jnp.broadcast_to(jax.nn.sigmoid(z), (16, 128)))

        for i in range(3):
            r = _dot(x, _cat([jnp.concatenate([w_p[i, j, pl.ds(PITCH * c, 64), :] for c in range(8)],
                                              axis=0) for j in range(NB)]))
            for j in range(NB):
                qkv_s[i * NB + j, pl.ds(HALO, TB), :] = r[:, 128 * j:128 * (j + 1)]
                if i * NB + j < TB // 16:
                    gate_rows(16 * (i * NB + j), r[ANCH:ANCH + 8, 128 * j:128 * (j + 1)])
        groups = list(range(0, TB, RG))
        nslots = 2 * (NF - NFA) - NSK
        hs = []
        slot = 0
        done = 0

        def release(anchor):
            nonlocal slot, done
            slot += 1
            want = min(len(groups), -(-slot * len(groups) // nslots))
            if want > done:
                for r0 in groups[done:want]:
                    dep = pltpu.bitcast(anchor, i32)
                    if GDEP:
                        dep = dep | pltpu.bitcast(gates[r0 // 16][r0 % 16:r0 % 16 + 8], i32)
                    attend(r0, base, pltpu.bitcast(sbits | (dep & zvec), f32), zvec)
                done = want

        for c in range(NFA, NF, 2):
            g = _dot(x, _cat([wg_u[c], wg_u[c + 1]]))
            for n in range(2):
                release(g[ANCH:ANCH + 8, 128 * n:128 * (n + 1)])
            u = _dot(x, _cat([wu_u[c], wu_u[c + 1]]))
            for n in range(2):
                release(u[ANCH:ANCH + 8, 128 * n:128 * (n + 1)])
            hs.append(_reglu(g, u))
        assert done == len(groups)
        qkv_s[pl.ds(NB, 2 * NB), pl.ds(0, HALO), :] = qkv_s[pl.ds(NB, 2 * NB), pl.ds(TB, HALO), :]
        g = jnp.concatenate(gates, axis=0)
        g1 = 1.0 - g

        def down():
            wd = _cat([wd_u[j, pl.ds(64 * NFA, 64 * (NF - NFA)), :] for j in range(NB)])
            return (bacc[0, pl.ds(base, TB), :] + bacc[1, pl.ds(base, TB), :]
                    + _dot(_cat(hs), wd))

        if ORDER == 1:
            b = down()
        wo = _cat([jnp.concatenate([w_p[3, j, pl.ds(8 * m + c, 8, stride=PITCH), :]
                                    for c in range(8) for m in range(8)], axis=0)
                   for j in range(NB)])
        o_s[0, pl.ds(TB + zero, 8), :] = jnp.zeros((8, 128), f32)
        o = jnp.concatenate([o_s[j, pl.ds(0, TB), :] for j in range(NB)], axis=1)
        a = _dot(o.astype(bf16), wo)
        if ORDER == 0:
            b = down()
        for c0, c1 in OUTP:
            n = c1 - c0
            res = (jnp.concatenate([g] * (n // 128), axis=1) * a[:, c0:c1]
                   + jnp.concatenate([g1] * (n // 128), axis=1) * b[:, c0:c1])
            out_v[pl.ds(base, TB), pl.ds(c0, n)] = res.astype(bf16)
            start(out_v.at[pl.ds(base, TB), pl.ds(c0, n)], out_hbm.at[pl.ds(base, TB), pl.ds(c0, n)], 9)
        return carry

    with _scope("B"):
        jax.lax.fori_loop(0, S // TB, phase_b, 0)
    wait(9, out_v)


@jax.jit
def pallas_gated_mix__sliding_local_dilated__glu_gated_reglu__prompt_kernel(
    A_x: jax.Array,
    A_wqkv: jax.Array,
    A_wo: jax.Array,
    B_x: jax.Array,
    B_W_gate: jax.Array,
    B_W_up: jax.Array,
    B_W_down: jax.Array,
    gate_w: jax.Array,
):
    del B_x
    x = A_x.reshape(S, D)
    hbm = pl.BlockSpec(memory_space=pl.ANY)
    out = pl.pallas_call(
        _kernel,
        out_shape=jax.ShapeDtypeStruct((S, D), bf16),
        in_specs=[hbm] * 7,
        out_specs=hbm,
        scratch_shapes=[
            pltpu.VMEM((S, D), bf16),
            pltpu.VMEM((4, D, D), bf16),
            pltpu.VMEM((NF, D, 128), bf16),
            pltpu.VMEM((NF, D, 128), bf16),
            pltpu.VMEM((NB, F, 128), bf16),
            pltpu.VMEM((D,), bf16),
            pltpu.VMEM((4, NB, 8 * PITCH, 128), u32),
            pltpu.VMEM((2, S, D), f32),
            pltpu.VMEM((3 * NB, HALO + TB + 8, 128), f32),
            pltpu.VMEM((NB, TB + 8, 128), f32),
            pltpu.VMEM((S, D), bf16),
            pltpu.SMEM((1,), i32),
            pltpu.SemaphoreType.DMA((10,)),
        ],
        compiler_params=pltpu.CompilerParams(
            vmem_limit_bytes=110 * 1024 * 1024,
            disable_bounds_checks=not CHECKS,
            disable_semaphore_checks=not CHECKS,
        ),
    )(x, A_wqkv, A_wo, B_W_gate, B_W_up, B_W_down, gate_w)
    return out.reshape(1, S, D)
```

```python
import os
import jax
import jax.numpy as jnp
import jax.experimental.pallas as pl
import jax.experimental.pallas.tpu as pltpu

S, D, F = 2048, 1024, 3584
H, DH, WIN, DIL = 32, 32, 8, 2
NB = D // 128
NF = F // 128
HALO = 16
BA = 3
NFA = 2 * BA
TA = 512
NA = (S // TA) * 2
TB = 256
RG = 8
ANCH = int(os.environ.get('ANCH', 248))
NSK = int(os.environ.get('NSK', 2))
ORDER = int(os.environ.get('ORDER', 0))
OUTP = {0: ((0, 256, 0, 512), (0, 256, 512, 768), (0, 256, 768, 1024)),
        1: ((0, 256, 0, 512), (0, 256, 512, 768), (0, 192, 768, 1024), (192, 256, 768, 1024)),
        2: ((0, 256, 0, 512), (0, 256, 512, 896), (0, 192, 896, 1024), (192, 256, 896, 1024)),
        3: ((0, 256, 0, 768), (0, 128, 768, 1024), (128, 224, 768, 1024), (224, 256, 768, 1024)),
        }[int(os.environ.get('OUTP', 2))]
GDEP = int(os.environ.get('GDEP', 1))
PVS = int(os.environ.get('PVS', 2))
LGS = int(os.environ.get('LGS', 4))
P0M = int(os.environ.get('P0M', 0))
SCOPES = int(os.environ.get("SCOPES", 0))
CHECKS = int(os.environ.get("CHECKS", 0))
PITCH = 65
CPU = 5
NCH = 4 * 8
LOG2E = 1.4426950408889634
SCALE = DH ** -0.5 * LOG2E
NEG = -1e9 * LOG2E

f32 = jnp.float32
bf16 = jnp.bfloat16
u32 = jnp.uint32
i32 = jnp.int32


def _dot(a, b):
    return jnp.dot(a, b, preferred_element_type=f32)


def _lane(shape):
    return jax.lax.broadcasted_iota(i32, shape, 1)


def _cat(blocks):
    return jnp.concatenate([pltpu.bitcast(b, bf16) for b in blocks], axis=1)


def _reglu(g, u):
    return pltpu.bitcast((jnp.maximum(g, 0.0) * u).astype(bf16), u32)


class _NoScope:
    def __enter__(self):
        return self

    def __exit__(self, *a):
        return False


def _scope(name):
    return jax.named_scope(name) if SCOPES else _NoScope()


def _kernel(x_hbm, wqkv_hbm, wo_hbm, wg_hbm, wu_hbm, wd_hbm, gw_hbm, out_hbm,
            x_v, w_v, wg_v, wu_v, wda_v, wd_v, gw_v, w_p, bacc,
            qkv_s, o_s, out_v, zero_s, sems):
    def start(src, dst, grp):
        pltpu.make_async_copy(src, dst, sems.at[grp]).start()

    def wait(grp, *dsts):
        with _scope("w%d" % grp):
            for d in dsts:
                pltpu.make_async_copy(d, d, sems.at[grp]).wait()

    def xrows(a, n):
        return x_v.at[pl.ds(a, n), :]

    def get_x(a, n, grp):
        start(x_hbm.at[pl.ds(a, n), :], xrows(a, n), grp)

    def get_cols(hbm, dst, b0, b1, grp):
        for b in range(b0, b1):
            start(hbm.at[:, pl.ds(128 * b, 128)], dst.at[b], grp)

    def wda_rows(b0, b1):
        return wda_v.at[pl.ds(128 * b0, 128 * (b1 - b0)), :]

    def get_wda(b0, b1, grp):
        start(wd_hbm.at[pl.ds(128 * b0, 128 * (b1 - b0)), :], wda_rows(b0, b1), grp)

    def w_rows(c0, c1):
        out = []
        for p in range(4):
            a, b = max(c0, 8 * p), min(c1, 8 * p + 8)
            if a < b:
                out.append((p, 128 * (a - 8 * p), 128 * (b - a)))
        return out

    def w_dst(c0, c1):
        return [w_v.at[p, pl.ds(r, n), :] for p, r, n in w_rows(c0, c1)]

    def get_w(c0, c1, grp):
        for p, r, n in w_rows(c0, c1):
            src = (wqkv_hbm.at[pl.ds(r, n), pl.ds(p * D, D)] if p < 3
                   else wo_hbm.at[pl.ds(r, n), :])
            start(src, w_v.at[p, pl.ds(r, n), :], grp)

    get_x(0, 128, 0)
    get_cols(wg_hbm, wg_v, 0, 1, 0)
    get_x(128, 128, 1)
    get_cols(wu_hbm, wu_v, 0, 1, 2)
    get_x(256, 128, 3)
    get_cols(wg_hbm, wg_v, 1, 2, 4)
    get_x(384, 128, 5)
    get_cols(wu_hbm, wu_v, 1, 2, 5)
    get_cols(wg_hbm, wg_v, 2, 3, 6)
    get_cols(wu_hbm, wu_v, 2, 3, 6)
    get_wda(0, 2, 6)
    get_wda(2, 3, 7)
    get_x(TA, TA, 8)
    get_w(0, CPU, 8)
    get_x(2 * TA, TA, 9)
    get_w(CPU, 2 * CPU, 9)
    get_x(3 * TA, TA, 10)
    get_w(2 * CPU, 3 * CPU, 10)
    get_cols(wg_hbm, wg_v, BA, NFA, 11)
    get_cols(wu_hbm, wu_v, BA, NFA, 11)
    get_wda(BA, NFA, 11)
    get_w(3 * CPU, NCH, 11)
    start(gw_hbm, gw_v, 12)
    for j in range(NB):
        start(wd_hbm.at[pl.ds(128 * NFA, F - 128 * NFA), pl.ds(128 * j, 128)], wd_v.at[j], 12)
    get_cols(wg_hbm, wg_v, NFA, NF, 12)

    wg_u, wu_u, wd_u = (r.bitcast(u32) for r in (wg_v, wu_v, wd_v))

    zero_s[0] = 0
    qkv_s[pl.ds(NB, 2 * NB), pl.ds(0, HALO), :] = jnp.zeros((2 * NB, HALO, 128), f32)

    def repack(ch):
        p = jax.lax.shift_right_logical(ch, 3)
        rc = ch & 7
        on = jnp.where(ch < 24, -1, 0).astype(i32)
        r0 = pl.multiple_of(rc * 128, 128)
        blk = [pltpu.bitcast(w_v[p, pl.ds(r0, 128), pl.ds(128 * j, 128)], u32) for j in range(NB)]
        lane = _lane((64, 128))
        for bb, lb in ((2, 3), (1, 2), (0, 1)):
            sh = 1 << lb
            keep_a = (lane & (on & sh)) == 0
            take_a = ((lane & sh) | (~on & 1)) == 0
            for j in range(NB):
                if j & (1 << bb):
                    continue
                a, b = blk[j], blk[j | (1 << bb)]
                blk[j] = jnp.where(keep_a, a, pltpu.roll(b, sh, 1))
                blk[j | (1 << bb)] = jnp.where(take_a, pltpu.roll(a, 128 - sh, 1), b)
        for j in range(NB):
            w_p[p, j, pl.ds(rc * PITCH, 64), :] = blk[j]

    def xr(a, b):
        return x_v[pl.ds(a, b - a), :]

    def rcat(*parts):
        return jnp.concatenate(parts, axis=0)

    wait(0, xrows(0, 128), wg_v.at[0])
    g0a = _dot(xr(0, 128), _cat([wg_u[0]]))
    wait(1, xrows(128, 128))
    g0b = _dot(xr(128, 256), _cat([wg_u[0]]))
    wait(2, wu_v.at[0])
    h0a = _reglu(rcat(g0a, g0b), _dot(xr(0, 256), _cat([wu_u[0]])))
    wait(3, xrows(256, 128))
    gu = _dot(xr(256, 384), _cat([wg_u[0], wu_u[0]]))
    h0b = _reglu(gu[:, :128], gu[:, 128:])
    wait(4, wg_v.at[1])
    g1a = _dot(xr(0, 384), _cat([wg_u[1]]))
    wait(5, xrows(384, 128), wu_v.at[1])
    gu = _dot(xr(384, 512), _cat([wg_u[0], wu_u[0], wg_u[1]]))
    h0c = _reglu(gu[:, :128], gu[:, 128:256])
    h1 = _reglu(rcat(g1a, gu[:, 256:]), _dot(xr(0, TA), _cat([wu_u[1]])))
    if P0M:
        wait(6, wg_v.at[2], wu_v.at[2], wda_rows(0, 2))
        wait(7, wda_rows(2, 3))
    else:
        wait(6, wg_v.at[2], wu_v.at[2], wda_rows(0, 2))
    gu = _dot(xr(0, TA), _cat([wg_u[2], wu_u[2]]))
    h2 = _reglu(gu[:, :128], gu[:, 128:])
    get_cols(wu_hbm, wu_v, NFA, NF, 12)
    if not P0M:
        wait(7, wda_rows(2, 3))
    bacc[0, pl.ds(0, TA), :] = _dot(_cat([rcat(h0a, h0b, h0c), h1, h2]), wda_v[pl.ds(0, 128 * BA), :])

    def phase_a(u, carry):
        pl.when(u == 1)(lambda: wait(8, xrows(TA, TA), *w_dst(0, CPU)))
        pl.when(u == 2)(lambda: wait(9, xrows(2 * TA, TA), *w_dst(CPU, 2 * CPU)))
        pl.when(u == 3)(lambda: wait(10, xrows(3 * TA, TA), *w_dst(2 * CPU, 3 * CPU)))
        pl.when(u == 4)(lambda: wait(11, wg_v.at[pl.ds(BA, BA)], wu_v.at[pl.ds(BA, BA)],
                                     wda_rows(BA, NFA), *w_dst(3 * CPU, NCH)))
        c = jax.lax.shift_right_logical(u, 2)
        a = pl.multiple_of((u & 3) * TA, TA)
        x = x_v[pl.ds(a, TA), :]
        h = _reglu(_dot(x, _cat([wg_u[c * BA + k] for k in range(BA)])),
                   _dot(x, _cat([wu_u[c * BA + k] for k in range(BA)])))
        for k in range(CPU):
            repack(jnp.minimum(CPU * (u - 1) + k, NCH - 1))
        r = pl.multiple_of(c * (128 * BA), 128)
        bacc[c, pl.ds(a, TA), :] = _dot(_cat([h]), wda_v[pl.ds(r, 128 * BA), :])
        return carry

    jax.lax.fori_loop(1, NA, phase_a, 0)
    wait(12, gw_v, wg_v.at[pl.ds(NFA, NF - NFA)], wu_v.at[pl.ds(NFA, NF - NFA)], wd_v)

    m16 = (_lane((RG, 128)) & 16) == 0
    m1 = (_lane((RG, 128)) & 1) == 0

    def attend(r0, base, scale, zvec):
        logits = []
        for w in range(WIN):
            if w % LGS == 0:
                if w:
                    scale = pltpu.bitcast(
                        pltpu.bitcast(scale, i32) | (pltpu.bitcast(raw, i32) & zvec), f32)
                q = [qkv_s[j, pl.ds(HALO + r0, RG), :] * scale for j in range(NB)]
            off = HALO + r0 - DIL * w
            acc = q[0] * qkv_s[NB, pl.ds(off, RG), :]
            for j in range(1, NB):
                acc = acc + q[j] * qkv_s[NB + j, pl.ds(off, RG), :]
            raw = acc
            acc = acc + jnp.where(m16, pltpu.roll(acc, 128 - 16, 1), pltpu.roll(acc, 16, 1))
            acc = acc + jnp.where(m1, pltpu.roll(acc, 128 - 1, 1), pltpu.roll(acc, 1, 1))
            if r0 < DIL * w:
                pos = base + r0 + jax.lax.broadcasted_iota(i32, (RG, 128), 0)
                acc = jnp.where(pos >= DIL * w, acc, NEG)
            logits.append(acc)
        m = logits[0]
        for w in range(1, WIN):
            m = jnp.maximum(m, logits[w])
        e = [jnp.exp2(l - m) for l in logits]
        s = e[0]
        for w in range(1, WIN):
            s = s + e[w]
        inv = pl.reciprocal(s, approx=True)
        inv = inv * (2.0 - s * inv)
        for j in range(NB):
            if j % PVS == 0:
                if j:
                    inv = pltpu.bitcast(pltpu.bitcast(inv, i32) | (pltpu.bitcast(o, i32) & zvec), f32)
                p = [x * inv for x in e]
            o = p[0] * qkv_s[2 * NB + j, pl.ds(HALO + r0, RG), :]
            for w in range(1, WIN):
                o = o + p[w] * qkv_s[2 * NB + j, pl.ds(HALO + r0 - DIL * w, RG), :]
            o_s[j, pl.ds(r0, RG), :] = o

    def phase_b(t, carry):
        base = pl.multiple_of(t * TB, TB)
        zero = zero_s[0]
        zvec = jnp.full((RG, 128), zero, i32)
        sbits = pltpu.bitcast(jnp.full((RG, 128), SCALE, f32), i32)
        x = x_v[pl.ds(base, TB), :]
        gw = pltpu.bitcast(jnp.broadcast_to(gw_v[...].astype(f32).reshape(1, D), (8, D)), i32)

        gates = []

        def gate_rows(r0, anchor):
            dep = pltpu.bitcast(anchor, i32) & zvec
            xr = x[r0:r0 + 16, :].astype(f32)
            acc = None
            for j in range(NB):
                w = pltpu.bitcast(gw[:, 128 * j:128 * (j + 1)] | dep, f32)
                term = xr[:, 128 * j:128 * (j + 1)] * jnp.concatenate([w, w], axis=0)
                acc = term if acc is None else acc + term
            z = jnp.sum(acc, axis=-1, keepdims=True)
            gates.append(jnp.broadcast_to(jax.nn.sigmoid(z), (16, 128)))

        for i in range(3):
            r = _dot(x, _cat([jnp.concatenate([w_p[i, j, pl.ds(PITCH * c, 64), :] for c in range(8)],
                                              axis=0) for j in range(NB)]))
            for j in range(NB):
                qkv_s[i * NB + j, pl.ds(HALO, TB), :] = r[:, 128 * j:128 * (j + 1)]
                if i * NB + j < TB // 16:
                    gate_rows(16 * (i * NB + j), r[ANCH:ANCH + 8, 128 * j:128 * (j + 1)])
        groups = list(range(0, TB, RG))
        nslots = 2 * (NF - NFA) - NSK
        hs = []
        slot = 0
        done = 0

        def release(anchor):
            nonlocal slot, done
            slot += 1
            want = min(len(groups), -(-slot * len(groups) // nslots))
            if want > done:
                for r0 in groups[done:want]:
                    dep = pltpu.bitcast(anchor, i32)
                    if GDEP:
                        dep = dep | pltpu.bitcast(gates[r0 // 16][r0 % 16:r0 % 16 + 8], i32)
                    attend(r0, base, pltpu.bitcast(sbits | (dep & zvec), f32), zvec)
                done = want

        for c in range(NFA, NF, 2):
            g = _dot(x, _cat([wg_u[c], wg_u[c + 1]]))
            for n in range(2):
                release(g[ANCH:ANCH + 8, 128 * n:128 * (n + 1)])
            u = _dot(x, _cat([wu_u[c], wu_u[c + 1]]))
            for n in range(2):
                release(u[ANCH:ANCH + 8, 128 * n:128 * (n + 1)])
            hs.append(_reglu(g, u))
        assert done == len(groups)
        qkv_s[pl.ds(NB, 2 * NB), pl.ds(0, HALO), :] = qkv_s[pl.ds(NB, 2 * NB), pl.ds(TB, HALO), :]
        g = jnp.concatenate(gates, axis=0)
        g1 = 1.0 - g

        def down():
            wd = _cat([wd_u[j] for j in range(NB)])
            return (bacc[0, pl.ds(base, TB), :] + bacc[1, pl.ds(base, TB), :]
                    + _dot(_cat(hs), wd))

        if ORDER == 1:
            b = down()
        wo = _cat([jnp.concatenate([w_p[3, j, pl.ds(8 * m + c, 8, stride=PITCH), :]
                                    for c in range(8) for m in range(8)], axis=0)
                   for j in range(NB)])
        o_s[0, pl.ds(TB + zero, 8), :] = jnp.zeros((8, 128), f32)
        o = jnp.concatenate([o_s[j, pl.ds(0, TB), :] for j in range(NB)], axis=1)
        a = _dot(o.astype(bf16), wo)
        if ORDER == 0:
            b = down()
        for r0, r1, c0, c1 in OUTP:
            n = c1 - c0
            res = (jnp.concatenate([g[r0:r1]] * (n // 128), axis=1) * a[r0:r1, c0:c1]
                   + jnp.concatenate([g1[r0:r1]] * (n // 128), axis=1) * b[r0:r1, c0:c1])
            rs = pl.ds(pl.multiple_of(base + r0, 16), r1 - r0)
            out_v[rs, pl.ds(c0, n)] = res.astype(bf16)
            start(out_v.at[rs, pl.ds(c0, n)], out_hbm.at[rs, pl.ds(c0, n)], 13)
        return carry

    with _scope("B"):
        jax.lax.fori_loop(0, S // TB, phase_b, 0)
    wait(13, out_v)


@jax.jit
def pallas_gated_mix__sliding_local_dilated__glu_gated_reglu__prompt_kernel(
    A_x: jax.Array,
    A_wqkv: jax.Array,
    A_wo: jax.Array,
    B_x: jax.Array,
    B_W_gate: jax.Array,
    B_W_up: jax.Array,
    B_W_down: jax.Array,
    gate_w: jax.Array,
):
    del B_x
    x = A_x.reshape(S, D)
    hbm = pl.BlockSpec(memory_space=pl.ANY)
    out = pl.pallas_call(
        _kernel,
        out_shape=jax.ShapeDtypeStruct((S, D), bf16),
        in_specs=[hbm] * 7,
        out_specs=hbm,
        scratch_shapes=[
            pltpu.VMEM((S, D), bf16),
            pltpu.VMEM((4, D, D), bf16),
            pltpu.VMEM((NF, D, 128), bf16),
            pltpu.VMEM((NF, D, 128), bf16),
            pltpu.VMEM((128 * NFA, D), bf16),
            pltpu.VMEM((NB, F - 128 * NFA, 128), bf16),
            pltpu.VMEM((D,), bf16),
            pltpu.VMEM((4, NB, 8 * PITCH, 128), u32),
            pltpu.VMEM((2, S, D), f32),
            pltpu.VMEM((3 * NB, HALO + TB + 8, 128), f32),
            pltpu.VMEM((NB, TB + 8, 128), f32),
            pltpu.VMEM((S, D), bf16),
            pltpu.SMEM((1,), i32),
            pltpu.SemaphoreType.DMA((14,)),
        ],
        compiler_params=pltpu.CompilerParams(
            vmem_limit_bytes=110 * 1024 * 1024,
            disable_bounds_checks=not CHECKS,
            disable_semaphore_checks=not CHECKS,
        ),
    )(x, A_wqkv, A_wo, B_W_gate, B_W_up, B_W_down, gate_w)
    return out.reshape(1, S, D)
```

```python
import os
import jax
import jax.numpy as jnp
import jax.experimental.pallas as pl
import jax.experimental.pallas.tpu as pltpu

S, D, F = 2048, 1024, 3584
H, DH, WIN, DIL = 32, 32, 8, 2
NB = D // 128
NF = F // 128
HALO = 16
BA = 3
NFA = 2 * BA
R0 = 496
NA = 5
UR = (2 * S - R0) // NA
SUB = (0, (S - R0) % UR, UR)
TB = 256
RG = 8
ANCH = int(os.environ.get('ANCH', 248))
NSK = int(os.environ.get('NSK', 2))
ORDER = int(os.environ.get('ORDER', 0))
OUTP = {0: ((0, 256, 0, 512), (0, 256, 512, 768), (0, 256, 768, 1024)),
        1: ((0, 256, 0, 512), (0, 256, 512, 768), (0, 192, 768, 1024), (192, 256, 768, 1024)),
        2: ((0, 256, 0, 512), (0, 256, 512, 896), (0, 192, 896, 1024), (192, 256, 896, 1024)),
        3: ((0, 256, 0, 768), (0, 128, 768, 1024), (128, 224, 768, 1024), (224, 256, 768, 1024)),
        }[int(os.environ.get('OUTP', 2))]
GDEP = int(os.environ.get('GDEP', 1))
PVS = int(os.environ.get('PVS', 2))
LGS = int(os.environ.get('LGS', 4))
P0M = int(os.environ.get('P0M', 0))
SCOPES = int(os.environ.get("SCOPES", 0))
CHECKS = int(os.environ.get("CHECKS", 0))
PITCH = 65
CPU = int(os.environ.get('CPU', 8))
COFF = NA * CPU - 32
CH1 = max(CPU - COFF, 1)
NCH = 4 * 8
LOG2E = 1.4426950408889634
SCALE = DH ** -0.5 * LOG2E
NEG = -1e9 * LOG2E

f32 = jnp.float32
bf16 = jnp.bfloat16
u32 = jnp.uint32
i32 = jnp.int32


def _dot(a, b):
    return jnp.dot(a, b, preferred_element_type=f32)


def _lane(shape):
    return jax.lax.broadcasted_iota(i32, shape, 1)


def _cat(blocks):
    return jnp.concatenate([pltpu.bitcast(b, bf16) for b in blocks], axis=1)


def _reglu(g, u):
    return pltpu.bitcast((jnp.maximum(g, 0.0) * u).astype(bf16), u32)


class _NoScope:
    def __enter__(self):
        return self

    def __exit__(self, *a):
        return False


def _scope(name):
    return jax.named_scope(name) if SCOPES else _NoScope()


def _kernel(x_hbm, wqkv_hbm, wo_hbm, wg_hbm, wu_hbm, wd_hbm, gw_hbm, out_hbm,
            x_v, w_v, wg_v, wu_v, wda_v, wd_v, gw_v, w_p, bacc,
            qkv_s, o_s, out_v, zero_s, sems):
    def start(src, dst, grp):
        pltpu.make_async_copy(src, dst, sems.at[grp]).start()

    def wait(grp, *dsts):
        with _scope("w%d" % grp):
            for d in dsts:
                pltpu.make_async_copy(d, d, sems.at[grp]).wait()

    def xrows(a, n):
        return x_v.at[pl.ds(a, n), :]

    def get_x(a, n, grp):
        start(x_hbm.at[pl.ds(a, n), :], xrows(a, n), grp)

    def get_cols(hbm, dst, b0, b1, grp):
        for b in range(b0, b1):
            start(hbm.at[:, pl.ds(128 * b, 128)], dst.at[b], grp)

    def wda_rows(b0, b1):
        return wda_v.at[pl.ds(128 * b0, 128 * (b1 - b0)), :]

    def get_wda(b0, b1, grp):
        start(wd_hbm.at[pl.ds(128 * b0, 128 * (b1 - b0)), :], wda_rows(b0, b1), grp)

    def w_rows(c0, c1):
        out = []
        for p in range(4):
            a, b = max(c0, 8 * p), min(c1, 8 * p + 8)
            if a < b:
                out.append((p, 128 * (a - 8 * p), 128 * (b - a)))
        return out

    def w_dst(c0, c1):
        return [w_v.at[p, pl.ds(r, n), :] for p, r, n in w_rows(c0, c1)]

    def get_w(c0, c1, grp):
        for p, r, n in w_rows(c0, c1):
            src = (wqkv_hbm.at[pl.ds(r, n), pl.ds(p * D, D)] if p < 3
                   else wo_hbm.at[pl.ds(r, n), :])
            start(src, w_v.at[p, pl.ds(r, n), :], grp)

    get_x(0, 128, 0)
    get_cols(wg_hbm, wg_v, 0, 1, 0)
    get_x(128, 128, 1)
    get_cols(wu_hbm, wu_v, 0, 1, 2)
    get_x(256, 128, 3)
    get_cols(wg_hbm, wg_v, 1, 2, 4)
    get_x(384, R0 - 384, 5)
    get_cols(wu_hbm, wu_v, 1, 2, 5)
    get_cols(wg_hbm, wg_v, 2, 3, 6)
    get_cols(wu_hbm, wu_v, 2, 3, 6)
    get_wda(0, 2, 6)
    get_wda(2, 3, 7)
    get_x(R0, UR, 8)
    get_w(0, CH1, 8)
    get_x(R0 + UR, UR, 9)
    get_w(CH1, 2 * CPU - COFF, 9)
    get_x(R0 + 2 * UR, S - R0 - 2 * UR, 10)
    get_cols(wg_hbm, wg_v, BA, NFA, 10)
    get_cols(wu_hbm, wu_v, BA, NFA, 10)
    get_wda(BA, NFA, 10)
    get_w(2 * CPU - COFF, NCH, 10)
    start(gw_hbm, gw_v, 12)
    for j in range(NB):
        start(wd_hbm.at[pl.ds(128 * NFA, F - 128 * NFA), pl.ds(128 * j, 128)], wd_v.at[j], 12)
    get_cols(wg_hbm, wg_v, NFA, NF, 12)

    wg_u, wu_u, wd_u = (r.bitcast(u32) for r in (wg_v, wu_v, wd_v))

    zero_s[0] = 0
    qkv_s[pl.ds(NB, 2 * NB), pl.ds(0, HALO), :] = jnp.zeros((2 * NB, HALO, 128), f32)

    def repack(ch):
        p = jax.lax.shift_right_logical(ch, 3)
        rc = ch & 7
        on = jnp.where(ch < 24, -1, 0).astype(i32)
        r0 = pl.multiple_of(rc * 128, 128)
        blk = [pltpu.bitcast(w_v[p, pl.ds(r0, 128), pl.ds(128 * j, 128)], u32) for j in range(NB)]
        lane = _lane((64, 128))
        for bb, lb in ((2, 3), (1, 2), (0, 1)):
            sh = 1 << lb
            keep_a = (lane & (on & sh)) == 0
            take_a = ((lane & sh) | (~on & 1)) == 0
            for j in range(NB):
                if j & (1 << bb):
                    continue
                a, b = blk[j], blk[j | (1 << bb)]
                blk[j] = jnp.where(keep_a, a, pltpu.roll(b, sh, 1))
                blk[j | (1 << bb)] = jnp.where(take_a, pltpu.roll(a, 128 - sh, 1), b)
        for j in range(NB):
            w_p[p, j, pl.ds(rc * PITCH, 64), :] = blk[j]

    def xr(a, b):
        return x_v[pl.ds(a, b - a), :]

    def rcat(*parts):
        return jnp.concatenate(parts, axis=0)

    wait(0, xrows(0, 128), wg_v.at[0])
    g0a = _dot(xr(0, 128), _cat([wg_u[0]]))
    wait(1, xrows(128, 128))
    g0b = _dot(xr(128, 256), _cat([wg_u[0]]))
    wait(2, wu_v.at[0])
    h0a = _reglu(rcat(g0a, g0b), _dot(xr(0, 256), _cat([wu_u[0]])))
    wait(3, xrows(256, 128))
    gu = _dot(xr(256, 384), _cat([wg_u[0], wu_u[0]]))
    h0b = _reglu(gu[:, :128], gu[:, 128:])
    wait(4, wg_v.at[1])
    g1a = _dot(xr(0, 384), _cat([wg_u[1]]))
    wait(5, xrows(384, R0 - 384), wu_v.at[1])
    gu = _dot(xr(384, R0), _cat([wg_u[0], wu_u[0], wg_u[1]]))
    h0c = _reglu(gu[:, :128], gu[:, 128:256])
    h1 = _reglu(rcat(g1a, gu[:, 256:]), _dot(xr(0, R0), _cat([wu_u[1]])))
    if P0M:
        wait(6, wg_v.at[2], wu_v.at[2], wda_rows(0, 2))
        wait(7, wda_rows(2, 3))
    else:
        wait(6, wg_v.at[2], wu_v.at[2], wda_rows(0, 2))
    gu = _dot(xr(0, R0), _cat([wg_u[2], wu_u[2]]))
    h2 = _reglu(gu[:, :128], gu[:, 128:])
    get_cols(wu_hbm, wu_v, NFA, NF, 12)
    if not P0M:
        wait(7, wda_rows(2, 3))
    bacc[0, pl.ds(0, R0), :] = _dot(_cat([rcat(h0a, h0b, h0c), h1, h2]), wda_v[pl.ds(0, 128 * BA), :])

    def phase_a(u, carry):
        pl.when(u == 0)(lambda: wait(8, xrows(R0, UR), *w_dst(0, CH1)))
        pl.when(u == 1)(lambda: wait(9, xrows(R0 + UR, UR), *w_dst(CH1, 2 * CPU - COFF)))
        pl.when(u == 2)(lambda: wait(10, xrows(R0 + 2 * UR, S - R0 - 2 * UR), wg_v.at[pl.ds(BA, BA)],
                                     wu_v.at[pl.ds(BA, BA)], wda_rows(BA, NFA),
                                     *w_dst(2 * CPU - COFF, NCH)))
        parts = []
        for v0, v1 in zip(SUB[:-1], SUB[1:]):
            v = u * UR + v0
            c = (v >= S - R0).astype(i32)
            a = pl.multiple_of(v + R0 - c * S, 16)
            x = x_v[pl.ds(a, v1 - v0), :]
            h = _reglu(_dot(x, _cat([wg_u[c * BA + k] for k in range(BA)])),
                       _dot(x, _cat([wu_u[c * BA + k] for k in range(BA)])))
            parts.append((c, a, v1 - v0, h))
        for k in range(CPU):
            repack(jnp.maximum(CPU * u + k - COFF, 0))
        for c, a, n, h in parts:
            r = pl.multiple_of(c * (128 * BA), 128)
            bacc[c, pl.ds(a, n), :] = _dot(_cat([h]), wda_v[pl.ds(r, 128 * BA), :])
        return carry

    jax.lax.fori_loop(0, NA, phase_a, 0)
    wait(12, gw_v, wg_v.at[pl.ds(NFA, NF - NFA)], wu_v.at[pl.ds(NFA, NF - NFA)], wd_v)

    m16 = (_lane((RG, 128)) & 16) == 0
    m1 = (_lane((RG, 128)) & 1) == 0

    def attend(r0, base, scale, zvec):
        logits = []
        for w in range(WIN):
            if w % LGS == 0:
                if w:
                    scale = pltpu.bitcast(
                        pltpu.bitcast(scale, i32) | (pltpu.bitcast(raw, i32) & zvec), f32)
                q = [qkv_s[j, pl.ds(HALO + r0, RG), :] * scale for j in range(NB)]
            off = HALO + r0 - DIL * w
            acc = q[0] * qkv_s[NB, pl.ds(off, RG), :]
            for j in range(1, NB):
                acc = acc + q[j] * qkv_s[NB + j, pl.ds(off, RG), :]
            raw = acc
            acc = acc + jnp.where(m16, pltpu.roll(acc, 128 - 16, 1), pltpu.roll(acc, 16, 1))
            acc = acc + jnp.where(m1, pltpu.roll(acc, 128 - 1, 1), pltpu.roll(acc, 1, 1))
            if r0 < DIL * w:
                pos = base + r0 + jax.lax.broadcasted_iota(i32, (RG, 128), 0)
                acc = jnp.where(pos >= DIL * w, acc, NEG)
            logits.append(acc)
        m = logits[0]
        for w in range(1, WIN):
            m = jnp.maximum(m, logits[w])
        e = [jnp.exp2(l - m) for l in logits]
        s = e[0]
        for w in range(1, WIN):
            s = s + e[w]
        inv = pl.reciprocal(s, approx=True)
        inv = inv * (2.0 - s * inv)
        for j in range(NB):
            if j % PVS == 0:
                if j:
                    inv = pltpu.bitcast(pltpu.bitcast(inv, i32) | (pltpu.bitcast(o, i32) & zvec), f32)
                p = [x * inv for x in e]
            o = p[0] * qkv_s[2 * NB + j, pl.ds(HALO + r0, RG), :]
            for w in range(1, WIN):
                o = o + p[w] * qkv_s[2 * NB + j, pl.ds(HALO + r0 - DIL * w, RG), :]
            o_s[j, pl.ds(r0, RG), :] = o

    def phase_b(t, carry):
        base = pl.multiple_of(t * TB, TB)
        zero = zero_s[0]
        zvec = jnp.full((RG, 128), zero, i32)
        sbits = pltpu.bitcast(jnp.full((RG, 128), SCALE, f32), i32)
        x = x_v[pl.ds(base, TB), :]
        gw = pltpu.bitcast(jnp.broadcast_to(gw_v[...].astype(f32).reshape(1, D), (8, D)), i32)

        gates = []

        def gate_rows(r0, anchor):
            dep = pltpu.bitcast(anchor, i32) & zvec
            xr = x[r0:r0 + 16, :].astype(f32)
            acc = None
            for j in range(NB):
                w = pltpu.bitcast(gw[:, 128 * j:128 * (j + 1)] | dep, f32)
                term = xr[:, 128 * j:128 * (j + 1)] * jnp.concatenate([w, w], axis=0)
                acc = term if acc is None else acc + term
            z = jnp.sum(acc, axis=-1, keepdims=True)
            gates.append(jnp.broadcast_to(jax.nn.sigmoid(z), (16, 128)))

        for i in range(3):
            r = _dot(x, _cat([jnp.concatenate([w_p[i, j, pl.ds(PITCH * c, 64), :] for c in range(8)],
                                              axis=0) for j in range(NB)]))
            for j in range(NB):
                qkv_s[i * NB + j, pl.ds(HALO, TB), :] = r[:, 128 * j:128 * (j + 1)]
                if i * NB + j < TB // 16:
                    gate_rows(16 * (i * NB + j), r[ANCH:ANCH + 8, 128 * j:128 * (j + 1)])
        groups = list(range(0, TB, RG))
        nslots = 2 * (NF - NFA) - NSK
        hs = []
        slot = 0
        done = 0

        def release(anchor):
            nonlocal slot, done
            slot += 1
            want = min(len(groups), -(-slot * len(groups) // nslots))
            if want > done:
                for r0 in groups[done:want]:
                    dep = pltpu.bitcast(anchor, i32)
                    if GDEP:
                        dep = dep | pltpu.bitcast(gates[r0 // 16][r0 % 16:r0 % 16 + 8], i32)
                    attend(r0, base, pltpu.bitcast(sbits | (dep & zvec), f32), zvec)
                done = want

        for c in range(NFA, NF, 2):
            g = _dot(x, _cat([wg_u[c], wg_u[c + 1]]))
            for n in range(2):
                release(g[ANCH:ANCH + 8, 128 * n:128 * (n + 1)])
            u = _dot(x, _cat([wu_u[c], wu_u[c + 1]]))
            for n in range(2):
                release(u[ANCH:ANCH + 8, 128 * n:128 * (n + 1)])
            hs.append(_reglu(g, u))
        assert done == len(groups)
        qkv_s[pl.ds(NB, 2 * NB), pl.ds(0, HALO), :] = qkv_s[pl.ds(NB, 2 * NB), pl.ds(TB, HALO), :]
        g = jnp.concatenate(gates, axis=0)
        g1 = 1.0 - g

        def down():
            wd = _cat([wd_u[j] for j in range(NB)])
            return (bacc[0, pl.ds(base, TB), :] + bacc[1, pl.ds(base, TB), :]
                    + _dot(_cat(hs), wd))

        if ORDER == 1:
            b = down()
        wo = _cat([jnp.concatenate([w_p[3, j, pl.ds(8 * m + c, 8, stride=PITCH), :]
                                    for c in range(8) for m in range(8)], axis=0)
                   for j in range(NB)])
        o_s[0, pl.ds(TB + zero, 8), :] = jnp.zeros((8, 128), f32)
        o = jnp.concatenate([o_s[j, pl.ds(0, TB), :] for j in range(NB)], axis=1)
        a = _dot(o.astype(bf16), wo)
        if ORDER == 0:
            b = down()
        for r0, r1, c0, c1 in OUTP:
            n = c1 - c0
            res = (jnp.concatenate([g[r0:r1]] * (n // 128), axis=1) * a[r0:r1, c0:c1]
                   + jnp.concatenate([g1[r0:r1]] * (n // 128), axis=1) * b[r0:r1, c0:c1])
            rs = pl.ds(pl.multiple_of(base + r0, 16), r1 - r0)
            out_v[rs, pl.ds(c0, n)] = res.astype(bf16)
            start(out_v.at[rs, pl.ds(c0, n)], out_hbm.at[rs, pl.ds(c0, n)], 13)
        return carry

    with _scope("B"):
        jax.lax.fori_loop(0, S // TB, phase_b, 0)
    wait(13, out_v)


@jax.jit
def pallas_gated_mix__sliding_local_dilated__glu_gated_reglu__prompt_kernel(
    A_x: jax.Array,
    A_wqkv: jax.Array,
    A_wo: jax.Array,
    B_x: jax.Array,
    B_W_gate: jax.Array,
    B_W_up: jax.Array,
    B_W_down: jax.Array,
    gate_w: jax.Array,
):
    del B_x
    x = A_x.reshape(S, D)
    hbm = pl.BlockSpec(memory_space=pl.ANY)
    out = pl.pallas_call(
        _kernel,
        out_shape=jax.ShapeDtypeStruct((S, D), bf16),
        in_specs=[hbm] * 7,
        out_specs=hbm,
        scratch_shapes=[
            pltpu.VMEM((S, D), bf16),
            pltpu.VMEM((4, D, D), bf16),
            pltpu.VMEM((NF, D, 128), bf16),
            pltpu.VMEM((NF, D, 128), bf16),
            pltpu.VMEM((128 * NFA, D), bf16),
            pltpu.VMEM((NB, F - 128 * NFA, 128), bf16),
            pltpu.VMEM((D,), bf16),
            pltpu.VMEM((4, NB, 8 * PITCH, 128), u32),
            pltpu.VMEM((2, S, D), f32),
            pltpu.VMEM((3 * NB, HALO + TB + 8, 128), f32),
            pltpu.VMEM((NB, TB + 8, 128), f32),
            pltpu.VMEM((S, D), bf16),
            pltpu.SMEM((1,), i32),
            pltpu.SemaphoreType.DMA((14,)),
        ],
        compiler_params=pltpu.CompilerParams(
            vmem_limit_bytes=110 * 1024 * 1024,
            disable_bounds_checks=not CHECKS,
            disable_semaphore_checks=not CHECKS,
        ),
    )(x, A_wqkv, A_wo, B_W_gate, B_W_up, B_W_down, gate_w)
    return out.reshape(1, S, D)
```

```python
import os
import jax
import jax.numpy as jnp
import jax.experimental.pallas as pl
import jax.experimental.pallas.tpu as pltpu

S, D, F = 2048, 1024, 3584
H, DH, WIN, DIL = 32, 32, 8, 2
NB = D // 128
NF = F // 128
HALO = 16
BA = 3
NFA = 2 * BA
R0 = 496
NA = 5
UR = (2 * S - R0) // NA
SUB = (0, (S - R0) % UR, UR)
TB = 256
RG = 8
ANCH = int(os.environ.get('ANCH', 248))
NSK = int(os.environ.get('NSK', 4))
ORDER = int(os.environ.get('ORDER', 0))
OUTP = {0: ((0, 256, 0, 512), (0, 256, 512, 768), (0, 256, 768, 1024)),
        1: ((0, 256, 0, 512), (0, 256, 512, 768), (0, 192, 768, 1024), (192, 256, 768, 1024)),
        2: ((0, 256, 0, 512), (0, 256, 512, 896), (0, 192, 896, 1024), (192, 256, 896, 1024)),
        3: ((0, 256, 0, 768), (0, 128, 768, 1024), (128, 224, 768, 1024), (224, 256, 768, 1024)),
        }[int(os.environ.get('OUTP', 2))]
GDEP = int(os.environ.get('GDEP', 1))
PVS = int(os.environ.get('PVS', 2))
LGS = int(os.environ.get('LGS', 4))
P0M = int(os.environ.get('P0M', 0))
CHAIN = int(os.environ.get('CHAIN', 1))
SCOPES = int(os.environ.get("SCOPES", 0))
CHECKS = int(os.environ.get("CHECKS", 0))
PITCH = 65
CPU = int(os.environ.get('CPU', 8))
COFF = NA * CPU - 32
CH1 = max(CPU - COFF, 1)
NCH = 4 * 8
LOG2E = 1.4426950408889634
SCALE = DH ** -0.5 * LOG2E
NEG = -1e9 * LOG2E

f32 = jnp.float32
bf16 = jnp.bfloat16
u32 = jnp.uint32
i32 = jnp.int32


def _dot(a, b):
    return jnp.dot(a, b, preferred_element_type=f32)


def _lane(shape):
    return jax.lax.broadcasted_iota(i32, shape, 1)


def _cat(blocks):
    return jnp.concatenate([pltpu.bitcast(b, bf16) for b in blocks], axis=1)


def _reglu(g, u):
    return pltpu.bitcast((jnp.maximum(g, 0.0) * u).astype(bf16), u32)


class _NoScope:
    def __enter__(self):
        return self

    def __exit__(self, *a):
        return False


def _scope(name):
    return jax.named_scope(name) if SCOPES else _NoScope()


def _kernel(x_hbm, wqkv_hbm, wo_hbm, wg_hbm, wu_hbm, wd_hbm, gw_hbm, out_hbm,
            x_v, w_v, wg_v, wu_v, wda_v, wd_v, gw_v, w_p, bacc,
            qkv_s, o_s, out_v, zero_s, sems):
    def start(src, dst, grp):
        pltpu.make_async_copy(src, dst, sems.at[grp]).start()

    def wait(grp, *dsts):
        with _scope("w%d" % grp):
            for d in dsts:
                pltpu.make_async_copy(d, d, sems.at[grp]).wait()

    def xrows(a, n):
        return x_v.at[pl.ds(a, n), :]

    def get_x(a, n, grp):
        start(x_hbm.at[pl.ds(a, n), :], xrows(a, n), grp)

    def get_cols(hbm, dst, b0, b1, grp):
        for b in range(b0, b1):
            start(hbm.at[:, pl.ds(128 * b, 128)], dst.at[b], grp)

    def wda_rows(b0, b1):
        return wda_v.at[pl.ds(128 * b0, 128 * (b1 - b0)), :]

    def get_wda(b0, b1, grp):
        start(wd_hbm.at[pl.ds(128 * b0, 128 * (b1 - b0)), :], wda_rows(b0, b1), grp)

    def w_rows(c0, c1):
        out = []
        for p in range(4):
            a, b = max(c0, 8 * p), min(c1, 8 * p + 8)
            if a < b:
                out.append((p, 128 * (a - 8 * p), 128 * (b - a)))
        return out

    def w_dst(c0, c1):
        return [w_v.at[p, pl.ds(r, n), :] for p, r, n in w_rows(c0, c1)]

    def get_w(c0, c1, grp):
        for p, r, n in w_rows(c0, c1):
            src = (wqkv_hbm.at[pl.ds(r, n), pl.ds(p * D, D)] if p < 3
                   else wo_hbm.at[pl.ds(r, n), :])
            start(src, w_v.at[p, pl.ds(r, n), :], grp)

    get_x(0, 128, 0)
    get_cols(wg_hbm, wg_v, 0, 1, 0)
    get_x(128, 128, 1)
    get_cols(wu_hbm, wu_v, 0, 1, 2)
    get_x(256, 128, 3)
    get_cols(wg_hbm, wg_v, 1, 2, 4)
    get_x(384, R0 - 384, 5)
    get_cols(wu_hbm, wu_v, 1, 2, 5)
    get_cols(wg_hbm, wg_v, 2, 3, 6)
    get_cols(wu_hbm, wu_v, 2, 3, 6)
    get_wda(0, 2, 6)
    get_wda(2, 3, 7)
    get_x(R0, UR, 8)
    get_w(0, CH1, 8)
    get_x(R0 + UR, UR, 9)
    get_w(CH1, 2 * CPU - COFF, 9)
    get_x(R0 + 2 * UR, S - R0 - 2 * UR, 10)
    get_cols(wg_hbm, wg_v, BA, NFA, 10)
    get_cols(wu_hbm, wu_v, BA, NFA, 10)
    get_wda(BA, NFA, 10)
    get_w(2 * CPU - COFF, NCH, 10)
    start(gw_hbm, gw_v, 12)
    for j in range(NB):
        start(wd_hbm.at[pl.ds(128 * NFA, F - 128 * NFA), pl.ds(128 * j, 128)], wd_v.at[j], 12)
    get_cols(wg_hbm, wg_v, NFA, NF, 12)

    wg_u, wu_u, wd_u = (r.bitcast(u32) for r in (wg_v, wu_v, wd_v))

    zero_s[0] = 0
    qkv_s[pl.ds(NB, 2 * NB), pl.ds(0, HALO), :] = jnp.zeros((2 * NB, HALO, 128), f32)

    def repack(ch):
        p = jax.lax.shift_right_logical(ch, 3)
        rc = ch & 7
        on = jnp.where(ch < 24, -1, 0).astype(i32)
        r0 = pl.multiple_of(rc * 128, 128)
        blk = [pltpu.bitcast(w_v[p, pl.ds(r0, 128), pl.ds(128 * j, 128)], u32) for j in range(NB)]
        lane = _lane((64, 128))
        for bb, lb in ((2, 3), (1, 2), (0, 1)):
            sh = 1 << lb
            keep_a = (lane & (on & sh)) == 0
            take_a = ((lane & sh) | (~on & 1)) == 0
            for j in range(NB):
                if j & (1 << bb):
                    continue
                a, b = blk[j], blk[j | (1 << bb)]
                blk[j] = jnp.where(keep_a, a, pltpu.roll(b, sh, 1))
                blk[j | (1 << bb)] = jnp.where(take_a, pltpu.roll(a, 128 - sh, 1), b)
        for j in range(NB):
            w_p[p, j, pl.ds(rc * PITCH, 64), :] = blk[j]

    def xr(a, b):
        return x_v[pl.ds(a, b - a), :]

    def rcat(*parts):
        return jnp.concatenate(parts, axis=0)

    wait(0, xrows(0, 128), wg_v.at[0])
    g0a = _dot(xr(0, 128), _cat([wg_u[0]]))
    wait(1, xrows(128, 128))
    g0b = _dot(xr(128, 256), _cat([wg_u[0]]))
    wait(2, wu_v.at[0])
    h0a = _reglu(rcat(g0a, g0b), _dot(xr(0, 256), _cat([wu_u[0]])))
    wait(3, xrows(256, 128))
    gu = _dot(xr(256, 384), _cat([wg_u[0], wu_u[0]]))
    h0b = _reglu(gu[:, :128], gu[:, 128:])
    wait(4, wg_v.at[1])
    g1a = _dot(xr(0, 384), _cat([wg_u[1]]))
    wait(5, xrows(384, R0 - 384), wu_v.at[1])
    gu = _dot(xr(384, R0), _cat([wg_u[0], wu_u[0], wg_u[1]]))
    h0c = _reglu(gu[:, :128], gu[:, 128:256])
    h1 = _reglu(rcat(g1a, gu[:, 256:]), _dot(xr(0, R0), _cat([wu_u[1]])))
    if P0M:
        wait(6, wg_v.at[2], wu_v.at[2], wda_rows(0, 2))
        wait(7, wda_rows(2, 3))
    else:
        wait(6, wg_v.at[2], wu_v.at[2], wda_rows(0, 2))
    gu = _dot(xr(0, R0), _cat([wg_u[2], wu_u[2]]))
    h2 = _reglu(gu[:, :128], gu[:, 128:])
    get_cols(wu_hbm, wu_v, NFA, NF, 12)
    if not P0M:
        wait(7, wda_rows(2, 3))
    bacc[0, pl.ds(0, R0), :] = _dot(_cat([rcat(h0a, h0b, h0c), h1, h2]), wda_v[pl.ds(0, 128 * BA), :])

    def phase_a(u, carry):
        pl.when(u == 0)(lambda: wait(8, xrows(R0, UR), *w_dst(0, CH1)))
        pl.when(u == 1)(lambda: wait(9, xrows(R0 + UR, UR), *w_dst(CH1, 2 * CPU - COFF)))
        pl.when(u == 2)(lambda: wait(10, xrows(R0 + 2 * UR, S - R0 - 2 * UR), wg_v.at[pl.ds(BA, BA)],
                                     wu_v.at[pl.ds(BA, BA)], wda_rows(BA, NFA),
                                     *w_dst(2 * CPU - COFF, NCH)))
        parts = []
        for v0, v1 in zip(SUB[:-1], SUB[1:]):
            v = u * UR + v0
            c = (v >= S - R0).astype(i32)
            a = pl.multiple_of(v + R0 - c * S, 16)
            x = x_v[pl.ds(a, v1 - v0), :]
            h = _reglu(_dot(x, _cat([wg_u[c * BA + k] for k in range(BA)])),
                       _dot(x, _cat([wu_u[c * BA + k] for k in range(BA)])))
            parts.append((c, a, v1 - v0, h))
        for k in range(CPU):
            repack(jnp.maximum(CPU * u + k - COFF, 0))
        for c, a, n, h in parts:
            r = pl.multiple_of(c * (128 * BA), 128)
            bacc[c, pl.ds(a, n), :] = _dot(_cat([h]), wda_v[pl.ds(r, 128 * BA), :])
        return carry

    jax.lax.fori_loop(0, NA, phase_a, 0)
    wait(12, gw_v, wg_v.at[pl.ds(NFA, NF - NFA)], wu_v.at[pl.ds(NFA, NF - NFA)], wd_v)

    m16 = (_lane((RG, 128)) & 16) == 0
    m1 = (_lane((RG, 128)) & 1) == 0

    def attend(r0, base, scale, zvec):
        logits = []
        for w in range(WIN):
            if w % LGS == 0:
                if w:
                    scale = pltpu.bitcast(
                        pltpu.bitcast(scale, i32) | (pltpu.bitcast(raw, i32) & zvec), f32)
                q = [qkv_s[j, pl.ds(HALO + r0, RG), :] * scale for j in range(NB)]
            off = HALO + r0 - DIL * w
            acc = q[0] * qkv_s[NB, pl.ds(off, RG), :]
            for j in range(1, NB):
                acc = acc + q[j] * qkv_s[NB + j, pl.ds(off, RG), :]
            raw = acc
            acc = acc + jnp.where(m16, pltpu.roll(acc, 128 - 16, 1), pltpu.roll(acc, 16, 1))
            acc = acc + jnp.where(m1, pltpu.roll(acc, 128 - 1, 1), pltpu.roll(acc, 1, 1))
            if r0 < DIL * w:
                pos = base + r0 + jax.lax.broadcasted_iota(i32, (RG, 128), 0)
                acc = jnp.where(pos >= DIL * w, acc, NEG)
            logits.append(acc)
        m = logits[0]
        for w in range(1, WIN):
            m = jnp.maximum(m, logits[w])
        e = [jnp.exp2(l - m) for l in logits]
        s = e[0]
        for w in range(1, WIN):
            s = s + e[w]
        inv = pl.reciprocal(s, approx=True)
        inv = inv * (2.0 - s * inv)
        for j in range(NB):
            if j % PVS == 0:
                if j:
                    inv = pltpu.bitcast(pltpu.bitcast(inv, i32) | (pltpu.bitcast(o, i32) & zvec), f32)
                p = [x * inv for x in e]
            o = p[0] * qkv_s[2 * NB + j, pl.ds(HALO + r0, RG), :]
            for w in range(1, WIN):
                o = o + p[w] * qkv_s[2 * NB + j, pl.ds(HALO + r0 - DIL * w, RG), :]
            o_s[j, pl.ds(r0, RG), :] = o
        return o

    def phase_b(t, carry):
        base = pl.multiple_of(t * TB, TB)
        zero = zero_s[0]
        zvec = jnp.full((RG, 128), zero, i32)
        sbits = pltpu.bitcast(jnp.full((RG, 128), SCALE, f32), i32)
        x = x_v[pl.ds(base, TB), :]
        gw = pltpu.bitcast(jnp.broadcast_to(gw_v[...].astype(f32).reshape(1, D), (8, D)), i32)

        gates = []

        def gate_rows(r0, anchor):
            dep = pltpu.bitcast(anchor, i32) & zvec
            xr = x[r0:r0 + 16, :].astype(f32)
            acc = None
            for j in range(NB):
                w = pltpu.bitcast(gw[:, 128 * j:128 * (j + 1)] | dep, f32)
                term = xr[:, 128 * j:128 * (j + 1)] * jnp.concatenate([w, w], axis=0)
                acc = term if acc is None else acc + term
            z = jnp.sum(acc, axis=-1, keepdims=True)
            gates.append(jnp.broadcast_to(jax.nn.sigmoid(z), (16, 128)))

        for i in range(3):
            r = _dot(x, _cat([jnp.concatenate([w_p[i, j, pl.ds(PITCH * c, 64), :] for c in range(8)],
                                              axis=0) for j in range(NB)]))
            for j in range(NB):
                qkv_s[i * NB + j, pl.ds(HALO, TB), :] = r[:, 128 * j:128 * (j + 1)]
                if i * NB + j < TB // 16:
                    gate_rows(16 * (i * NB + j), r[ANCH:ANCH + 8, 128 * j:128 * (j + 1)])
        groups = list(range(0, TB, RG))
        nslots = 2 * (NF - NFA) - NSK
        hs = []
        slot = 0
        done = 0
        last = []

        def release(anchor):
            nonlocal slot, done
            slot += 1
            want = min(len(groups), -(-slot * len(groups) // nslots))
            if want > done:
                for r0 in groups[done:want]:
                    dep = pltpu.bitcast(anchor, i32)
                    if GDEP:
                        dep = dep | pltpu.bitcast(gates[r0 // 16][r0 % 16:r0 % 16 + 8], i32)
                    if last and (CHAIN == 1 or (CHAIN == 2 and r0 == TB - RG)):
                        dep = dep | pltpu.bitcast(last[-1], i32)
                    last.append(attend(r0, base, pltpu.bitcast(sbits | (dep & zvec), f32), zvec))
                done = want

        for c in range(NFA, NF, 2):
            g = _dot(x, _cat([wg_u[c], wg_u[c + 1]]))
            for n in range(2):
                release(g[ANCH:ANCH + 8, 128 * n:128 * (n + 1)])
            u = _dot(x, _cat([wu_u[c], wu_u[c + 1]]))
            for n in range(2):
                release(u[ANCH:ANCH + 8, 128 * n:128 * (n + 1)])
            hs.append(_reglu(g, u))
        assert done == len(groups)
        qkv_s[pl.ds(NB, 2 * NB), pl.ds(0, HALO), :] = qkv_s[pl.ds(NB, 2 * NB), pl.ds(TB, HALO), :]
        g = jnp.concatenate(gates, axis=0)
        g1 = 1.0 - g

        def down():
            wd = _cat([wd_u[j] for j in range(NB)])
            return (bacc[0, pl.ds(base, TB), :] + bacc[1, pl.ds(base, TB), :]
                    + _dot(_cat(hs), wd))

        if ORDER == 1:
            b = down()
        wo = _cat([jnp.concatenate([w_p[3, j, pl.ds(8 * m + c, 8, stride=PITCH), :]
                                    for c in range(8) for m in range(8)], axis=0)
                   for j in range(NB)])
        o_s[0, pl.ds(TB + zero, 8), :] = jnp.zeros((8, 128), f32)
        o = jnp.concatenate([o_s[j, pl.ds(0, TB), :] for j in range(NB)], axis=1)
        a = _dot(o.astype(bf16), wo)
        if ORDER == 0:
            b = down()
        for r0, r1, c0, c1 in OUTP:
            n = c1 - c0
            res = (jnp.concatenate([g[r0:r1]] * (n // 128), axis=1) * a[r0:r1, c0:c1]
                   + jnp.concatenate([g1[r0:r1]] * (n // 128), axis=1) * b[r0:r1, c0:c1])
            rs = pl.ds(pl.multiple_of(base + r0, 16), r1 - r0)
            out_v[rs, pl.ds(c0, n)] = res.astype(bf16)
            start(out_v.at[rs, pl.ds(c0, n)], out_hbm.at[rs, pl.ds(c0, n)], 13)
        return carry

    with _scope("B"):
        jax.lax.fori_loop(0, S // TB, phase_b, 0)
    wait(13, out_v)


@jax.jit
def pallas_gated_mix__sliding_local_dilated__glu_gated_reglu__prompt_kernel(
    A_x: jax.Array,
    A_wqkv: jax.Array,
    A_wo: jax.Array,
    B_x: jax.Array,
    B_W_gate: jax.Array,
    B_W_up: jax.Array,
    B_W_down: jax.Array,
    gate_w: jax.Array,
):
    del B_x
    x = A_x.reshape(S, D)
    hbm = pl.BlockSpec(memory_space=pl.ANY)
    out = pl.pallas_call(
        _kernel,
        out_shape=jax.ShapeDtypeStruct((S, D), bf16),
        in_specs=[hbm] * 7,
        out_specs=hbm,
        scratch_shapes=[
            pltpu.VMEM((S, D), bf16),
            pltpu.VMEM((4, D, D), bf16),
            pltpu.VMEM((NF, D, 128), bf16),
            pltpu.VMEM((NF, D, 128), bf16),
            pltpu.VMEM((128 * NFA, D), bf16),
            pltpu.VMEM((NB, F - 128 * NFA, 128), bf16),
            pltpu.VMEM((D,), bf16),
            pltpu.VMEM((4, NB, 8 * PITCH, 128), u32),
            pltpu.VMEM((2, S, D), f32),
            pltpu.VMEM((3 * NB, HALO + TB + 8, 128), f32),
            pltpu.VMEM((NB, TB + 8, 128), f32),
            pltpu.VMEM((S, D), bf16),
            pltpu.SMEM((1,), i32),
            pltpu.SemaphoreType.DMA((14,)),
        ],
        compiler_params=pltpu.CompilerParams(
            vmem_limit_bytes=110 * 1024 * 1024,
            disable_bounds_checks=not CHECKS,
            disable_semaphore_checks=not CHECKS,
        ),
    )(x, A_wqkv, A_wo, B_W_gate, B_W_up, B_W_down, gate_w)
    return out.reshape(1, S, D)
```

```python
import os
import jax
import jax.numpy as jnp
import jax.experimental.pallas as pl
import jax.experimental.pallas.tpu as pltpu

S, D, F = 2048, 1024, 3584
H, DH, WIN, DIL = 32, 32, 8, 2
NB = D // 128
NF = F // 128
HALO = 16
BA = 3
NFA = 2 * BA
R0 = 496
NA = 5
UR = (2 * S - R0) // NA
SUB = (0, (S - R0) % UR, UR)
TB = 256
RG = 8
ANCH = int(os.environ.get('ANCH', 248))
NSK = int(os.environ.get('NSK', 4))
ORDER = int(os.environ.get('ORDER', 0))
OUTP = {0: ((0, 256, 0, 512), (0, 256, 512, 768), (0, 256, 768, 1024)),
        1: ((0, 256, 0, 512), (0, 256, 512, 768), (0, 192, 768, 1024), (192, 256, 768, 1024)),
        2: ((0, 256, 0, 512), (0, 256, 512, 896), (0, 192, 896, 1024), (192, 256, 896, 1024)),
        3: ((0, 256, 0, 768), (0, 128, 768, 1024), (128, 224, 768, 1024), (224, 256, 768, 1024)),
        }[int(os.environ.get('OUTP', 2))]
GDEP = int(os.environ.get('GDEP', 1))
PVS = int(os.environ.get('PVS', 2))
LGS = int(os.environ.get('LGS', 4))
P0M = int(os.environ.get('P0M', 0))
CHAIN = int(os.environ.get('CHAIN', 1))
SCOPES = int(os.environ.get("SCOPES", 0))
CHECKS = int(os.environ.get("CHECKS", 0))
PITCH = 65
CPU = int(os.environ.get('CPU', 8))
COFF = NA * CPU - 32
CH1 = max(CPU - COFF, 1)
NCH = 4 * 8
LOG2E = 1.4426950408889634
SCALE = DH ** -0.5 * LOG2E
NEG = -1e9 * LOG2E

f32 = jnp.float32
bf16 = jnp.bfloat16
u32 = jnp.uint32
i32 = jnp.int32


def _dot(a, b):
    return jnp.dot(a, b, preferred_element_type=f32)


def _lane(shape):
    return jax.lax.broadcasted_iota(i32, shape, 1)


def _cat(blocks):
    return jnp.concatenate([pltpu.bitcast(b, bf16) for b in blocks], axis=1)


def _reglu(g, u):
    return pltpu.bitcast((jnp.maximum(g, 0.0) * u).astype(bf16), u32)


class _NoScope:
    def __enter__(self):
        return self

    def __exit__(self, *a):
        return False


def _scope(name):
    return jax.named_scope(name) if SCOPES else _NoScope()


def _kernel(x_hbm, wqkv_hbm, wo_hbm, wg_hbm, wu_hbm, wd_hbm, gw_hbm, out_hbm,
            x_v, w_v, wg_v, wu_v, wda_v, wd_v, gw_v, w_p, bacc,
            qkv_s, o_s, out_v, zero_s, sems):
    def start(src, dst, grp):
        pltpu.make_async_copy(src, dst, sems.at[grp]).start()

    def wait(grp, *dsts):
        with _scope("w%d" % grp):
            for d in dsts:
                pltpu.make_async_copy(d, d, sems.at[grp]).wait()

    def xrows(a, n):
        return x_v.at[pl.ds(a, n), :]

    def get_x(a, n, grp):
        start(x_hbm.at[pl.ds(a, n), :], xrows(a, n), grp)

    def get_cols(hbm, dst, b0, b1, grp):
        for b in range(b0, b1):
            start(hbm.at[:, pl.ds(128 * b, 128)], dst.at[b], grp)

    def wda_rows(b0, b1):
        return wda_v.at[pl.ds(128 * b0, 128 * (b1 - b0)), :]

    def get_wda(b0, b1, grp):
        start(wd_hbm.at[pl.ds(128 * b0, 128 * (b1 - b0)), :], wda_rows(b0, b1), grp)

    def w_rows(c0, c1):
        out = []
        for p in range(4):
            a, b = max(c0, 8 * p), min(c1, 8 * p + 8)
            if a < b:
                out.append((p, 128 * (a - 8 * p), 128 * (b - a)))
        return out

    def w_dst(c0, c1):
        return [w_v.at[p, pl.ds(r, n), :] for p, r, n in w_rows(c0, c1)]

    def get_w(c0, c1, grp):
        for p, r, n in w_rows(c0, c1):
            src = (wqkv_hbm.at[pl.ds(r, n), pl.ds(p * D, D)] if p < 3
                   else wo_hbm.at[pl.ds(r, n), :])
            start(src, w_v.at[p, pl.ds(r, n), :], grp)

    get_x(0, 128, 0)
    get_cols(wg_hbm, wg_v, 0, 1, 0)
    get_x(128, 128, 1)
    get_cols(wu_hbm, wu_v, 0, 1, 2)
    get_x(256, 128, 3)
    get_cols(wg_hbm, wg_v, 1, 2, 4)
    get_x(384, R0 - 384, 5)
    get_cols(wu_hbm, wu_v, 1, 2, 5)
    get_cols(wg_hbm, wg_v, 2, 3, 6)
    get_cols(wu_hbm, wu_v, 2, 3, 6)
    get_wda(0, 2, 6)
    get_wda(2, 3, 7)
    get_x(R0, UR, 8)
    get_w(0, CH1, 8)
    get_x(R0 + UR, UR, 9)
    get_w(CH1, 2 * CPU - COFF, 9)
    get_x(R0 + 2 * UR, S - R0 - 2 * UR, 10)
    get_cols(wg_hbm, wg_v, BA, NFA, 10)
    get_cols(wu_hbm, wu_v, BA, NFA, 10)
    get_wda(BA, NFA, 10)
    get_w(2 * CPU - COFF, NCH, 10)
    start(gw_hbm, gw_v, 12)
    for j in range(NB):
        start(wd_hbm.at[pl.ds(128 * NFA, F - 128 * NFA), pl.ds(128 * j, 128)], wd_v.at[j], 12)
    get_cols(wg_hbm, wg_v, NFA, NF, 12)

    wg_u, wu_u, wd_u = (r.bitcast(u32) for r in (wg_v, wu_v, wd_v))

    zero_s[0] = 0
    qkv_s[pl.ds(NB, 2 * NB), pl.ds(0, HALO), :] = jnp.zeros((2 * NB, HALO, 128), f32)

    def repack(ch):
        p = jax.lax.shift_right_logical(ch, 3)
        rc = ch & 7
        on = jnp.where(ch < 24, -1, 0).astype(i32)
        r0 = pl.multiple_of(rc * 128, 128)
        blk = [pltpu.bitcast(w_v[p, pl.ds(r0, 128), pl.ds(128 * j, 128)], u32) for j in range(NB)]
        lane = _lane((64, 128))
        for bb, lb in ((2, 3), (1, 2), (0, 1)):
            sh = 1 << lb
            keep_a = (lane & (on & sh)) == 0
            take_a = ((lane & sh) | (~on & 1)) == 0
            for j in range(NB):
                if j & (1 << bb):
                    continue
                a, b = blk[j], blk[j | (1 << bb)]
                blk[j] = jnp.where(keep_a, a, pltpu.roll(b, sh, 1))
                blk[j | (1 << bb)] = jnp.where(take_a, pltpu.roll(a, 128 - sh, 1), b)
        for j in range(NB):
            w_p[p, j, pl.ds(rc * PITCH, 64), :] = blk[j]

    def main(_, carry0):
        def xr(a, b):
            return x_v[pl.ds(a, b - a), :]

        def rcat(*parts):
            return jnp.concatenate(parts, axis=0)

        wait(0, xrows(0, 128), wg_v.at[0])
        g0a = _dot(xr(0, 128), _cat([wg_u[0]]))
        wait(1, xrows(128, 128))
        g0b = _dot(xr(128, 256), _cat([wg_u[0]]))
        wait(2, wu_v.at[0])
        h0a = _reglu(rcat(g0a, g0b), _dot(xr(0, 256), _cat([wu_u[0]])))
        wait(3, xrows(256, 128))
        gu = _dot(xr(256, 384), _cat([wg_u[0], wu_u[0]]))
        h0b = _reglu(gu[:, :128], gu[:, 128:])
        wait(4, wg_v.at[1])
        g1a = _dot(xr(0, 384), _cat([wg_u[1]]))
        wait(5, xrows(384, R0 - 384), wu_v.at[1])
        gu = _dot(xr(384, R0), _cat([wg_u[0], wu_u[0], wg_u[1]]))
        h0c = _reglu(gu[:, :128], gu[:, 128:256])
        h1 = _reglu(rcat(g1a, gu[:, 256:]), _dot(xr(0, R0), _cat([wu_u[1]])))
        if P0M:
            wait(6, wg_v.at[2], wu_v.at[2], wda_rows(0, 2))
            wait(7, wda_rows(2, 3))
        else:
            wait(6, wg_v.at[2], wu_v.at[2], wda_rows(0, 2))
        gu = _dot(xr(0, R0), _cat([wg_u[2], wu_u[2]]))
        h2 = _reglu(gu[:, :128], gu[:, 128:])
        get_cols(wu_hbm, wu_v, NFA, NF, 12)
        if not P0M:
            wait(7, wda_rows(2, 3))
        bacc[0, pl.ds(0, R0), :] = _dot(_cat([rcat(h0a, h0b, h0c), h1, h2]), wda_v[pl.ds(0, 128 * BA), :])

        def phase_a(u, carry):
            pl.when(u == 0)(lambda: wait(8, xrows(R0, UR), *w_dst(0, CH1)))
            pl.when(u == 1)(lambda: wait(9, xrows(R0 + UR, UR), *w_dst(CH1, 2 * CPU - COFF)))
            pl.when(u == 2)(lambda: wait(10, xrows(R0 + 2 * UR, S - R0 - 2 * UR), wg_v.at[pl.ds(BA, BA)],
                                         wu_v.at[pl.ds(BA, BA)], wda_rows(BA, NFA),
                                         *w_dst(2 * CPU - COFF, NCH)))
            parts = []
            for v0, v1 in zip(SUB[:-1], SUB[1:]):
                v = u * UR + v0
                c = (v >= S - R0).astype(i32)
                a = pl.multiple_of(v + R0 - c * S, 16)
                x = x_v[pl.ds(a, v1 - v0), :]
                h = _reglu(_dot(x, _cat([wg_u[c * BA + k] for k in range(BA)])),
                           _dot(x, _cat([wu_u[c * BA + k] for k in range(BA)])))
                parts.append((c, a, v1 - v0, h))
            for k in range(CPU):
                repack(jnp.maximum(CPU * u + k - COFF, 0))
            for c, a, n, h in parts:
                r = pl.multiple_of(c * (128 * BA), 128)
                bacc[c, pl.ds(a, n), :] = _dot(_cat([h]), wda_v[pl.ds(r, 128 * BA), :])
            return carry

        jax.lax.fori_loop(0, NA, phase_a, 0)
        wait(12, gw_v, wg_v.at[pl.ds(NFA, NF - NFA)], wu_v.at[pl.ds(NFA, NF - NFA)], wd_v)

        m16 = (_lane((RG, 128)) & 16) == 0
        m1 = (_lane((RG, 128)) & 1) == 0

        def attend(r0, base, scale, zvec):
            logits = []
            for w in range(WIN):
                if w % LGS == 0:
                    if w:
                        scale = pltpu.bitcast(
                            pltpu.bitcast(scale, i32) | (pltpu.bitcast(raw, i32) & zvec), f32)
                    q = [qkv_s[j, pl.ds(HALO + r0, RG), :] * scale for j in range(NB)]
                off = HALO + r0 - DIL * w
                acc = q[0] * qkv_s[NB, pl.ds(off, RG), :]
                for j in range(1, NB):
                    acc = acc + q[j] * qkv_s[NB + j, pl.ds(off, RG), :]
                raw = acc
                acc = acc + jnp.where(m16, pltpu.roll(acc, 128 - 16, 1), pltpu.roll(acc, 16, 1))
                acc = acc + jnp.where(m1, pltpu.roll(acc, 128 - 1, 1), pltpu.roll(acc, 1, 1))
                if r0 < DIL * w:
                    pos = base + r0 + jax.lax.broadcasted_iota(i32, (RG, 128), 0)
                    acc = jnp.where(pos >= DIL * w, acc, NEG)
                logits.append(acc)
            m = logits[0]
            for w in range(1, WIN):
                m = jnp.maximum(m, logits[w])
            e = [jnp.exp2(l - m) for l in logits]
            s = e[0]
            for w in range(1, WIN):
                s = s + e[w]
            inv = pl.reciprocal(s, approx=True)
            inv = inv * (2.0 - s * inv)
            for j in range(NB):
                if j % PVS == 0:
                    if j:
                        inv = pltpu.bitcast(pltpu.bitcast(inv, i32) | (pltpu.bitcast(o, i32) & zvec), f32)
                    p = [x * inv for x in e]
                o = p[0] * qkv_s[2 * NB + j, pl.ds(HALO + r0, RG), :]
                for w in range(1, WIN):
                    o = o + p[w] * qkv_s[2 * NB + j, pl.ds(HALO + r0 - DIL * w, RG), :]
                o_s[j, pl.ds(r0, RG), :] = o
            return o

        def phase_b(t, carry):
            base = pl.multiple_of(t * TB, TB)
            zero = zero_s[0]
            zvec = jnp.full((RG, 128), zero, i32)
            sbits = pltpu.bitcast(jnp.full((RG, 128), SCALE, f32), i32)
            x = x_v[pl.ds(base, TB), :]
            gw = pltpu.bitcast(jnp.broadcast_to(gw_v[...].astype(f32).reshape(1, D), (8, D)), i32)

            gates = []

            def gate_rows(r0, anchor):
                dep = pltpu.bitcast(anchor, i32) & zvec
                xr = x[r0:r0 + 16, :].astype(f32)
                acc = None
                for j in range(NB):
                    w = pltpu.bitcast(gw[:, 128 * j:128 * (j + 1)] | dep, f32)
                    term = xr[:, 128 * j:128 * (j + 1)] * jnp.concatenate([w, w], axis=0)
                    acc = term if acc is None else acc + term
                z = jnp.sum(acc, axis=-1, keepdims=True)
                gates.append(jnp.broadcast_to(jax.nn.sigmoid(z), (16, 128)))

            for i in range(3):
                r = _dot(x, _cat([jnp.concatenate([w_p[i, j, pl.ds(PITCH * c, 64), :] for c in range(8)],
                                                  axis=0) for j in range(NB)]))
                for j in range(NB):
                    qkv_s[i * NB + j, pl.ds(HALO, TB), :] = r[:, 128 * j:128 * (j + 1)]
                    if i * NB + j < TB // 16:
                        gate_rows(16 * (i * NB + j), r[ANCH:ANCH + 8, 128 * j:128 * (j + 1)])
            groups = list(range(0, TB, RG))
            nslots = 2 * (NF - NFA) - NSK
            hs = []
            slot = 0
            done = 0
            last = []

            def release(anchor):
                nonlocal slot, done
                slot += 1
                want = min(len(groups), -(-slot * len(groups) // nslots))
                if want > done:
                    for r0 in groups[done:want]:
                        dep = pltpu.bitcast(anchor, i32)
                        if GDEP:
                            dep = dep | pltpu.bitcast(gates[r0 // 16][r0 % 16:r0 % 16 + 8], i32)
                        if last and (CHAIN == 1 or (CHAIN == 2 and r0 == TB - RG)):
                            dep = dep | pltpu.bitcast(last[-1], i32)
                        last.append(attend(r0, base, pltpu.bitcast(sbits | (dep & zvec), f32), zvec))
                    done = want

            for c in range(NFA, NF, 2):
                g = _dot(x, _cat([wg_u[c], wg_u[c + 1]]))
                for n in range(2):
                    release(g[ANCH:ANCH + 8, 128 * n:128 * (n + 1)])
                u = _dot(x, _cat([wu_u[c], wu_u[c + 1]]))
                for n in range(2):
                    release(u[ANCH:ANCH + 8, 128 * n:128 * (n + 1)])
                hs.append(_reglu(g, u))
            assert done == len(groups)
            qkv_s[pl.ds(NB, 2 * NB), pl.ds(0, HALO), :] = qkv_s[pl.ds(NB, 2 * NB), pl.ds(TB, HALO), :]
            g = jnp.concatenate(gates, axis=0)
            g1 = 1.0 - g

            def down():
                wd = _cat([wd_u[j] for j in range(NB)])
                return (bacc[0, pl.ds(base, TB), :] + bacc[1, pl.ds(base, TB), :]
                        + _dot(_cat(hs), wd))

            if ORDER == 1:
                b = down()
            wo = _cat([jnp.concatenate([w_p[3, j, pl.ds(8 * m + c, 8, stride=PITCH), :]
                                        for c in range(8) for m in range(8)], axis=0)
                       for j in range(NB)])
            o_s[0, pl.ds(TB + zero, 8), :] = jnp.zeros((8, 128), f32)
            o = jnp.concatenate([o_s[j, pl.ds(0, TB), :] for j in range(NB)], axis=1)
            a = _dot(o.astype(bf16), wo)
            if ORDER == 0:
                b = down()
            for r0, r1, c0, c1 in OUTP:
                n = c1 - c0
                res = (jnp.concatenate([g[r0:r1]] * (n // 128), axis=1) * a[r0:r1, c0:c1]
                       + jnp.concatenate([g1[r0:r1]] * (n // 128), axis=1) * b[r0:r1, c0:c1])
                rs = pl.ds(pl.multiple_of(base + r0, 16), r1 - r0)
                out_v[rs, pl.ds(c0, n)] = res.astype(bf16)
                start(out_v.at[rs, pl.ds(c0, n)], out_hbm.at[rs, pl.ds(c0, n)], 13)
            return carry

        with _scope("B"):
            jax.lax.fori_loop(0, S // TB, phase_b, 0)
        return carry0

    jax.lax.fori_loop(0, zero_s[0] + 1, main, 0)
    wait(13, out_v)


@jax.jit
def pallas_gated_mix__sliding_local_dilated__glu_gated_reglu__prompt_kernel(
    A_x: jax.Array,
    A_wqkv: jax.Array,
    A_wo: jax.Array,
    B_x: jax.Array,
    B_W_gate: jax.Array,
    B_W_up: jax.Array,
    B_W_down: jax.Array,
    gate_w: jax.Array,
):
    del B_x
    x = A_x.reshape(S, D)
    hbm = pl.BlockSpec(memory_space=pl.ANY)
    out = pl.pallas_call(
        _kernel,
        out_shape=jax.ShapeDtypeStruct((S, D), bf16),
        in_specs=[hbm] * 7,
        out_specs=hbm,
        scratch_shapes=[
            pltpu.VMEM((S, D), bf16),
            pltpu.VMEM((4, D, D), bf16),
            pltpu.VMEM((NF, D, 128), bf16),
            pltpu.VMEM((NF, D, 128), bf16),
            pltpu.VMEM((128 * NFA, D), bf16),
            pltpu.VMEM((NB, F - 128 * NFA, 128), bf16),
            pltpu.VMEM((D,), bf16),
            pltpu.VMEM((4, NB, 8 * PITCH, 128), u32),
            pltpu.VMEM((2, S, D), f32),
            pltpu.VMEM((3 * NB, HALO + TB + 8, 128), f32),
            pltpu.VMEM((NB, TB + 8, 128), f32),
            pltpu.VMEM((S, D), bf16),
            pltpu.SMEM((1,), i32),
            pltpu.SemaphoreType.DMA((14,)),
        ],
        compiler_params=pltpu.CompilerParams(
            vmem_limit_bytes=110 * 1024 * 1024,
            disable_bounds_checks=not CHECKS,
            disable_semaphore_checks=not CHECKS,
        ),
    )(x, A_wqkv, A_wo, B_W_gate, B_W_up, B_W_down, gate_w)
    return out.reshape(1, S, D)
```

```python
import os
import jax
import jax.numpy as jnp
import jax.experimental.pallas as pl
import jax.experimental.pallas.tpu as pltpu

S, D, F = 2048, 1024, 3584
H, DH, WIN, DIL = 32, 32, 8, 2
NB = D // 128
NF = F // 128
HALO = 16
BA = 3
NFA = 2 * BA
R0 = int(os.environ.get('R0', 640))
NA = int(os.environ.get('NA', 4))
UR = (2 * S - R0) // NA
SUB = (0, (S - R0) % UR, UR)
TB = 256
RG = 8
ANCH = int(os.environ.get('ANCH', 248))
NSK = int(os.environ.get('NSK', 4))
ORDER = int(os.environ.get('ORDER', 0))
OUTP = {0: ((0, 256, 0, 512), (0, 256, 512, 768), (0, 256, 768, 1024)),
        1: ((0, 256, 0, 512), (0, 256, 512, 768), (0, 192, 768, 1024), (192, 256, 768, 1024)),
        2: ((0, 256, 0, 512), (0, 256, 512, 896), (0, 192, 896, 1024), (192, 256, 896, 1024)),
        3: ((0, 256, 0, 768), (0, 128, 768, 1024), (128, 224, 768, 1024), (224, 256, 768, 1024)),
        }[int(os.environ.get('OUTP', 2))]
GDEP = int(os.environ.get('GDEP', 1))
PVS = int(os.environ.get('PVS', 2))
LGS = int(os.environ.get('LGS', 4))
CHAIN = int(os.environ.get('CHAIN', 1))
SCOPES = int(os.environ.get("SCOPES", 0))
CHECKS = int(os.environ.get("CHECKS", 0))
PITCH = 65
CPU = int(os.environ.get('CPU', 9))
COFF = NA * CPU - 32
CH1 = max(CPU - COFF, 1)
NCH = 4 * 8
LOG2E = 1.4426950408889634
SCALE = DH ** -0.5 * LOG2E
NEG = -1e9 * LOG2E

f32 = jnp.float32
bf16 = jnp.bfloat16
u32 = jnp.uint32
i32 = jnp.int32


def _dot(a, b):
    return jnp.dot(a, b, preferred_element_type=f32)


def _lane(shape):
    return jax.lax.broadcasted_iota(i32, shape, 1)


def _cat(blocks):
    return jnp.concatenate([pltpu.bitcast(b, bf16) for b in blocks], axis=1)


def _reglu(g, u):
    return jnp.maximum(g, 0.0) * u


def _hcat(hs):
    return jnp.concatenate(hs, axis=1).astype(bf16)


class _NoScope:
    def __enter__(self):
        return self

    def __exit__(self, *a):
        return False


def _scope(name):
    return jax.named_scope(name) if SCOPES else _NoScope()


def _kernel(x_hbm, wqkv_hbm, wo_hbm, wg_hbm, wu_hbm, wd_hbm, gw_hbm, out_hbm,
            x_v, w_v, wg_v, wu_v, wda_v, wd_v, gw_v, w_p, bacc,
            qkv_s, o_s, out_v, zero_s, sems):
    def start(src, dst, grp):
        pltpu.make_async_copy(src, dst, sems.at[grp]).start()

    def wait(grp, *dsts):
        with _scope("w%d" % grp):
            for d in dsts:
                pltpu.make_async_copy(d, d, sems.at[grp]).wait()

    def xrows(a, n):
        return x_v.at[pl.ds(a, n), :]

    def get_x(a, n, grp):
        start(x_hbm.at[pl.ds(a, n), :], xrows(a, n), grp)

    def get_cols(hbm, dst, b0, b1, grp):
        for b in range(b0, b1):
            start(hbm.at[:, pl.ds(128 * b, 128)], dst.at[b], grp)

    def wda_rows(b0, b1):
        return wda_v.at[pl.ds(128 * b0, 128 * (b1 - b0)), :]

    def get_wda(b0, b1, grp):
        start(wd_hbm.at[pl.ds(128 * b0, 128 * (b1 - b0)), :], wda_rows(b0, b1), grp)

    def w_rows(c0, c1):
        out = []
        for p in range(4):
            a, b = max(c0, 8 * p), min(c1, 8 * p + 8)
            if a < b:
                out.append((p, 128 * (a - 8 * p), 128 * (b - a)))
        return out

    def w_dst(c0, c1):
        return [w_v.at[p, pl.ds(r, n), :] for p, r, n in w_rows(c0, c1)]

    def get_w(c0, c1, grp):
        for p, r, n in w_rows(c0, c1):
            src = (wqkv_hbm.at[pl.ds(r, n), pl.ds(p * D, D)] if p < 3
                   else wo_hbm.at[pl.ds(r, n), :])
            start(src, w_v.at[p, pl.ds(r, n), :], grp)

    get_x(0, 128, 0)
    get_cols(wg_hbm, wg_v, 0, 1, 0)
    get_x(128, 128, 1)
    get_cols(wu_hbm, wu_v, 0, 1, 2)
    get_x(256, 128, 3)
    get_cols(wg_hbm, wg_v, 1, 2, 4)
    get_x(384, R0 - 384, 5)
    get_cols(wu_hbm, wu_v, 1, 2, 6)
    get_cols(wg_hbm, wg_v, 2, 3, 6)
    get_cols(wu_hbm, wu_v, 2, 3, 6)
    get_wda(0, BA, 7)
    ucross = (S - R0) // UR
    udst = []
    for u in range(3):
        dst = []
        x0, x1 = min(S, R0 + u * UR), (min(S, R0 + (u + 1) * UR) if u < 2 else S)
        if x0 < x1:
            get_x(x0, x1 - x0, 8 + u)
            dst.append(xrows(x0, x1 - x0))
        if u == min(ucross, 2):
            get_cols(wg_hbm, wg_v, BA, NFA, 8 + u)
            get_cols(wu_hbm, wu_v, BA, NFA, 8 + u)
            get_wda(BA, NFA, 8 + u)
            dst += [wg_v.at[pl.ds(BA, BA)], wu_v.at[pl.ds(BA, BA)], wda_rows(BA, NFA)]
        c0, c1 = (0, CH1, 2 * CPU - COFF, NCH)[u:u + 2]
        get_w(c0, c1, 8 + u)
        udst.append(dst + w_dst(c0, c1))
    start(gw_hbm, gw_v, 12)
    for j in range(NB):
        start(wd_hbm.at[pl.ds(128 * NFA, F - 128 * NFA), pl.ds(128 * j, 128)], wd_v.at[j], 12)
    get_cols(wg_hbm, wg_v, NFA, NF, 12)

    wg_u, wu_u, wd_u = (r.bitcast(u32) for r in (wg_v, wu_v, wd_v))

    zero_s[0] = 0
    qkv_s[pl.ds(NB, 2 * NB), pl.ds(0, HALO), :] = jnp.zeros((2 * NB, HALO, 128), f32)

    def repack(ch):
        p = jax.lax.shift_right_logical(ch, 3)
        rc = ch & 7
        on = jnp.where(ch < 24, -1, 0).astype(i32)
        r0 = pl.multiple_of(rc * 128, 128)
        blk = [pltpu.bitcast(w_v[p, pl.ds(r0, 128), pl.ds(128 * j, 128)], u32) for j in range(NB)]
        lane = _lane((64, 128))
        for bb, lb in ((2, 3), (1, 2), (0, 1)):
            sh = 1 << lb
            keep_a = (lane & (on & sh)) == 0
            take_a = ((lane & sh) | (~on & 1)) == 0
            for j in range(NB):
                if j & (1 << bb):
                    continue
                a, b = blk[j], blk[j | (1 << bb)]
                blk[j] = jnp.where(keep_a, a, pltpu.roll(b, sh, 1))
                blk[j | (1 << bb)] = jnp.where(take_a, pltpu.roll(a, 128 - sh, 1), b)
        for j in range(NB):
            w_p[p, j, pl.ds(rc * PITCH, 64), :] = blk[j]

    def main(_, carry0):
        def xr(a, b):
            return x_v[pl.ds(a, b - a), :]

        def rcat(*parts):
            return jnp.concatenate(parts, axis=0)

        wait(0, xrows(0, 128), wg_v.at[0])
        g0a = _dot(xr(0, 128), _cat([wg_u[0]]))
        wait(1, xrows(128, 128))
        g0b = _dot(xr(128, 256), _cat([wg_u[0]]))
        wait(2, wu_v.at[0])
        h0a = _reglu(rcat(g0a, g0b), _dot(xr(0, 256), _cat([wu_u[0]])))
        wait(3, xrows(256, 128))
        gu = _dot(xr(256, 384), _cat([wg_u[0], wu_u[0]]))
        h0b = _reglu(gu[:, :128], gu[:, 128:])
        wait(4, wg_v.at[1])
        g1a = _dot(xr(0, 384), _cat([wg_u[1]]))
        wait(5, xrows(384, R0 - 384))
        gu = _dot(xr(384, R0), _cat([wg_u[0], wu_u[0], wg_u[1]]))
        h0c = _reglu(gu[:, :128], gu[:, 128:256])
        g1 = rcat(g1a, gu[:, 256:])
        wait(6, wu_v.at[pl.ds(1, 2)], wg_v.at[2])
        gu = _dot(xr(0, R0), _cat([wu_u[1], wg_u[2], wu_u[2]]))
        h1 = _reglu(g1, gu[:, :128])
        h2 = _reglu(gu[:, 128:256], gu[:, 256:])
        get_cols(wu_hbm, wu_v, NFA, NF, 12)
        wait(7, wda_rows(0, BA))
        bacc[0, pl.ds(0, R0), :] = _dot(_hcat([rcat(h0a, h0b, h0c), h1, h2]),
                                        wda_v[pl.ds(0, 128 * BA), :])

        def phase_a(u, carry):
            for k in range(3):
                pl.when(u == k)(lambda k=k: wait(8 + k, *udst[k]))
            parts = []
            for v0, v1 in zip(SUB[:-1], SUB[1:]):
                v = u * UR + v0
                c = (v >= S - R0).astype(i32)
                a = pl.multiple_of(v + R0 - c * S, 16)
                x = x_v[pl.ds(a, v1 - v0), :]
                h = _reglu(_dot(x, _cat([wg_u[c * BA + k] for k in range(BA)])),
                           _dot(x, _cat([wu_u[c * BA + k] for k in range(BA)])))
                parts.append((c, a, v1 - v0, h))
            for k in range(CPU):
                repack(jnp.maximum(CPU * u + k - COFF, 0))
            for c, a, n, h in parts:
                r = pl.multiple_of(c * (128 * BA), 128)
                bacc[c, pl.ds(a, n), :] = _dot(_hcat([h]), wda_v[pl.ds(r, 128 * BA), :])
            return carry

        jax.lax.fori_loop(0, NA, phase_a, 0)
        wait(12, gw_v, wg_v.at[pl.ds(NFA, NF - NFA)], wu_v.at[pl.ds(NFA, NF - NFA)], wd_v)

        m16 = (_lane((RG, 128)) & 16) == 0
        m1 = (_lane((RG, 128)) & 1) == 0

        def attend(r0, base, scale, zvec):
            logits = []
            for w in range(WIN):
                if w % LGS == 0:
                    if w:
                        scale = pltpu.bitcast(
                            pltpu.bitcast(scale, i32) | (pltpu.bitcast(raw, i32) & zvec), f32)
                    q = [qkv_s[j, pl.ds(HALO + r0, RG), :] * scale for j in range(NB)]
                off = HALO + r0 - DIL * w
                acc = q[0] * qkv_s[NB, pl.ds(off, RG), :]
                for j in range(1, NB):
                    acc = acc + q[j] * qkv_s[NB + j, pl.ds(off, RG), :]
                raw = acc
                acc = acc + jnp.where(m16, pltpu.roll(acc, 128 - 16, 1), pltpu.roll(acc, 16, 1))
                acc = acc + jnp.where(m1, pltpu.roll(acc, 128 - 1, 1), pltpu.roll(acc, 1, 1))
                if r0 < DIL * w:
                    pos = base + r0 + jax.lax.broadcasted_iota(i32, (RG, 128), 0)
                    acc = jnp.where(pos >= DIL * w, acc, NEG)
                logits.append(acc)
            m = logits[0]
            for w in range(1, WIN):
                m = jnp.maximum(m, logits[w])
            e = [jnp.exp2(l - m) for l in logits]
            s = e[0]
            for w in range(1, WIN):
                s = s + e[w]
            inv = pl.reciprocal(s, approx=True)
            inv = inv * (2.0 - s * inv)
            for j in range(NB):
                if j % PVS == 0:
                    if j:
                        inv = pltpu.bitcast(pltpu.bitcast(inv, i32) | (pltpu.bitcast(o, i32) & zvec), f32)
                    p = [x * inv for x in e]
                o = p[0] * qkv_s[2 * NB + j, pl.ds(HALO + r0, RG), :]
                for w in range(1, WIN):
                    o = o + p[w] * qkv_s[2 * NB + j, pl.ds(HALO + r0 - DIL * w, RG), :]
                o_s[j, pl.ds(r0, RG), :] = o
            return o

        def phase_b(t, carry):
            base = pl.multiple_of(t * TB, TB)
            zero = zero_s[0]
            zvec = jnp.full((RG, 128), zero, i32)
            sbits = pltpu.bitcast(jnp.full((RG, 128), SCALE, f32), i32)
            x = x_v[pl.ds(base, TB), :]
            gw = pltpu.bitcast(jnp.broadcast_to(gw_v[...].astype(f32).reshape(1, D), (8, D)), i32)

            gates = []

            def gate_rows(r0, anchor):
                dep = pltpu.bitcast(anchor, i32) & zvec
                xr = x[r0:r0 + 16, :].astype(f32)
                acc = None
                for j in range(NB):
                    w = pltpu.bitcast(gw[:, 128 * j:128 * (j + 1)] | dep, f32)
                    term = xr[:, 128 * j:128 * (j + 1)] * jnp.concatenate([w, w], axis=0)
                    acc = term if acc is None else acc + term
                z = jnp.sum(acc, axis=-1, keepdims=True)
                gates.append(jnp.broadcast_to(jax.nn.sigmoid(z), (16, 128)))

            for i in range(3):
                r = _dot(x, _cat([jnp.concatenate([w_p[i, j, pl.ds(PITCH * c, 64), :] for c in range(8)],
                                                  axis=0) for j in range(NB)]))
                for j in range(NB):
                    qkv_s[i * NB + j, pl.ds(HALO, TB), :] = r[:, 128 * j:128 * (j + 1)]
                    if i * NB + j < TB // 16:
                        gate_rows(16 * (i * NB + j), r[ANCH:ANCH + 8, 128 * j:128 * (j + 1)])
            groups = list(range(0, TB, RG))
            nslots = 2 * (NF - NFA) - NSK
            hs = []
            slot = 0
            done = 0
            last = []

            def release(anchor):
                nonlocal slot, done
                slot += 1
                want = min(len(groups), -(-slot * len(groups) // nslots))
                if want > done:
                    for r0 in groups[done:want]:
                        dep = pltpu.bitcast(anchor, i32)
                        if GDEP:
                            dep = dep | pltpu.bitcast(gates[r0 // 16][r0 % 16:r0 % 16 + 8], i32)
                        if last and (CHAIN == 1 or (CHAIN == 2 and r0 == TB - RG)):
                            dep = dep | pltpu.bitcast(last[-1], i32)
                        last.append(attend(r0, base, pltpu.bitcast(sbits | (dep & zvec), f32), zvec))
                    done = want

            for c in range(NFA, NF, 2):
                g = _dot(x, _cat([wg_u[c], wg_u[c + 1]]))
                for n in range(2):
                    release(g[ANCH:ANCH + 8, 128 * n:128 * (n + 1)])
                u = _dot(x, _cat([wu_u[c], wu_u[c + 1]]))
                for n in range(2):
                    release(u[ANCH:ANCH + 8, 128 * n:128 * (n + 1)])
                hs.append(_reglu(g, u))
            assert done == len(groups)
            qkv_s[pl.ds(NB, 2 * NB), pl.ds(0, HALO), :] = qkv_s[pl.ds(NB, 2 * NB), pl.ds(TB, HALO), :]
            g = jnp.concatenate(gates, axis=0)
            g1 = 1.0 - g

            def down():
                wd = _cat([wd_u[j] for j in range(NB)])
                return (bacc[0, pl.ds(base, TB), :] + bacc[1, pl.ds(base, TB), :]
                        + _dot(_hcat(hs), wd))

            if ORDER == 1:
                b = down()
            wo = _cat([jnp.concatenate([w_p[3, j, pl.ds(8 * m + c, 8, stride=PITCH), :]
                                        for c in range(8) for m in range(8)], axis=0)
                       for j in range(NB)])
            o_s[0, pl.ds(TB + zero, 8), :] = jnp.zeros((8, 128), f32)
            o = jnp.concatenate([o_s[j, pl.ds(0, TB), :] for j in range(NB)], axis=1)
            a = _dot(o.astype(bf16), wo)
            if ORDER == 0:
                b = down()
            for r0, r1, c0, c1 in OUTP:
                n = c1 - c0
                res = (jnp.concatenate([g[r0:r1]] * (n // 128), axis=1) * a[r0:r1, c0:c1]
                       + jnp.concatenate([g1[r0:r1]] * (n // 128), axis=1) * b[r0:r1, c0:c1])
                rs = pl.ds(pl.multiple_of(base + r0, 16), r1 - r0)
                out_v[rs, pl.ds(c0, n)] = res.astype(bf16)
                start(out_v.at[rs, pl.ds(c0, n)], out_hbm.at[rs, pl.ds(c0, n)], 13)
            return carry

        with _scope("B"):
            jax.lax.fori_loop(0, S // TB, phase_b, 0)
        return carry0

    jax.lax.fori_loop(0, zero_s[0] + 1, main, 0)
    wait(13, out_v)


@jax.jit
def pallas_gated_mix__sliding_local_dilated__glu_gated_reglu__prompt_kernel(
    A_x: jax.Array,
    A_wqkv: jax.Array,
    A_wo: jax.Array,
    B_x: jax.Array,
    B_W_gate: jax.Array,
    B_W_up: jax.Array,
    B_W_down: jax.Array,
    gate_w: jax.Array,
):
    del B_x
    x = A_x.reshape(S, D)
    hbm = pl.BlockSpec(memory_space=pl.ANY)
    out = pl.pallas_call(
        _kernel,
        out_shape=jax.ShapeDtypeStruct((S, D), bf16),
        in_specs=[hbm] * 7,
        out_specs=hbm,
        scratch_shapes=[
            pltpu.VMEM((S, D), bf16),
            pltpu.VMEM((4, D, D), bf16),
            pltpu.VMEM((NF, D, 128), bf16),
            pltpu.VMEM((NF, D, 128), bf16),
            pltpu.VMEM((128 * NFA, D), bf16),
            pltpu.VMEM((NB, F - 128 * NFA, 128), bf16),
            pltpu.VMEM((D,), bf16),
            pltpu.VMEM((4, NB, 8 * PITCH, 128), u32),
            pltpu.VMEM((2, S, D), f32),
            pltpu.VMEM((3 * NB, HALO + TB + 8, 128), f32),
            pltpu.VMEM((NB, TB + 8, 128), f32),
            pltpu.VMEM((S, D), bf16),
            pltpu.SMEM((1,), i32),
            pltpu.SemaphoreType.DMA((14,)),
        ],
        compiler_params=pltpu.CompilerParams(
            vmem_limit_bytes=110 * 1024 * 1024,
            disable_bounds_checks=not CHECKS,
            disable_semaphore_checks=not CHECKS,
        ),
    )(x, A_wqkv, A_wo, B_W_gate, B_W_up, B_W_down, gate_w)
    return out.reshape(1, S, D)
```

```python
import jax
import jax.numpy as jnp
import jax.experimental.pallas as pl
import jax.experimental.pallas.tpu as pltpu

S, D, F = 2048, 1024, 3584
H, DH, WIN, DIL = 32, 32, 8, 2
NB = D // 128
NF = F // 128
HALO = 16
BA = 3
NFA = 2 * BA
R0 = 640
NA = 4
UR = (2 * S - R0) // NA
SUB = (0, (S - R0) % UR, UR)
CPU = 9
NCH = 4 * 8
COFF = NA * CPU - NCH
CH1 = max(CPU - COFF, 1)
PITCH = 65
TB = 256
RG = 8
ANCH = 248
NSK = 4
LGS = 4
PVS = 2
OUTP = ((0, 256, 0, 512), (0, 256, 512, 896), (0, 192, 896, 1024), (192, 256, 896, 1024))
LOG2E = 1.4426950408889634
SCALE = DH ** -0.5 * LOG2E
NEG = -1e9 * LOG2E

f32 = jnp.float32
bf16 = jnp.bfloat16
u32 = jnp.uint32
i32 = jnp.int32


def _dot(a, b):
    return jnp.dot(a, b, preferred_element_type=f32)


def _lane(shape):
    return jax.lax.broadcasted_iota(i32, shape, 1)


def _cat(blocks):
    return jnp.concatenate([pltpu.bitcast(b, bf16) for b in blocks], axis=1)


def _reglu(g, u):
    return jnp.maximum(g, 0.0) * u


def _hcat(hs):
    return jnp.concatenate(hs, axis=1).astype(bf16)


def _kernel(x_hbm, wqkv_hbm, wo_hbm, wg_hbm, wu_hbm, wd_hbm, gw_hbm, out_hbm,
            x_v, w_v, wg_v, wu_v, wda_v, wd_v, gw_v, w_p, bacc,
            qkv_s, o_s, out_v, zero_s, sems):
    def start(src, dst, grp):
        pltpu.make_async_copy(src, dst, sems.at[grp]).start()

    def wait(grp, *dsts):
        for d in dsts:
            pltpu.make_async_copy(d, d, sems.at[grp]).wait()

    def xrows(a, n):
        return x_v.at[pl.ds(a, n), :]

    def get_x(a, n, grp):
        start(x_hbm.at[pl.ds(a, n), :], xrows(a, n), grp)

    def get_cols(hbm, dst, b0, b1, grp):
        for b in range(b0, b1):
            start(hbm.at[:, pl.ds(128 * b, 128)], dst.at[b], grp)

    def wda_rows(b0, b1):
        return wda_v.at[pl.ds(128 * b0, 128 * (b1 - b0)), :]

    def get_wda(b0, b1, grp):
        start(wd_hbm.at[pl.ds(128 * b0, 128 * (b1 - b0)), :], wda_rows(b0, b1), grp)

    def w_rows(c0, c1):
        out = []
        for p in range(4):
            a, b = max(c0, 8 * p), min(c1, 8 * p + 8)
            if a < b:
                out.append((p, 128 * (a - 8 * p), 128 * (b - a)))
        return out

    def w_dst(c0, c1):
        return [w_v.at[p, pl.ds(r, n), :] for p, r, n in w_rows(c0, c1)]

    def get_w(c0, c1, grp):
        for p, r, n in w_rows(c0, c1):
            src = (wqkv_hbm.at[pl.ds(r, n), pl.ds(p * D, D)] if p < 3
                   else wo_hbm.at[pl.ds(r, n), :])
            start(src, w_v.at[p, pl.ds(r, n), :], grp)

    get_x(0, 128, 0)
    get_cols(wg_hbm, wg_v, 0, 1, 0)
    get_x(128, 128, 1)
    get_cols(wu_hbm, wu_v, 0, 1, 2)
    get_x(256, 128, 3)
    get_cols(wg_hbm, wg_v, 1, 2, 4)
    get_x(384, R0 - 384, 5)
    get_cols(wu_hbm, wu_v, 1, 2, 6)
    get_cols(wg_hbm, wg_v, 2, 3, 6)
    get_cols(wu_hbm, wu_v, 2, 3, 6)
    get_wda(0, BA, 7)
    ucross = (S - R0) // UR
    udst = []
    for u in range(3):
        dst = []
        x0, x1 = min(S, R0 + u * UR), (min(S, R0 + (u + 1) * UR) if u < 2 else S)
        if x0 < x1:
            get_x(x0, x1 - x0, 8 + u)
            dst.append(xrows(x0, x1 - x0))
        if u == min(ucross, 2):
            get_cols(wg_hbm, wg_v, BA, NFA, 8 + u)
            get_cols(wu_hbm, wu_v, BA, NFA, 8 + u)
            get_wda(BA, NFA, 8 + u)
            dst += [wg_v.at[pl.ds(BA, BA)], wu_v.at[pl.ds(BA, BA)], wda_rows(BA, NFA)]
        c0, c1 = (0, CH1, 2 * CPU - COFF, NCH)[u:u + 2]
        get_w(c0, c1, 8 + u)
        udst.append(dst + w_dst(c0, c1))
    start(gw_hbm, gw_v, 12)
    for j in range(NB):
        start(wd_hbm.at[pl.ds(128 * NFA, F - 128 * NFA), pl.ds(128 * j, 128)], wd_v.at[j], 12)
    get_cols(wg_hbm, wg_v, NFA, NF, 12)

    wg_u, wu_u, wd_u = (r.bitcast(u32) for r in (wg_v, wu_v, wd_v))

    zero_s[0] = 0
    qkv_s[pl.ds(NB, 2 * NB), pl.ds(0, HALO), :] = jnp.zeros((2 * NB, HALO, 128), f32)

    def repack(ch):
        p = jax.lax.shift_right_logical(ch, 3)
        rc = ch & 7
        on = jnp.where(ch < 24, -1, 0).astype(i32)
        r0 = pl.multiple_of(rc * 128, 128)
        blk = [pltpu.bitcast(w_v[p, pl.ds(r0, 128), pl.ds(128 * j, 128)], u32) for j in range(NB)]
        lane = _lane((64, 128))
        for bb, lb in ((2, 3), (1, 2), (0, 1)):
            sh = 1 << lb
            keep_a = (lane & (on & sh)) == 0
            take_a = ((lane & sh) | (~on & 1)) == 0
            for j in range(NB):
                if j & (1 << bb):
                    continue
                a, b = blk[j], blk[j | (1 << bb)]
                blk[j] = jnp.where(keep_a, a, pltpu.roll(b, sh, 1))
                blk[j | (1 << bb)] = jnp.where(take_a, pltpu.roll(a, 128 - sh, 1), b)
        for j in range(NB):
            w_p[p, j, pl.ds(rc * PITCH, 64), :] = blk[j]

    def main(_, carry0):
        def xr(a, b):
            return x_v[pl.ds(a, b - a), :]

        def rcat(*parts):
            return jnp.concatenate(parts, axis=0)

        wait(0, xrows(0, 128), wg_v.at[0])
        g0a = _dot(xr(0, 128), _cat([wg_u[0]]))
        wait(1, xrows(128, 128))
        g0b = _dot(xr(128, 256), _cat([wg_u[0]]))
        wait(2, wu_v.at[0])
        h0a = _reglu(rcat(g0a, g0b), _dot(xr(0, 256), _cat([wu_u[0]])))
        wait(3, xrows(256, 128))
        gu = _dot(xr(256, 384), _cat([wg_u[0], wu_u[0]]))
        h0b = _reglu(gu[:, :128], gu[:, 128:])
        wait(4, wg_v.at[1])
        g1a = _dot(xr(0, 384), _cat([wg_u[1]]))
        wait(5, xrows(384, R0 - 384))
        gu = _dot(xr(384, R0), _cat([wg_u[0], wu_u[0], wg_u[1]]))
        h0c = _reglu(gu[:, :128], gu[:, 128:256])
        g1 = rcat(g1a, gu[:, 256:])
        wait(6, wu_v.at[pl.ds(1, 2)], wg_v.at[2])
        gu = _dot(xr(0, R0), _cat([wu_u[1], wg_u[2], wu_u[2]]))
        h1 = _reglu(g1, gu[:, :128])
        h2 = _reglu(gu[:, 128:256], gu[:, 256:])
        get_cols(wu_hbm, wu_v, NFA, NF, 12)
        wait(7, wda_rows(0, BA))
        bacc[0, pl.ds(0, R0), :] = _dot(_hcat([rcat(h0a, h0b, h0c), h1, h2]),
                                        wda_v[pl.ds(0, 128 * BA), :])

        def phase_a(u, carry):
            for k in range(3):
                pl.when(u == k)(lambda k=k: wait(8 + k, *udst[k]))
            parts = []
            for v0, v1 in zip(SUB[:-1], SUB[1:]):
                v = u * UR + v0
                c = (v >= S - R0).astype(i32)
                a = pl.multiple_of(v + R0 - c * S, 16)
                x = x_v[pl.ds(a, v1 - v0), :]
                h = _reglu(_dot(x, _cat([wg_u[c * BA + k] for k in range(BA)])),
                           _dot(x, _cat([wu_u[c * BA + k] for k in range(BA)])))
                parts.append((c, a, v1 - v0, h))
            for k in range(CPU):
                repack(jnp.maximum(CPU * u + k - COFF, 0))
            for c, a, n, h in parts:
                r = pl.multiple_of(c * (128 * BA), 128)
                bacc[c, pl.ds(a, n), :] = _dot(_hcat([h]), wda_v[pl.ds(r, 128 * BA), :])
            return carry

        jax.lax.fori_loop(0, NA, phase_a, 0)
        wait(12, gw_v, wg_v.at[pl.ds(NFA, NF - NFA)], wu_v.at[pl.ds(NFA, NF - NFA)], wd_v)

        m16 = (_lane((RG, 128)) & 16) == 0
        m1 = (_lane((RG, 128)) & 1) == 0

        def attend(r0, base, scale, zvec):
            logits = []
            for w in range(WIN):
                if w % LGS == 0:
                    if w:
                        scale = pltpu.bitcast(
                            pltpu.bitcast(scale, i32) | (pltpu.bitcast(raw, i32) & zvec), f32)
                    q = [qkv_s[j, pl.ds(HALO + r0, RG), :] * scale for j in range(NB)]
                off = HALO + r0 - DIL * w
                acc = q[0] * qkv_s[NB, pl.ds(off, RG), :]
                for j in range(1, NB):
                    acc = acc + q[j] * qkv_s[NB + j, pl.ds(off, RG), :]
                raw = acc
                acc = acc + jnp.where(m16, pltpu.roll(acc, 128 - 16, 1), pltpu.roll(acc, 16, 1))
                acc = acc + jnp.where(m1, pltpu.roll(acc, 128 - 1, 1), pltpu.roll(acc, 1, 1))
                if r0 < DIL * w:
                    pos = base + r0 + jax.lax.broadcasted_iota(i32, (RG, 128), 0)
                    acc = jnp.where(pos >= DIL * w, acc, NEG)
                logits.append(acc)
            m = logits[0]
            for w in range(1, WIN):
                m = jnp.maximum(m, logits[w])
            e = [jnp.exp2(l - m) for l in logits]
            s = e[0]
            for w in range(1, WIN):
                s = s + e[w]
            inv = pl.reciprocal(s, approx=True)
            inv = inv * (2.0 - s * inv)
            for j in range(NB):
                if j % PVS == 0:
                    if j:
                        inv = pltpu.bitcast(pltpu.bitcast(inv, i32) | (pltpu.bitcast(o, i32) & zvec), f32)
                    p = [x * inv for x in e]
                o = p[0] * qkv_s[2 * NB + j, pl.ds(HALO + r0, RG), :]
                for w in range(1, WIN):
                    o = o + p[w] * qkv_s[2 * NB + j, pl.ds(HALO + r0 - DIL * w, RG), :]
                o_s[j, pl.ds(r0, RG), :] = o
            return o

        def phase_b(t, carry):
            base = pl.multiple_of(t * TB, TB)
            zero = zero_s[0]
            zvec = jnp.full((RG, 128), zero, i32)
            sbits = pltpu.bitcast(jnp.full((RG, 128), SCALE, f32), i32)
            x = x_v[pl.ds(base, TB), :]
            gw = pltpu.bitcast(jnp.broadcast_to(gw_v[...].astype(f32).reshape(1, D), (8, D)), i32)

            gates = []

            def gate_rows(r0, anchor):
                dep = pltpu.bitcast(anchor, i32) & zvec
                xr = x[r0:r0 + 16, :].astype(f32)
                acc = None
                for j in range(NB):
                    w = pltpu.bitcast(gw[:, 128 * j:128 * (j + 1)] | dep, f32)
                    term = xr[:, 128 * j:128 * (j + 1)] * jnp.concatenate([w, w], axis=0)
                    acc = term if acc is None else acc + term
                z = jnp.sum(acc, axis=-1, keepdims=True)
                gates.append(jnp.broadcast_to(jax.nn.sigmoid(z), (16, 128)))

            for i in range(3):
                r = _dot(x, _cat([jnp.concatenate([w_p[i, j, pl.ds(PITCH * c, 64), :] for c in range(8)],
                                                  axis=0) for j in range(NB)]))
                for j in range(NB):
                    qkv_s[i * NB + j, pl.ds(HALO, TB), :] = r[:, 128 * j:128 * (j + 1)]
                    if i * NB + j < TB // 16:
                        gate_rows(16 * (i * NB + j), r[ANCH:ANCH + 8, 128 * j:128 * (j + 1)])
            groups = list(range(0, TB, RG))
            nslots = 2 * (NF - NFA) - NSK
            hs = []
            slot = 0
            done = 0
            last = []

            def release(anchor):
                nonlocal slot, done
                slot += 1
                want = min(len(groups), -(-slot * len(groups) // nslots))
                if want > done:
                    for r0 in groups[done:want]:
                        dep = pltpu.bitcast(anchor, i32)
                        dep = dep | pltpu.bitcast(gates[r0 // 16][r0 % 16:r0 % 16 + 8], i32)
                        if last:
                            dep = dep | pltpu.bitcast(last[-1], i32)
                        last.append(attend(r0, base, pltpu.bitcast(sbits | (dep & zvec), f32), zvec))
                    done = want

            for c in range(NFA, NF, 2):
                g = _dot(x, _cat([wg_u[c], wg_u[c + 1]]))
                for n in range(2):
                    release(g[ANCH:ANCH + 8, 128 * n:128 * (n + 1)])
                u = _dot(x, _cat([wu_u[c], wu_u[c + 1]]))
                for n in range(2):
                    release(u[ANCH:ANCH + 8, 128 * n:128 * (n + 1)])
                hs.append(_reglu(g, u))
            assert done == len(groups)
            qkv_s[pl.ds(NB, 2 * NB), pl.ds(0, HALO), :] = qkv_s[pl.ds(NB, 2 * NB), pl.ds(TB, HALO), :]
            g = jnp.concatenate(gates, axis=0)
            g1 = 1.0 - g

            wo = _cat([jnp.concatenate([w_p[3, j, pl.ds(8 * m + c, 8, stride=PITCH), :]
                                        for c in range(8) for m in range(8)], axis=0)
                       for j in range(NB)])
            o_s[0, pl.ds(TB + zero, 8), :] = jnp.zeros((8, 128), f32)
            o = jnp.concatenate([o_s[j, pl.ds(0, TB), :] for j in range(NB)], axis=1)
            a = _dot(o.astype(bf16), wo)
            b = (bacc[0, pl.ds(base, TB), :] + bacc[1, pl.ds(base, TB), :]
                 + _dot(_hcat(hs), _cat([wd_u[j] for j in range(NB)])))
            for r0, r1, c0, c1 in OUTP:
                n = c1 - c0
                res = (jnp.concatenate([g[r0:r1]] * (n // 128), axis=1) * a[r0:r1, c0:c1]
                       + jnp.concatenate([g1[r0:r1]] * (n // 128), axis=1) * b[r0:r1, c0:c1])
                rs = pl.ds(pl.multiple_of(base + r0, 16), r1 - r0)
                out_v[rs, pl.ds(c0, n)] = res.astype(bf16)
                start(out_v.at[rs, pl.ds(c0, n)], out_hbm.at[rs, pl.ds(c0, n)], 13)
            return carry

        jax.lax.fori_loop(0, S // TB, phase_b, 0)
        return carry0

    jax.lax.fori_loop(0, zero_s[0] + 1, main, 0)
    wait(13, out_v)


@jax.jit
def pallas_gated_mix__sliding_local_dilated__glu_gated_reglu__prompt_kernel(
    A_x: jax.Array,
    A_wqkv: jax.Array,
    A_wo: jax.Array,
    B_x: jax.Array,
    B_W_gate: jax.Array,
    B_W_up: jax.Array,
    B_W_down: jax.Array,
    gate_w: jax.Array,
):
    del B_x
    x = A_x.reshape(S, D)
    hbm = pl.BlockSpec(memory_space=pl.ANY)
    out = pl.pallas_call(
        _kernel,
        out_shape=jax.ShapeDtypeStruct((S, D), bf16),
        in_specs=[hbm] * 7,
        out_specs=hbm,
        scratch_shapes=[
            pltpu.VMEM((S, D), bf16),
            pltpu.VMEM((4, D, D), bf16),
            pltpu.VMEM((NF, D, 128), bf16),
            pltpu.VMEM((NF, D, 128), bf16),
            pltpu.VMEM((128 * NFA, D), bf16),
            pltpu.VMEM((NB, F - 128 * NFA, 128), bf16),
            pltpu.VMEM((D,), bf16),
            pltpu.VMEM((4, NB, 8 * PITCH, 128), u32),
            pltpu.VMEM((2, S, D), f32),
            pltpu.VMEM((3 * NB, HALO + TB + 8, 128), f32),
            pltpu.VMEM((NB, TB + 8, 128), f32),
            pltpu.VMEM((S, D), bf16),
            pltpu.SMEM((1,), i32),
            pltpu.SemaphoreType.DMA((14,)),
        ],
        compiler_params=pltpu.CompilerParams(
            vmem_limit_bytes=110 * 1024 * 1024,
            disable_bounds_checks=True,
            disable_semaphore_checks=True,
        ),
    )(x, A_wqkv, A_wo, B_W_gate, B_W_up, B_W_down, gate_w)
    return out.reshape(1, S, D)
```

```python
import jax
import jax.numpy as jnp
import jax.experimental.pallas as pl
import jax.experimental.pallas.tpu as pltpu

S, D, F = 2048, 1024, 3584
H, DH, WIN, DIL = 32, 32, 8, 2
NB = D // 128
NF = F // 128
HALO = 16
BA = 3
NFA = 2 * BA
FB = F - 128 * NFA
R0 = 640
NA = 4
UR = (2 * S - R0) // NA
SUB = (0, (S - R0) % UR, UR)
CPU = 9
NCH = 4 * 8
COFF = NA * CPU - NCH
CH1 = max(CPU - COFF, 1)
PITCH = 65
TB = 256
RG = 8
ANCH = 248
NSK = 4
LGS = 4
PVS = 2
OUTP = ((0, 256, 0, 512), (0, 256, 512, 896), (0, 192, 896, 1024), (192, 256, 896, 1024))
LOG2E = 1.4426950408889634
SCALE = DH ** -0.5 * LOG2E
NEG = -1e9 * LOG2E

f32 = jnp.float32
bf16 = jnp.bfloat16
u32 = jnp.uint32
i32 = jnp.int32


def _dot(a, b):
    return jnp.dot(a, b, preferred_element_type=f32)


def _lane(shape):
    return jax.lax.broadcasted_iota(i32, shape, 1)


def _cat(blocks):
    return jnp.concatenate([pltpu.bitcast(b, bf16) for b in blocks], axis=1)


def _reglu(g, u):
    return jnp.maximum(g, 0.0) * u


def _hcat(hs):
    return jnp.concatenate(hs, axis=1).astype(bf16)


def _kernel(x_hbm, wqkv_hbm, wo_hbm, wg_hbm, wu_hbm, wd_hbm, gw_hbm, out_hbm,
            x_v, w_v, wga_v, wua_v, wda_v, wg_v, wu_v, wd_v, gw_v, w_p, bacc,
            qkv_s, o_s, out_v, zero_s, sems):
    def start(src, dst, grp):
        pltpu.make_async_copy(src, dst, sems.at[grp]).start()

    def wait(grp, *dsts):
        for d in dsts:
            pltpu.make_async_copy(d, d, sems.at[grp]).wait()

    def xrows(a, n):
        return x_v.at[pl.ds(a, n), :]

    def get_x(a, n, grp):
        start(x_hbm.at[pl.ds(a, n), :], xrows(a, n), grp)

    def acols(ref, b0, b1):
        c = b0 // BA
        return ref.at[c, :, pl.ds(128 * (b0 - c * BA), 128 * (b1 - b0))]

    def get_cols(hbm, dst, b0, b1, grp):
        start(hbm.at[:, pl.ds(128 * b0, 128 * (b1 - b0))], acols(dst, b0, b1), grp)

    def wda_rows(b0, b1):
        return wda_v.at[pl.ds(128 * b0, 128 * (b1 - b0)), :]

    def get_wda(b0, b1, grp):
        start(wd_hbm.at[pl.ds(128 * b0, 128 * (b1 - b0)), :], wda_rows(b0, b1), grp)

    def w_rows(c0, c1):
        out = []
        for p in range(4):
            a, b = max(c0, 8 * p), min(c1, 8 * p + 8)
            if a < b:
                out.append((p, 128 * (a - 8 * p), 128 * (b - a)))
        return out

    def w_dst(c0, c1):
        return [w_v.at[p, pl.ds(r, n), :] for p, r, n in w_rows(c0, c1)]

    def get_w(c0, c1, grp):
        for p, r, n in w_rows(c0, c1):
            src = (wqkv_hbm.at[pl.ds(r, n), pl.ds(p * D, D)] if p < 3
                   else wo_hbm.at[pl.ds(r, n), :])
            start(src, w_v.at[p, pl.ds(r, n), :], grp)

    get_x(0, 128, 0)
    get_cols(wg_hbm, wga_v, 0, 1, 0)
    get_x(128, 128, 1)
    get_cols(wu_hbm, wua_v, 0, 1, 2)
    get_x(256, 128, 3)
    get_cols(wg_hbm, wga_v, 1, 2, 4)
    get_x(384, R0 - 384, 5)
    get_cols(wu_hbm, wua_v, 1, 3, 6)
    get_cols(wg_hbm, wga_v, 2, 3, 6)
    get_wda(0, BA, 7)
    ucross = (S - R0) // UR
    udst = []
    for u in range(3):
        dst = []
        x0, x1 = min(S, R0 + u * UR), (min(S, R0 + (u + 1) * UR) if u < 2 else S)
        if x0 < x1:
            get_x(x0, x1 - x0, 8 + u)
            dst.append(xrows(x0, x1 - x0))
        if u == min(ucross, 2):
            get_cols(wg_hbm, wga_v, BA, NFA, 8 + u)
            get_cols(wu_hbm, wua_v, BA, NFA, 8 + u)
            get_wda(BA, NFA, 8 + u)
            dst += [wga_v.at[1], wua_v.at[1], wda_rows(BA, NFA)]
        c0, c1 = (0, CH1, 2 * CPU - COFF, NCH)[u:u + 2]
        get_w(c0, c1, 8 + u)
        udst.append(dst + w_dst(c0, c1))
    start(gw_hbm, gw_v, 12)
    start(wd_hbm.at[pl.ds(128 * NFA, FB), :], wd_v, 12)
    start(wg_hbm.at[:, pl.ds(128 * NFA, FB)], wg_v, 12)
    start(wu_hbm.at[:, pl.ds(128 * NFA, FB)], wu_v, 12)


    zero_s[0] = 0
    qkv_s[pl.ds(NB, 2 * NB), pl.ds(0, HALO), :] = jnp.zeros((2 * NB, HALO, 128), f32)

    def repack(ch):
        p = jax.lax.shift_right_logical(ch, 3)
        rc = ch & 7
        on = jnp.where(ch < 24, -1, 0).astype(i32)
        r0 = pl.multiple_of(rc * 128, 128)
        blk = [pltpu.bitcast(w_v[p, pl.ds(r0, 128), pl.ds(128 * j, 128)], u32) for j in range(NB)]
        lane = _lane((64, 128))
        for bb, lb in ((2, 3), (1, 2), (0, 1)):
            sh = 1 << lb
            keep_a = (lane & (on & sh)) == 0
            take_a = ((lane & sh) | (~on & 1)) == 0
            for j in range(NB):
                if j & (1 << bb):
                    continue
                a, b = blk[j], blk[j | (1 << bb)]
                blk[j] = jnp.where(keep_a, a, pltpu.roll(b, sh, 1))
                blk[j | (1 << bb)] = jnp.where(take_a, pltpu.roll(a, 128 - sh, 1), b)
        for j in range(NB):
            w_p[p, j, pl.ds(rc * PITCH, 64), :] = blk[j]

    def main(_, carry0):
        def xr(a, b):
            return x_v[pl.ds(a, b - a), :]

        def wg(b):
            return wga_v[0, :, pl.ds(128 * b, 128)]

        def wu(b):
            return wua_v[0, :, pl.ds(128 * b, 128)]

        def rcat(*parts):
            return jnp.concatenate(parts, axis=0)

        def ccat(*parts):
            return jnp.concatenate(parts, axis=1)

        wait(0, xrows(0, 128), acols(wga_v, 0, 1))
        g0a = _dot(xr(0, 128), wg(0))
        wait(1, xrows(128, 128))
        g0b = _dot(xr(128, 256), wg(0))
        wait(2, acols(wua_v, 0, 1))
        h0a = _reglu(rcat(g0a, g0b), _dot(xr(0, 256), wu(0)))
        wait(3, xrows(256, 128))
        gu = _dot(xr(256, 384), ccat(wg(0), wu(0)))
        h0b = _reglu(gu[:, :128], gu[:, 128:])
        wait(4, acols(wga_v, 1, 2))
        g1a = _dot(xr(0, 384), wg(1))
        wait(5, xrows(384, R0 - 384))
        gu = _dot(xr(384, R0), ccat(wg(0), wu(0), wg(1)))
        h0c = _reglu(gu[:, :128], gu[:, 128:256])
        g1 = rcat(g1a, gu[:, 256:])
        wait(6, acols(wua_v, 1, 3), acols(wga_v, 2, 3))
        gu = _dot(xr(0, R0), ccat(wu(1), wg(2), wu(2)))
        h1 = _reglu(g1, gu[:, :128])
        h2 = _reglu(gu[:, 128:256], gu[:, 256:])
        wait(7, wda_rows(0, BA))
        bacc[0, pl.ds(0, R0), :] = _dot(_hcat([rcat(h0a, h0b, h0c), h1, h2]),
                                        wda_v[pl.ds(0, 128 * BA), :])

        def phase_a(u, carry):
            for k in range(3):
                pl.when(u == k)(lambda k=k: wait(8 + k, *udst[k]))
            parts = []
            for v0, v1 in zip(SUB[:-1], SUB[1:]):
                v = u * UR + v0
                c = (v >= S - R0).astype(i32)
                a = pl.multiple_of(v + R0 - c * S, 16)
                x = x_v[pl.ds(a, v1 - v0), :]
                h = _reglu(_dot(x, wga_v[c]), _dot(x, wua_v[c]))
                parts.append((c, a, v1 - v0, h))
            for k in range(CPU):
                repack(jnp.maximum(CPU * u + k - COFF, 0))
            for c, a, n, h in parts:
                r = pl.multiple_of(c * (128 * BA), 128)
                bacc[c, pl.ds(a, n), :] = _dot(_hcat([h]), wda_v[pl.ds(r, 128 * BA), :])
            return carry

        jax.lax.fori_loop(0, NA, phase_a, 0)
        wait(12, gw_v, wg_v, wu_v, wd_v)

        m16 = (_lane((RG, 128)) & 16) == 0
        m1 = (_lane((RG, 128)) & 1) == 0

        def attend(r0, base, scale, zvec):
            logits = []
            for w in range(WIN):
                if w % LGS == 0:
                    if w:
                        scale = pltpu.bitcast(
                            pltpu.bitcast(scale, i32) | (pltpu.bitcast(raw, i32) & zvec), f32)
                    q = [qkv_s[j, pl.ds(HALO + r0, RG), :] * scale for j in range(NB)]
                off = HALO + r0 - DIL * w
                acc = q[0] * qkv_s[NB, pl.ds(off, RG), :]
                for j in range(1, NB):
                    acc = acc + q[j] * qkv_s[NB + j, pl.ds(off, RG), :]
                raw = acc
                acc = acc + jnp.where(m16, pltpu.roll(acc, 128 - 16, 1), pltpu.roll(acc, 16, 1))
                acc = acc + jnp.where(m1, pltpu.roll(acc, 128 - 1, 1), pltpu.roll(acc, 1, 1))
                if r0 < DIL * w:
                    pos = base + r0 + jax.lax.broadcasted_iota(i32, (RG, 128), 0)
                    acc = jnp.where(pos >= DIL * w, acc, NEG)
                logits.append(acc)
            m = logits[0]
            for w in range(1, WIN):
                m = jnp.maximum(m, logits[w])
            e = [jnp.exp2(l - m) for l in logits]
            s = e[0]
            for w in range(1, WIN):
                s = s + e[w]
            inv = pl.reciprocal(s, approx=True)
            inv = inv * (2.0 - s * inv)
            for j in range(NB):
                if j % PVS == 0:
                    if j:
                        inv = pltpu.bitcast(pltpu.bitcast(inv, i32) | (pltpu.bitcast(o, i32) & zvec), f32)
                    p = [x * inv for x in e]
                o = p[0] * qkv_s[2 * NB + j, pl.ds(HALO + r0, RG), :]
                for w in range(1, WIN):
                    o = o + p[w] * qkv_s[2 * NB + j, pl.ds(HALO + r0 - DIL * w, RG), :]
                o_s[j, pl.ds(r0, RG), :] = o
            return o

        def phase_b(t, carry):
            base = pl.multiple_of(t * TB, TB)
            zero = zero_s[0]
            zvec = jnp.full((RG, 128), zero, i32)
            sbits = pltpu.bitcast(jnp.full((RG, 128), SCALE, f32), i32)
            x = x_v[pl.ds(base, TB), :]
            gw = pltpu.bitcast(jnp.broadcast_to(gw_v[...].astype(f32).reshape(1, D), (8, D)), i32)

            gates = []

            def gate_rows(r0, anchor):
                dep = pltpu.bitcast(anchor, i32) & zvec
                xr = x[r0:r0 + 16, :].astype(f32)
                acc = None
                for j in range(NB):
                    w = pltpu.bitcast(gw[:, 128 * j:128 * (j + 1)] | dep, f32)
                    term = xr[:, 128 * j:128 * (j + 1)] * jnp.concatenate([w, w], axis=0)
                    acc = term if acc is None else acc + term
                z = jnp.sum(acc, axis=-1, keepdims=True)
                gates.append(jnp.broadcast_to(jax.nn.sigmoid(z), (16, 128)))

            for i in range(3):
                r = _dot(x, _cat([jnp.concatenate([w_p[i, j, pl.ds(PITCH * c, 64), :] for c in range(8)],
                                                  axis=0) for j in range(NB)]))
                for j in range(NB):
                    qkv_s[i * NB + j, pl.ds(HALO, TB), :] = r[:, 128 * j:128 * (j + 1)]
                    if i * NB + j < TB // 16:
                        gate_rows(16 * (i * NB + j), r[ANCH:ANCH + 8, 128 * j:128 * (j + 1)])
            groups = list(range(0, TB, RG))
            nslots = 2 * (NF - NFA) - NSK
            hs = []
            slot = 0
            done = 0
            last = []

            def release(anchor):
                nonlocal slot, done
                slot += 1
                want = min(len(groups), -(-slot * len(groups) // nslots))
                if want > done:
                    for r0 in groups[done:want]:
                        dep = pltpu.bitcast(anchor, i32)
                        dep = dep | pltpu.bitcast(gates[r0 // 16][r0 % 16:r0 % 16 + 8], i32)
                        if last:
                            dep = dep | pltpu.bitcast(last[-1], i32)
                        last.append(attend(r0, base, pltpu.bitcast(sbits | (dep & zvec), f32), zvec))
                    done = want

            for c in range(0, FB, 256):
                g = _dot(x, wg_v[:, pl.ds(c, 256)])
                for n in range(2):
                    release(g[ANCH:ANCH + 8, 128 * n:128 * (n + 1)])
                u = _dot(x, wu_v[:, pl.ds(c, 256)])
                for n in range(2):
                    release(u[ANCH:ANCH + 8, 128 * n:128 * (n + 1)])
                hs.append(_reglu(g, u))
            assert done == len(groups)
            qkv_s[pl.ds(NB, 2 * NB), pl.ds(0, HALO), :] = qkv_s[pl.ds(NB, 2 * NB), pl.ds(TB, HALO), :]
            g = jnp.concatenate(gates, axis=0)
            g1 = 1.0 - g

            wo = _cat([jnp.concatenate([w_p[3, j, pl.ds(8 * m + c, 8, stride=PITCH), :]
                                        for c in range(8) for m in range(8)], axis=0)
                       for j in range(NB)])
            o_s[0, pl.ds(TB + zero, 8), :] = jnp.zeros((8, 128), f32)
            o = jnp.concatenate([o_s[j, pl.ds(0, TB), :] for j in range(NB)], axis=1)
            a = _dot(o.astype(bf16), wo)
            b = (bacc[0, pl.ds(base, TB), :] + bacc[1, pl.ds(base, TB), :]
                 + _dot(_hcat(hs), wd_v[...]))
            for r0, r1, c0, c1 in OUTP:
                n = c1 - c0
                res = (jnp.concatenate([g[r0:r1]] * (n // 128), axis=1) * a[r0:r1, c0:c1]
                       + jnp.concatenate([g1[r0:r1]] * (n // 128), axis=1) * b[r0:r1, c0:c1])
                rs = pl.ds(pl.multiple_of(base + r0, 16), r1 - r0)
                out_v[rs, pl.ds(c0, n)] = res.astype(bf16)
                start(out_v.at[rs, pl.ds(c0, n)], out_hbm.at[rs, pl.ds(c0, n)], 13)
            return carry

        jax.lax.fori_loop(0, S // TB, phase_b, 0)
        return carry0

    jax.lax.fori_loop(0, zero_s[0] + 1, main, 0)
    wait(13, out_v)


@jax.jit
def pallas_gated_mix__sliding_local_dilated__glu_gated_reglu__prompt_kernel(
    A_x: jax.Array,
    A_wqkv: jax.Array,
    A_wo: jax.Array,
    B_x: jax.Array,
    B_W_gate: jax.Array,
    B_W_up: jax.Array,
    B_W_down: jax.Array,
    gate_w: jax.Array,
):
    del B_x
    x = A_x.reshape(S, D)
    hbm = pl.BlockSpec(memory_space=pl.ANY)
    out = pl.pallas_call(
        _kernel,
        out_shape=jax.ShapeDtypeStruct((S, D), bf16),
        in_specs=[hbm] * 7,
        out_specs=hbm,
        scratch_shapes=[
            pltpu.VMEM((S, D), bf16),
            pltpu.VMEM((4, D, D), bf16),
            pltpu.VMEM((2, D, 128 * BA), bf16),
            pltpu.VMEM((2, D, 128 * BA), bf16),
            pltpu.VMEM((128 * NFA, D), bf16),
            pltpu.VMEM((D, FB), bf16),
            pltpu.VMEM((D, FB), bf16),
            pltpu.VMEM((FB, D), bf16),
            pltpu.VMEM((D,), bf16),
            pltpu.VMEM((4, NB, 8 * PITCH, 128), u32),
            pltpu.VMEM((2, S, D), f32),
            pltpu.VMEM((3 * NB, HALO + TB + 8, 128), f32),
            pltpu.VMEM((NB, TB + 8, 128), f32),
            pltpu.VMEM((S, D), bf16),
            pltpu.SMEM((1,), i32),
            pltpu.SemaphoreType.DMA((14,)),
        ],
        compiler_params=pltpu.CompilerParams(
            vmem_limit_bytes=110 * 1024 * 1024,
            disable_bounds_checks=True,
            disable_semaphore_checks=True,
        ),
    )(x, A_wqkv, A_wo, B_W_gate, B_W_up, B_W_down, gate_w)
    return out.reshape(1, S, D)
```

```python
import jax
import jax.numpy as jnp
import jax.experimental.pallas as pl
import jax.experimental.pallas.tpu as pltpu

S, D, F = 2048, 1024, 3584
H, DH, WIN, DIL = 32, 32, 8, 2
NB = D // 128
NF = F // 128
HALO = 16
BA = 3
NFA = 2 * BA
FB = F - 128 * NFA
R0 = 704
NA = 4
UR = (2 * S - R0) // NA
SUB = (0, (S - R0) % UR, UR)
CPU = 9
NCH = 4 * 8
COFF = NA * CPU - NCH
CH1 = max(CPU - COFF, 1)
KS = (0, 256, 512, 768, 1024)
X1 = 256
PITCH = 65
TB = 256
RG = 8
ANCH = 56
NSK = 4
LGS = 4
PVS = 2
OUTP = ((0, 256, 0, 512), (0, 256, 512, 896), (0, 192, 896, 1024), (192, 256, 896, 1024))
LOG2E = 1.4426950408889634
SCALE = DH ** -0.5 * LOG2E
NEG = -1e9 * LOG2E

f32 = jnp.float32
bf16 = jnp.bfloat16
u32 = jnp.uint32
i32 = jnp.int32


def _dot(a, b):
    return jnp.dot(a, b, preferred_element_type=f32)


def _lane(shape):
    return jax.lax.broadcasted_iota(i32, shape, 1)


def _cat(blocks):
    return jnp.concatenate([pltpu.bitcast(b, bf16) for b in blocks], axis=1)


def _reglu(g, u):
    return jnp.maximum(g, 0.0) * u


def _hcat(hs):
    return jnp.concatenate(hs, axis=1).astype(bf16)


def _kernel(x_hbm, wqkv_hbm, wo_hbm, wg_hbm, wu_hbm, wd_hbm, gw_hbm, out_hbm,
            x_v, w_v, wga_v, wua_v, wda_v, wg_v, wu_v, wd_v, gw_v, w_p, bacc,
            qkv_s, o_s, out_v, zero_s, sems):
    def start(src, dst, grp):
        pltpu.make_async_copy(src, dst, sems.at[grp]).start()

    def wait(grp, *dsts):
        for d in dsts:
            pltpu.make_async_copy(d, d, sems.at[grp]).wait()

    def xrows(a, n):
        return x_v.at[pl.ds(a, n), :]

    def get_x(a, n, grp):
        start(x_hbm.at[pl.ds(a, n), :], xrows(a, n), grp)

    def wda_rows(b0, b1):
        return wda_v.at[pl.ds(128 * b0, 128 * (b1 - b0)), :]

    def get_wda(b0, b1, grp):
        start(wd_hbm.at[pl.ds(128 * b0, 128 * (b1 - b0)), :], wda_rows(b0, b1), grp)

    def w_rows(c0, c1):
        out = []
        for p in range(4):
            a, b = max(c0, 8 * p), min(c1, 8 * p + 8)
            if a < b:
                out.append((p, 128 * (a - 8 * p), 128 * (b - a)))
        return out

    def w_dst(c0, c1):
        return [w_v.at[p, pl.ds(r, n), :] for p, r, n in w_rows(c0, c1)]

    def get_w(c0, c1, grp):
        for p, r, n in w_rows(c0, c1):
            src = (wqkv_hbm.at[pl.ds(r, n), pl.ds(p * D, D)] if p < 3
                   else wo_hbm.at[pl.ds(r, n), :])
            start(src, w_v.at[p, pl.ds(r, n), :], grp)

    def xpart(r0, r1, k):
        sl = (pl.ds(r0, r1 - r0), pl.ds(KS[k], KS[k + 1] - KS[k]))
        return x_hbm.at[sl], x_v.at[sl]

    def wpart(hbm, buf, k, b0=0, b1=BA):
        sl = (pl.ds(KS[k], KS[k + 1] - KS[k]), pl.ds(128 * b0, 128 * (b1 - b0)))
        return hbm.at[sl], buf.at[(0,) + sl]

    p0 = [[xpart(0, X1, 0), wpart(wg_hbm, wga_v, 0, 0, 2)], [xpart(X1, R0, 0)],
          [wpart(wg_hbm, wga_v, 0, 2, BA), wpart(wu_hbm, wua_v, 0)]]
    for k in range(1, len(KS) - 1):
        p0.append([xpart(0, R0, k), wpart(wg_hbm, wga_v, k), wpart(wu_hbm, wua_v, k)])
    p0[-1].append((wd_hbm.at[pl.ds(0, 128 * BA), :], wda_rows(0, BA)))
    for grp, pieces in enumerate(p0):
        for src, dst in pieces:
            start(src, dst, grp)
    ucross = (S - R0) // UR
    udst = []
    for u in range(3):
        dst = []
        x0, x1 = min(S, R0 + u * UR), (min(S, R0 + (u + 1) * UR) if u < 2 else S)
        if x0 < x1:
            get_x(x0, x1 - x0, 6 + u)
            dst.append(xrows(x0, x1 - x0))
        if u == min(ucross, 2):
            start(wg_hbm.at[:, pl.ds(128 * BA, 128 * BA)], wga_v.at[1], 6 + u)
            start(wu_hbm.at[:, pl.ds(128 * BA, 128 * BA)], wua_v.at[1], 6 + u)
            get_wda(BA, NFA, 6 + u)
            dst += [wga_v.at[1], wua_v.at[1], wda_rows(BA, NFA)]
        c0, c1 = (0, CH1, 2 * CPU - COFF, NCH)[u:u + 2]
        get_w(c0, c1, 6 + u)
        udst.append(dst + w_dst(c0, c1))
    start(gw_hbm, gw_v, 9)
    start(wd_hbm.at[pl.ds(128 * NFA, FB), :], wd_v, 9)
    start(wg_hbm.at[:, pl.ds(128 * NFA, FB)], wg_v, 9)
    start(wu_hbm.at[:, pl.ds(128 * NFA, FB)], wu_v, 9)


    zero_s[0] = 0
    qkv_s[pl.ds(NB, 2 * NB), pl.ds(0, HALO), :] = jnp.zeros((2 * NB, HALO, 128), f32)

    def repack(ch):
        p = jax.lax.shift_right_logical(ch, 3)
        rc = ch & 7
        on = jnp.where(ch < 24, -1, 0).astype(i32)
        r0 = pl.multiple_of(rc * 128, 128)
        blk = [pltpu.bitcast(w_v[p, pl.ds(r0, 128), pl.ds(128 * j, 128)], u32) for j in range(NB)]
        lane = _lane((64, 128))
        for bb, lb in ((2, 3), (1, 2), (0, 1)):
            sh = 1 << lb
            keep_a = (lane & (on & sh)) == 0
            take_a = ((lane & sh) | (~on & 1)) == 0
            for j in range(NB):
                if j & (1 << bb):
                    continue
                a, b = blk[j], blk[j | (1 << bb)]
                blk[j] = jnp.where(keep_a, a, pltpu.roll(b, sh, 1))
                blk[j | (1 << bb)] = jnp.where(take_a, pltpu.roll(a, 128 - sh, 1), b)
        for j in range(NB):
            w_p[p, j, pl.ds(rc * PITCH, 64), :] = blk[j]

    def main(_, carry0):
        def wait0(grp):
            wait(grp, *[dst for _, dst in p0[grp]])

        def xk(r0, r1, k):
            return x_v[pl.ds(r0, r1 - r0), pl.ds(KS[k], KS[k + 1] - KS[k])]

        def wk(buf, k, b0=0, b1=BA):
            return buf[0, pl.ds(KS[k], KS[k + 1] - KS[k]), pl.ds(128 * b0, 128 * (b1 - b0))]

        wait0(0)
        ga = _dot(xk(0, X1, 0), wk(wga_v, 0, 0, 2))
        wait0(1)
        gb = _dot(xk(X1, R0, 0), wk(wga_v, 0, 0, 2))
        wait0(2)
        gc = _dot(xk(0, R0, 0), jnp.concatenate([wk(wga_v, 0, 2, BA), wk(wua_v, 0)], axis=1))
        gu = jnp.concatenate([jnp.concatenate([ga, gb], axis=0), gc], axis=1)
        for k in range(1, len(KS) - 1):
            wait0(2 + k)
            d = _dot(xk(0, R0, k), jnp.concatenate([wk(wga_v, k), wk(wua_v, k)], axis=1))
            gu = jnp.concatenate([gu[:, :128 * BA] + d[:, :128 * BA],
                                  gu[:, 128 * BA:] + d[:, 128 * BA:]], axis=1)
        g, up = gu[:, :128 * BA], gu[:, 128 * BA:]
        bacc[0, pl.ds(0, R0), :] = _dot(_hcat([_reglu(g, up)]), wda_v[pl.ds(0, 128 * BA), :])

        def phase_a(u, carry):
            for k in range(3):
                pl.when(u == k)(lambda k=k: wait(6 + k, *udst[k]))
            parts = []
            for v0, v1 in zip(SUB[:-1], SUB[1:]):
                v = u * UR + v0
                c = (v >= S - R0).astype(i32)
                a = pl.multiple_of(v + R0 - c * S, 16)
                x = x_v[pl.ds(a, v1 - v0), :]
                h = _reglu(_dot(x, wga_v[c]), _dot(x, wua_v[c]))
                parts.append((c, a, v1 - v0, h))
            for k in range(CPU):
                repack(jnp.maximum(CPU * u + k - COFF, 0))
            for c, a, n, h in parts:
                r = pl.multiple_of(c * (128 * BA), 128)
                bacc[c, pl.ds(a, n), :] = _dot(_hcat([h]), wda_v[pl.ds(r, 128 * BA), :])
            return carry

        jax.lax.fori_loop(0, NA, phase_a, 0)
        wait(9, gw_v, wg_v, wu_v, wd_v)

        m16 = (_lane((RG, 128)) & 16) == 0
        m1 = (_lane((RG, 128)) & 1) == 0

        def attend(r0, base, scale, zvec):
            logits = []
            for w in range(WIN):
                if w % LGS == 0:
                    if w:
                        scale = pltpu.bitcast(
                            pltpu.bitcast(scale, i32) | (pltpu.bitcast(raw, i32) & zvec), f32)
                    q = [qkv_s[j, pl.ds(HALO + r0, RG), :] * scale for j in range(NB)]
                off = HALO + r0 - DIL * w
                acc = q[0] * qkv_s[NB, pl.ds(off, RG), :]
                for j in range(1, NB):
                    acc = acc + q[j] * qkv_s[NB + j, pl.ds(off, RG), :]
                raw = acc
                acc = acc + jnp.where(m16, pltpu.roll(acc, 128 - 16, 1), pltpu.roll(acc, 16, 1))
                acc = acc + jnp.where(m1, pltpu.roll(acc, 128 - 1, 1), pltpu.roll(acc, 1, 1))
                if r0 < DIL * w:
                    pos = base + r0 + jax.lax.broadcasted_iota(i32, (RG, 128), 0)
                    acc = jnp.where(pos >= DIL * w, acc, NEG)
                logits.append(acc)
            m = logits[0]
            for w in range(1, WIN):
                m = jnp.maximum(m, logits[w])
            e = [jnp.exp2(l - m) for l in logits]
            s = e[0]
            for w in range(1, WIN):
                s = s + e[w]
            inv = pl.reciprocal(s, approx=True)
            inv = inv * (2.0 - s * inv)
            for j in range(NB):
                if j % PVS == 0:
                    if j:
                        inv = pltpu.bitcast(pltpu.bitcast(inv, i32) | (pltpu.bitcast(o, i32) & zvec), f32)
                    p = [x * inv for x in e]
                o = p[0] * qkv_s[2 * NB + j, pl.ds(HALO + r0, RG), :]
                for w in range(1, WIN):
                    o = o + p[w] * qkv_s[2 * NB + j, pl.ds(HALO + r0 - DIL * w, RG), :]
                o_s[j, pl.ds(r0, RG), :] = o
            return o

        def phase_b(t, carry):
            base = pl.multiple_of(t * TB, TB)
            zero = zero_s[0]
            zvec = jnp.full((RG, 128), zero, i32)
            sbits = pltpu.bitcast(jnp.full((RG, 128), SCALE, f32), i32)
            x = x_v[pl.ds(base, TB), :]
            gw = pltpu.bitcast(jnp.broadcast_to(gw_v[...].astype(f32).reshape(1, D), (8, D)), i32)

            gates = []

            def gate_rows(r0, anchor):
                dep = pltpu.bitcast(anchor, i32) & zvec
                xr = x[r0:r0 + 16, :].astype(f32)
                acc = None
                for j in range(NB):
                    w = pltpu.bitcast(gw[:, 128 * j:128 * (j + 1)] | dep, f32)
                    term = xr[:, 128 * j:128 * (j + 1)] * jnp.concatenate([w, w], axis=0)
                    acc = term if acc is None else acc + term
                z = jnp.sum(acc, axis=-1, keepdims=True)
                gates.append(jnp.broadcast_to(jax.nn.sigmoid(z), (16, 128)))

            for i in range(3):
                r = _dot(x, _cat([jnp.concatenate([w_p[i, j, pl.ds(PITCH * c, 64), :] for c in range(8)],
                                                  axis=0) for j in range(NB)]))
                for j in range(NB):
                    qkv_s[i * NB + j, pl.ds(HALO, TB), :] = r[:, 128 * j:128 * (j + 1)]
                    if i * NB + j < TB // 16:
                        gate_rows(16 * (i * NB + j), r[ANCH:ANCH + 8, 128 * j:128 * (j + 1)])
            groups = list(range(0, TB, RG))
            nslots = 2 * (NF - NFA) - NSK
            hs = []
            slot = 0
            done = 0
            last = []

            def release(anchor):
                nonlocal slot, done
                slot += 1
                want = min(len(groups), -(-slot * len(groups) // nslots))
                if want > done:
                    for r0 in groups[done:want]:
                        dep = pltpu.bitcast(anchor, i32)
                        dep = dep | pltpu.bitcast(gates[r0 // 16][r0 % 16:r0 % 16 + 8], i32)
                        if last:
                            dep = dep | pltpu.bitcast(last[-1], i32)
                        last.append(attend(r0, base, pltpu.bitcast(sbits | (dep & zvec), f32), zvec))
                    done = want

            for c in range(0, FB, 256):
                g = _dot(x, wg_v[:, pl.ds(c, 256)])
                for n in range(2):
                    release(g[ANCH:ANCH + 8, 128 * n:128 * (n + 1)])
                u = _dot(x, wu_v[:, pl.ds(c, 256)])
                for n in range(2):
                    release(u[ANCH:ANCH + 8, 128 * n:128 * (n + 1)])
                hs.append(_reglu(g, u))
            assert done == len(groups)
            qkv_s[pl.ds(NB, 2 * NB), pl.ds(0, HALO), :] = qkv_s[pl.ds(NB, 2 * NB), pl.ds(TB, HALO), :]
            g = jnp.concatenate(gates, axis=0)
            g1 = 1.0 - g

            wo = _cat([jnp.concatenate([w_p[3, j, pl.ds(8 * m + c, 8, stride=PITCH), :]
                                        for c in range(8) for m in range(8)], axis=0)
                       for j in range(NB)])
            o_s[0, pl.ds(TB + zero, 8), :] = jnp.zeros((8, 128), f32)
            o = jnp.concatenate([o_s[j, pl.ds(0, TB), :] for j in range(NB)], axis=1)
            a = _dot(o.astype(bf16), wo)
            b = (bacc[0, pl.ds(base, TB), :] + bacc[1, pl.ds(base, TB), :]
                 + _dot(_hcat(hs), wd_v[...]))
            for r0, r1, c0, c1 in OUTP:
                n = c1 - c0
                res = (jnp.concatenate([g[r0:r1]] * (n // 128), axis=1) * a[r0:r1, c0:c1]
                       + jnp.concatenate([g1[r0:r1]] * (n // 128), axis=1) * b[r0:r1, c0:c1])
                rs = pl.ds(pl.multiple_of(base + r0, 16), r1 - r0)
                out_v[rs, pl.ds(c0, n)] = res.astype(bf16)
                start(out_v.at[rs, pl.ds(c0, n)], out_hbm.at[rs, pl.ds(c0, n)], 10)
            return carry

        jax.lax.fori_loop(0, S // TB, phase_b, 0)
        return carry0

    jax.lax.fori_loop(0, zero_s[0] + 1, main, 0)
    wait(10, out_v)


@jax.jit
def pallas_gated_mix__sliding_local_dilated__glu_gated_reglu__prompt_kernel(
    A_x: jax.Array,
    A_wqkv: jax.Array,
    A_wo: jax.Array,
    B_x: jax.Array,
    B_W_gate: jax.Array,
    B_W_up: jax.Array,
    B_W_down: jax.Array,
    gate_w: jax.Array,
):
    del B_x
    x = A_x.reshape(S, D)
    hbm = pl.BlockSpec(memory_space=pl.ANY)
    out = pl.pallas_call(
        _kernel,
        out_shape=jax.ShapeDtypeStruct((S, D), bf16),
        in_specs=[hbm] * 7,
        out_specs=hbm,
        scratch_shapes=[
            pltpu.VMEM((S, D), bf16),
            pltpu.VMEM((4, D, D), bf16),
            pltpu.VMEM((2, D, 128 * BA), bf16),
            pltpu.VMEM((2, D, 128 * BA), bf16),
            pltpu.VMEM((128 * NFA, D), bf16),
            pltpu.VMEM((D, FB), bf16),
            pltpu.VMEM((D, FB), bf16),
            pltpu.VMEM((FB, D), bf16),
            pltpu.VMEM((D,), bf16),
            pltpu.VMEM((4, NB, 8 * PITCH + 64, 128), u32),
            pltpu.VMEM((2, S, D), f32),
            pltpu.VMEM((3 * NB, HALO + TB + 8, 128), f32),
            pltpu.VMEM((NB, TB + 8, 128), f32),
            pltpu.VMEM((S, D), bf16),
            pltpu.SMEM((1,), i32),
            pltpu.SemaphoreType.DMA((11,)),
        ],
        compiler_params=pltpu.CompilerParams(
            vmem_limit_bytes=110 * 1024 * 1024,
            disable_bounds_checks=True,
            disable_semaphore_checks=True,
        ),
    )(x, A_wqkv, A_wo, B_W_gate, B_W_up, B_W_down, gate_w)
    return out.reshape(1, S, D)
```

```python
import jax
import jax.numpy as jnp
import jax.experimental.pallas as pl
import jax.experimental.pallas.tpu as pltpu

S, D, F = 2048, 1024, 3584
H, DH, WIN, DIL = 32, 32, 8, 2
NB = D // 128
NF = F // 128
HALO = 16
BA = 3
NFA = 2 * BA
FB = F - 128 * NFA
R0 = 704
NA = 4
UR = (2 * S - R0) // NA
SUB = (0, (S - R0) % UR, UR)
CPU = 9
NCH = 4 * 8
COFF = NA * CPU - NCH
CH1 = max(CPU - COFF, 1)
KS = (0, 256, 512, 768, 1024)
X1 = 256
PITCH = 65
TB = 256
RG = 8
ANCH = 56
NSK = 4
LGS = 4
PVS = 2
OUTP = ((0, 256, 0, 512), (0, 256, 512, 896), (0, 160, 896, 1024), (160, 240, 896, 1024),
        (240, 256, 896, 1024))
LOG2E = 1.4426950408889634
SCALE = DH ** -0.5 * LOG2E
NEG = -1e9 * LOG2E

f32 = jnp.float32
bf16 = jnp.bfloat16
u32 = jnp.uint32
i32 = jnp.int32


def _dot(a, b):
    return jnp.dot(a, b, preferred_element_type=f32)


def _lane(shape):
    return jax.lax.broadcasted_iota(i32, shape, 1)


def _cat(blocks):
    return jnp.concatenate([pltpu.bitcast(b, bf16) for b in blocks], axis=1)


def _reglu(g, u):
    return jnp.maximum(g, 0.0) * u


def _hcat(hs):
    return jnp.concatenate(hs, axis=1).astype(bf16)


def _kernel(x_hbm, wqkv_hbm, wo_hbm, wg_hbm, wu_hbm, wd_hbm, gw_hbm, out_hbm,
            x_v, w_v, wga_v, wua_v, wda_v, wg_v, wu_v, wd_v, gw_v, w_p, bacc,
            qkv_s, o_s, out_v, zero_s, sems):
    def start(src, dst, grp):
        pltpu.make_async_copy(src, dst, sems.at[grp]).start()

    def wait(grp, *dsts):
        for d in dsts:
            pltpu.make_async_copy(d, d, sems.at[grp]).wait()

    def xrows(a, n):
        return x_v.at[pl.ds(a, n), :]

    def get_x(a, n, grp):
        start(x_hbm.at[pl.ds(a, n), :], xrows(a, n), grp)

    def wda_rows(b0, b1):
        return wda_v.at[pl.ds(128 * b0, 128 * (b1 - b0)), :]

    def get_wda(b0, b1, grp):
        start(wd_hbm.at[pl.ds(128 * b0, 128 * (b1 - b0)), :], wda_rows(b0, b1), grp)

    def w_rows(c0, c1):
        out = []
        for p in range(4):
            a, b = max(c0, 8 * p), min(c1, 8 * p + 8)
            if a < b:
                out.append((p, 128 * (a - 8 * p), 128 * (b - a)))
        return out

    def w_dst(c0, c1):
        return [w_v.at[p, pl.ds(r, n), :] for p, r, n in w_rows(c0, c1)]

    def get_w(c0, c1, grp):
        for p, r, n in w_rows(c0, c1):
            src = (wqkv_hbm.at[pl.ds(r, n), pl.ds(p * D, D)] if p < 3
                   else wo_hbm.at[pl.ds(r, n), :])
            start(src, w_v.at[p, pl.ds(r, n), :], grp)

    def xpart(r0, r1, k):
        sl = (pl.ds(r0, r1 - r0), pl.ds(KS[k], KS[k + 1] - KS[k]))
        return x_hbm.at[sl], x_v.at[sl]

    def wpart(hbm, buf, k, b0=0, b1=BA):
        sl = (pl.ds(KS[k], KS[k + 1] - KS[k]), pl.ds(128 * b0, 128 * (b1 - b0)))
        return hbm.at[sl], buf.at[(0,) + sl]

    p0 = [[xpart(0, X1, 0), wpart(wg_hbm, wga_v, 0, 0, 2)], [xpart(X1, R0, 0)],
          [wpart(wg_hbm, wga_v, 0, 2, BA), wpart(wu_hbm, wua_v, 0)]]
    for k in range(1, len(KS) - 1):
        p0.append([xpart(0, R0, k), wpart(wg_hbm, wga_v, k), wpart(wu_hbm, wua_v, k)])
    p0[-1].append((wd_hbm.at[pl.ds(0, 128 * BA), :], wda_rows(0, BA)))
    for grp, pieces in enumerate(p0):
        for src, dst in pieces:
            start(src, dst, grp)
    ucross = (S - R0) // UR
    udst = []
    for u in range(3):
        dst = []
        x0, x1 = min(S, R0 + u * UR), (min(S, R0 + (u + 1) * UR) if u < 2 else S)
        if x0 < x1:
            get_x(x0, x1 - x0, 6 + u)
            dst.append(xrows(x0, x1 - x0))
        if u == min(ucross, 2):
            start(wg_hbm.at[:, pl.ds(128 * BA, 128 * BA)], wga_v.at[1], 6 + u)
            start(wu_hbm.at[:, pl.ds(128 * BA, 128 * BA)], wua_v.at[1], 6 + u)
            get_wda(BA, NFA, 6 + u)
            dst += [wga_v.at[1], wua_v.at[1], wda_rows(BA, NFA)]
        c0, c1 = (0, CH1, 2 * CPU - COFF, NCH)[u:u + 2]
        get_w(c0, c1, 6 + u)
        udst.append(dst + w_dst(c0, c1))
    start(gw_hbm, gw_v, 9)
    start(wd_hbm.at[pl.ds(128 * NFA, FB), :], wd_v, 9)
    start(wg_hbm.at[:, pl.ds(128 * NFA, FB)], wg_v, 9)
    start(wu_hbm.at[:, pl.ds(128 * NFA, FB)], wu_v, 9)

    zero_s[0] = 0
    qkv_s[pl.ds(NB, 2 * NB), pl.ds(0, HALO), :] = jnp.zeros((2 * NB, HALO, 128), f32)

    def repack(ch):
        p = jax.lax.shift_right_logical(ch, 3)
        rc = ch & 7
        on = jnp.where(ch < 24, -1, 0).astype(i32)
        r0 = pl.multiple_of(rc * 128, 128)
        blk = [pltpu.bitcast(w_v[p, pl.ds(r0, 128), pl.ds(128 * j, 128)], u32) for j in range(NB)]
        lane = _lane((64, 128))
        for bb, lb in ((2, 3), (1, 2), (0, 1)):
            sh = 1 << lb
            keep_a = (lane & (on & sh)) == 0
            take_a = ((lane & sh) | (~on & 1)) == 0
            for j in range(NB):
                if j & (1 << bb):
                    continue
                a, b = blk[j], blk[j | (1 << bb)]
                blk[j] = jnp.where(keep_a, a, pltpu.roll(b, sh, 1))
                blk[j | (1 << bb)] = jnp.where(take_a, pltpu.roll(a, 128 - sh, 1), b)
        for j in range(NB):
            w_p[p, j, pl.ds(rc * PITCH, 64), :] = blk[j]

    def main(_, carry0):
        def wait0(grp):
            wait(grp, *[dst for _, dst in p0[grp]])

        def xk(r0, r1, k):
            return x_v[pl.ds(r0, r1 - r0), pl.ds(KS[k], KS[k + 1] - KS[k])]

        def wk(buf, k, b0=0, b1=BA):
            return buf[0, pl.ds(KS[k], KS[k + 1] - KS[k]), pl.ds(128 * b0, 128 * (b1 - b0))]

        wait0(0)
        ga = _dot(xk(0, X1, 0), wk(wga_v, 0, 0, 2))
        wait0(1)
        gb = _dot(xk(X1, R0, 0), wk(wga_v, 0, 0, 2))
        wait0(2)
        gc = _dot(xk(0, R0, 0), jnp.concatenate([wk(wga_v, 0, 2, BA), wk(wua_v, 0)], axis=1))
        gu = jnp.concatenate([jnp.concatenate([ga, gb], axis=0), gc], axis=1)
        for k in range(1, len(KS) - 1):
            wait0(2 + k)
            d = _dot(xk(0, R0, k), jnp.concatenate([wk(wga_v, k), wk(wua_v, k)], axis=1))
            gu = jnp.concatenate([gu[:, :128 * BA] + d[:, :128 * BA],
                                  gu[:, 128 * BA:] + d[:, 128 * BA:]], axis=1)
        g, up = gu[:, :128 * BA], gu[:, 128 * BA:]
        bacc[0, pl.ds(0, R0), :] = _dot(_hcat([_reglu(g, up)]), wda_v[pl.ds(0, 128 * BA), :])

        def phase_a(u, carry):
            for k in range(3):
                pl.when(u == k)(lambda k=k: wait(6 + k, *udst[k]))
            parts = []
            for v0, v1 in zip(SUB[:-1], SUB[1:]):
                v = u * UR + v0
                c = (v >= S - R0).astype(i32)
                a = pl.multiple_of(v + R0 - c * S, 16)
                x = x_v[pl.ds(a, v1 - v0), :]
                h = _reglu(_dot(x, wga_v[c]), _dot(x, wua_v[c]))
                parts.append((c, a, v1 - v0, h))
            for k in range(CPU):
                repack(jnp.maximum(CPU * u + k - COFF, 0))
            for c, a, n, h in parts:
                r = pl.multiple_of(c * (128 * BA), 128)
                bacc[c, pl.ds(a, n), :] = _dot(_hcat([h]), wda_v[pl.ds(r, 128 * BA), :])
            return carry

        jax.lax.fori_loop(0, NA, phase_a, 0)
        wait(9, gw_v, wg_v, wu_v, wd_v)

        m16 = (_lane((RG, 128)) & 16) == 0
        m1 = (_lane((RG, 128)) & 1) == 0

        def attend(r0, base, scale, zvec):
            logits = []
            for w in range(WIN):
                if w % LGS == 0:
                    if w:
                        scale = pltpu.bitcast(
                            pltpu.bitcast(scale, i32) | (pltpu.bitcast(raw, i32) & zvec), f32)
                    q = [qkv_s[j, pl.ds(HALO + r0, RG), :] * scale for j in range(NB)]
                off = HALO + r0 - DIL * w
                acc = q[0] * qkv_s[NB, pl.ds(off, RG), :]
                for j in range(1, NB):
                    acc = acc + q[j] * qkv_s[NB + j, pl.ds(off, RG), :]
                raw = acc
                acc = acc + jnp.where(m16, pltpu.roll(acc, 128 - 16, 1), pltpu.roll(acc, 16, 1))
                acc = acc + jnp.where(m1, pltpu.roll(acc, 128 - 1, 1), pltpu.roll(acc, 1, 1))
                if r0 < DIL * w:
                    pos = base + r0 + jax.lax.broadcasted_iota(i32, (RG, 128), 0)
                    acc = jnp.where(pos >= DIL * w, acc, NEG)
                logits.append(acc)
            m = logits[0]
            for w in range(1, WIN):
                m = jnp.maximum(m, logits[w])
            e = [jnp.exp2(l - m) for l in logits]
            s = e[0]
            for w in range(1, WIN):
                s = s + e[w]
            inv = pl.reciprocal(s, approx=True)
            inv = inv * (2.0 - s * inv)
            for j in range(NB):
                if j % PVS == 0:
                    if j:
                        inv = pltpu.bitcast(pltpu.bitcast(inv, i32) | (pltpu.bitcast(o, i32) & zvec), f32)
                    p = [x * inv for x in e]
                o = p[0] * qkv_s[2 * NB + j, pl.ds(HALO + r0, RG), :]
                for w in range(1, WIN):
                    o = o + p[w] * qkv_s[2 * NB + j, pl.ds(HALO + r0 - DIL * w, RG), :]
                o_s[j, pl.ds(r0, RG), :] = o
            return o

        def phase_b(t, carry):
            base = pl.multiple_of(t * TB, TB)
            zero = zero_s[0]
            zvec = jnp.full((RG, 128), zero, i32)
            sbits = pltpu.bitcast(jnp.full((RG, 128), SCALE, f32), i32)
            x = x_v[pl.ds(base, TB), :]
            gw = pltpu.bitcast(jnp.broadcast_to(gw_v[...].astype(f32).reshape(1, D), (8, D)), i32)

            gates = []

            def gate_rows(r0, anchor):
                dep = pltpu.bitcast(anchor, i32) & zvec
                xr = x[r0:r0 + 16, :].astype(f32)
                acc = None
                for j in range(NB):
                    w = pltpu.bitcast(gw[:, 128 * j:128 * (j + 1)] | dep, f32)
                    term = xr[:, 128 * j:128 * (j + 1)] * jnp.concatenate([w, w], axis=0)
                    acc = term if acc is None else acc + term
                z = jnp.sum(acc, axis=-1, keepdims=True)
                gates.append(jnp.broadcast_to(jax.nn.sigmoid(z), (16, 128)))

            for i in range(3):
                r = _dot(x, _cat([jnp.concatenate([w_p[i, j, pl.ds(PITCH * c, 64), :] for c in range(8)],
                                                  axis=0) for j in range(NB)]))
                for j in range(NB):
                    qkv_s[i * NB + j, pl.ds(HALO, TB), :] = r[:, 128 * j:128 * (j + 1)]
                    if i * NB + j < TB // 16:
                        gate_rows(16 * (i * NB + j), r[ANCH:ANCH + 8, 128 * j:128 * (j + 1)])
            groups = list(range(0, TB, RG))
            nslots = 2 * (NF - NFA) - NSK
            hs = []
            slot = 0
            done = 0
            last = []

            def release(anchor):
                nonlocal slot, done
                slot += 1
                want = min(len(groups), -(-slot * len(groups) // nslots))
                if want > done:
                    for r0 in groups[done:want]:
                        dep = pltpu.bitcast(anchor, i32)
                        dep = dep | pltpu.bitcast(gates[r0 // 16][r0 % 16:r0 % 16 + 8], i32)
                        if last:
                            dep = dep | pltpu.bitcast(last[-1], i32)
                        last.append(attend(r0, base, pltpu.bitcast(sbits | (dep & zvec), f32), zvec))
                    done = want

            for c in range(0, FB, 256):
                g = _dot(x, wg_v[:, pl.ds(c, 256)])
                for n in range(2):
                    release(g[ANCH:ANCH + 8, 128 * n:128 * (n + 1)])
                u = _dot(x, wu_v[:, pl.ds(c, 256)])
                for n in range(2):
                    release(u[ANCH:ANCH + 8, 128 * n:128 * (n + 1)])
                hs.append(_reglu(g, u))
            assert done == len(groups)
            qkv_s[pl.ds(NB, 2 * NB), pl.ds(0, HALO), :] = qkv_s[pl.ds(NB, 2 * NB), pl.ds(TB, HALO), :]
            g = jnp.concatenate(gates, axis=0)
            g1 = 1.0 - g

            wo = _cat([jnp.concatenate([w_p[3, j, pl.ds(8 * m + c, 8, stride=PITCH), :]
                                        for c in range(8) for m in range(8)], axis=0)
                       for j in range(NB)])
            o_s[0, pl.ds(TB + zero, 8), :] = jnp.zeros((8, 128), f32)
            o = jnp.concatenate([o_s[j, pl.ds(0, TB), :] for j in range(NB)], axis=1)
            a = _dot(o.astype(bf16), wo)
            b0 = bacc[0, pl.ds(base, TB), :] + bacc[1, pl.ds(base, TB), :]
            d = _dot(_hcat(hs), wd_v[...])
            for r0, r1, c0, c1 in OUTP:
                n = c1 - c0
                gg1 = jnp.concatenate([g1[r0:r1]] * (n // 128), axis=1)
                pre = (jnp.concatenate([g[r0:r1]] * (n // 128), axis=1) * a[r0:r1, c0:c1]
                       + gg1 * b0[r0:r1, c0:c1])
                res = pre + gg1 * d[r0:r1, c0:c1]
                rs = pl.ds(pl.multiple_of(base + r0, 16), r1 - r0)
                out_v[rs, pl.ds(c0, n)] = res.astype(bf16)
                start(out_v.at[rs, pl.ds(c0, n)], out_hbm.at[rs, pl.ds(c0, n)], 10)
            return carry

        jax.lax.fori_loop(0, S // TB, phase_b, 0)
        return carry0

    jax.lax.fori_loop(0, zero_s[0] + 1, main, 0)
    wait(10, out_v)


@jax.jit
def pallas_gated_mix__sliding_local_dilated__glu_gated_reglu__prompt_kernel(
    A_x: jax.Array,
    A_wqkv: jax.Array,
    A_wo: jax.Array,
    B_x: jax.Array,
    B_W_gate: jax.Array,
    B_W_up: jax.Array,
    B_W_down: jax.Array,
    gate_w: jax.Array,
):
    del B_x
    x = A_x.reshape(S, D)
    hbm = pl.BlockSpec(memory_space=pl.ANY)
    out = pl.pallas_call(
        _kernel,
        out_shape=jax.ShapeDtypeStruct((S, D), bf16),
        in_specs=[hbm] * 7,
        out_specs=hbm,
        scratch_shapes=[
            pltpu.VMEM((S, D), bf16),
            pltpu.VMEM((4, D, D), bf16),
            pltpu.VMEM((2, D, 128 * BA), bf16),
            pltpu.VMEM((2, D, 128 * BA), bf16),
            pltpu.VMEM((128 * NFA, D), bf16),
            pltpu.VMEM((D, FB), bf16),
            pltpu.VMEM((D, FB), bf16),
            pltpu.VMEM((FB, D), bf16),
            pltpu.VMEM((D,), bf16),
            pltpu.VMEM((4, NB, 8 * PITCH + 64, 128), u32),
            pltpu.VMEM((2, S, D), f32),
            pltpu.VMEM((3 * NB, HALO + TB + 8, 128), f32),
            pltpu.VMEM((NB, TB + 8, 128), f32),
            pltpu.VMEM((S, D), bf16),
            pltpu.SMEM((1,), i32),
            pltpu.SemaphoreType.DMA((11,)),
        ],
        compiler_params=pltpu.CompilerParams(
            vmem_limit_bytes=110 * 1024 * 1024,
            disable_bounds_checks=True,
            disable_semaphore_checks=True,
        ),
    )(x, A_wqkv, A_wo, B_W_gate, B_W_up, B_W_down, gate_w)
    return out.reshape(1, S, D)
```
